```python
import jax
import jax.numpy as jnp

def _softmax(x, axis=-1):
    return jax.nn.softmax(x, axis=axis)
def _gelu(x):
    return jax.nn.gelu(x, approximate=True)
def _silu(x):
    return jax.nn.silu(x)
def _sigmoid(x):
    return jax.nn.sigmoid(x)
def _layernorm(x, axis=-1, eps=1e-5):
    m = jnp.mean(x, axis=axis, keepdims=True)
    v = jnp.var(x, axis=axis, keepdims=True)
    return (x - m) / jnp.sqrt(v + eps)
def _scatter_add(tgt, idx, src, axis=0):
    return tgt.at[idx].add(src)
def _segment_sum(src, seg, n):
    return jax.ops.segment_sum(src, seg, n)
class _Rng:
    def __init__(self, key):
        self._k = key
    def _next(self):
        self._k, sub = jax.random.split(self._k)
        return sub
    def normal(self, shape):
        return jax.random.normal(self._next(), shape, dtype=jnp.bfloat16)
    def randint(self, lo, hi, shape):
        return jax.random.randint(self._next(), shape, lo, hi, dtype=jnp.int32)
    def uniform(self, shape, lo=0.0, hi=1.0):
        return jax.random.uniform(self._next(), shape, jnp.bfloat16, lo, hi)
    def permutation(self, n):
        return jax.random.permutation(self._next(), n)


kernel_name = 'recurrent_scan__linear_kernel_hedgehog__moe_arch_mod__prompt'

def setup_inputs():
    _rng = _Rng(jax.random.key(int.from_bytes(__import__("os").urandom(4), "little")))
    _w = (lambda a: (lambda t: t.astype(jnp.bfloat16) if jnp.issubdtype(t.dtype, jnp.floating) else t)(jnp.asarray(a)))
    def _A_setup():
        B, S, D, H = 1, 2048, 1024, 32
        Dh = D // H
        return {
            "x": _w((lambda *s: _rng.normal(s) * 0.05)(B, S, D)),
            "wqkv": _w((lambda *s: _rng.normal(s) * 0.05)(D, 3 * D)),
            "w_phi": _w((lambda *s: _rng.normal(s) * 0.05)(H, Dh, Dh) * (Dh ** -0.5)),
            "wo": _w((lambda *s: _rng.normal(s) * 0.05)(D, D)),
        }
    _A_in = _A_setup()

    def _B_setup():
        B, S, D, F, C = 1, 2048, 1024, 3584, 1
        return {
            "x": _w((lambda *s: _rng.normal(s) * 0.05)(B, S, D)),
            "w_r": _w((lambda *s: _rng.normal(s) * 0.05)(D)),
            "w_gate": _w((lambda *s: _rng.normal(s) * 0.05)(D, F)),
            "w_up": _w((lambda *s: _rng.normal(s) * 0.05)(D, F)),
            "w_down": _w((lambda *s: _rng.normal(s) * 0.05)(F, D)),
        }
    _B_in = _B_setup()

    return {
        "A_x": _A_in["x"],
        "A_wqkv": _A_in["wqkv"],
        "A_w_phi": _A_in["w_phi"],
        "A_wo": _A_in["wo"],
        "B_x": _B_in["x"],
        "B_w_r": _B_in["w_r"],
        "B_w_gate": _B_in["w_gate"],
        "B_w_up": _B_in["w_up"],
        "B_w_down": _B_in["w_down"],
    }

def reference(A_x, A_wqkv, A_w_phi, A_wo, B_x, B_w_r, B_w_gate, B_w_up, B_w_down):
    def _A_ref(x, wqkv, w_phi, wo):
        B, S, D = x.shape
        H = 32; Dh = D // H
        qkv = (lambda x, *d: x.transpose(*d))((x @ wqkv).reshape(B, S, 3, H, Dh), 2, 0, 3, 1, 4)
        q, k, v = qkv[0], qkv[1], qkv[2]
        pq = jnp.einsum("bhsd,hdf->bhsf", q, w_phi)
        pk = jnp.einsum("bhsd,hdf->bhsf", k, w_phi)
        phi_q = jnp.concatenate([_softmax(pq, axis=-1), _softmax(-pq, axis=-1)], axis=-1)
        phi_k = jnp.concatenate([_softmax(pk, axis=-1), _softmax(-pk, axis=-1)], axis=-1)
        kv = jnp.einsum("bhsf,bhsd->bhfd", phi_k, v)
        z  = jnp.einsum("bhsf->bhf", phi_k)
        num = jnp.einsum("bhqf,bhfd->bhqd", phi_q, kv)
        den = jnp.einsum("bhqf,bhf->bhq", phi_q, z)[..., None] + 1e-6
        o = num / den
        return (lambda x, *d: x.transpose(*d))(o, 0, 2, 1, 3).reshape(B, S, D) @ wo

    def _B_ref(x, w_r, w_gate, w_up, w_down):
        B, S, D = x.shape
        C = 1
        r = x @ w_r
        idx = jnp.argsort(-r, axis=-1)[:, :C]
        idx_e = jnp.repeat(idx.reshape(B, C, 1), D, axis=2)
        x_sel = jnp.take_along_axis(x, idx_e, axis=1)
        g = _silu(x_sel @ w_gate)
        u = x_sel @ w_up
        y = (g * u) @ w_down
        r_sel = _sigmoid(jnp.take_along_axis(r, idx, axis=1))
        y = y * r_sel.reshape(B, C, 1)
        b_off = (jnp.arange(B) * S).reshape(B, 1)
        flat_idx = (idx + b_off).reshape(B * C)
        zero = (x * 0.0).reshape(B * S, D)
        upd = _scatter_add(zero, flat_idx, y.reshape(B * C, D), axis=0)
        return x + upd.reshape(B, S, D)

    x = A_x
    xn = _layernorm(x, axis=-1)
    s = _A_ref(xn, A_wqkv, A_w_phi, A_wo)
    g = _silu(_B_ref(xn, B_w_r, B_w_gate, B_w_up, B_w_down))
    return x + s * g
```

```python
import jax
import jax.numpy as jnp
from jax import lax
import jax.experimental.pallas as pl
import jax.experimental.pallas.tpu as pltpu

S, D, H, DH, F = 2048, 1024, 32, 32, 3584
T = 256
NTILE = S // T
NPAIR = H // 2
PR = 2 * DH + 16
RB = 16
LOG2E = 1.4426950408889634
F32 = jnp.float32
BF16 = jnp.bfloat16


def _nt(a, b):
    return lax.dot_general(a, b, (((1,), (1,)), ((), ())), preferred_element_type=F32)


def _nn(a, b):
    return jnp.dot(a, b, preferred_element_type=F32)


def _rb(v):
    return v.astype(BF16).astype(F32)


def _sigmoid(v):
    return 0.5 * jnp.tanh(0.5 * v) + 0.5


def _dual_softmax_t(p):
    n = p.shape[-1]
    g = p.shape[0] // DH
    p3 = p.reshape(g, DH, n)
    mx = jnp.max(p3, axis=1, keepdims=True)
    mn = jnp.min(p3, axis=1, keepdims=True)
    ep = jnp.exp2(p3 - mx)
    en = jnp.exp2(mn - p3)
    rp = 1.0 / jnp.sum(ep, axis=1, keepdims=True)
    rn = 1.0 / jnp.sum(en, axis=1, keepdims=True)
    out = jnp.concatenate([ep * rp, en * rn], axis=1)
    return out.reshape(g * 2 * DH, n).astype(BF16)


def _kernel(x_hbm, wqkv_hbm, phi_hbm, wo_hbm, wr_hbm, wg_hbm, wu_hbm, wd_hbm, out_hbm,
            x_buf, xn_buf, gate_buf, out_buf, wraw, phi_buf, wr_buf, wo_buf, wg_buf, wu_buf, wd_buf,
            wq_t, wk_t, wv_t, phik, vaug, phiq, lmat, o_buf, r_buf,
            sem_x, sem_w, sem_o):
    def x_copy(i):
        return pltpu.make_async_copy(x_hbm.at[pl.ds(i * T, T)], x_buf.at[pl.ds(i * T, T)], sem_x.at[i])

    def out_copy(i):
        return pltpu.make_async_copy(out_buf.at[pl.ds(i * T, T)], out_hbm.at[pl.ds(i * T, T)], sem_o.at[i])

    def wqkv_copy(j):
        return pltpu.make_async_copy(wqkv_hbm.at[:, pl.ds(j * D, D)], wraw.at[j], sem_w.at[j])

    c_phi = pltpu.make_async_copy(phi_hbm, phi_buf, sem_w.at[3])
    c_wr = pltpu.make_async_copy(wr_hbm, wr_buf, sem_w.at[4])
    c_wo = pltpu.make_async_copy(wo_hbm, wo_buf, sem_w.at[5])
    c_wg = pltpu.make_async_copy(wg_hbm, wg_buf, sem_w.at[6])
    c_wu = pltpu.make_async_copy(wu_hbm, wu_buf, sem_w.at[7])
    c_wd = pltpu.make_async_copy(wd_hbm, wd_buf, sem_w.at[8])

    c_phi.start()
    c_wr.start()
    x_copy(0).start()
    wqkv_copy(1).start()
    x_copy(1).start()
    wqkv_copy(2).start()
    for i in range(2, NTILE):
        x_copy(i).start()
    wqkv_copy(0).start()
    c_wo.start()
    c_wg.start()
    c_wu.start()
    c_wd.start()

    for j in range(NPAIR):
        vaug[j, 2 * DH:PR, :] = jnp.ones((RB, S), BF16)

    c_phi.wait()
    c_wr.wait()
    phi2 = phi_buf[...].reshape(H * DH, DH)
    er = lax.broadcasted_iota(jnp.int32, (128, DH), 0)
    ec = lax.broadcasted_iota(jnp.int32, (128, DH), 1)
    eye4 = jnp.where((er % DH) == ec, 1.0, 0.0).astype(BF16)
    br = lax.broadcasted_iota(jnp.int32, (128, 128), 0) // DH
    bc = lax.broadcasted_iota(jnp.int32, (128, 128), 1) // DH
    bd = []
    for g in range(8):
        t = _nt(eye4, phi2[g * 128:(g + 1) * 128])
        bd.append(jnp.where(br == bc, t, 0.0).astype(BF16))

    wk_t[D:D + RB, :] = jnp.broadcast_to(
        wr_buf[...].reshape(1, D).astype(F32), (RB, D)).astype(BF16)

    def fold(j, dst):
        for g in range(8):
            w = wraw[j, :, g * 128:(g + 1) * 128]
            dst[g * 128:(g + 1) * 128, :] = (_nt(bd[g], w) * LOG2E).astype(BF16)

    def layernorm(i):
        rows = pl.ds(i * T, T)
        xf = x_buf[rows, :].astype(F32)
        mean = jnp.sum(xf, axis=-1, keepdims=True) * (1.0 / D)
        c = xf - mean
        var = jnp.sum(c * c, axis=-1, keepdims=True) * (1.0 / D)
        eps = _rb(jnp.full((1, 1), 1e-5, F32))
        sd = _rb(jnp.sqrt(_rb(_rb(var) + eps)))
        xn = (_rb(xf - _rb(mean)) * (1.0 / sd)).astype(BF16)
        xn_buf[rows, :] = xn
        xnf = xn.astype(F32)
        gate_buf[rows, :] = (xnf * _sigmoid(xnf)).astype(BF16)

    def stage_k(i):
        cols = pl.ds(i * T, T)
        pt = _nt(wk_t[...], xn_buf[cols, :])
        r_buf[:, cols] = pt[D:D + 8, :]
        phik[:, cols] = _dual_softmax_t(pt[:D, :])

    def stage_v(i):
        cols = pl.ds(i * T, T)
        vt = _nt(wv_t[...], xn_buf[cols, :]).astype(BF16)
        for j in range(NPAIR):
            vaug[j, 0:2 * DH, cols] = vt[j * 2 * DH:(j + 1) * 2 * DH, :]

    def stage_q(i):
        cols = pl.ds(i * T, T)
        phiq[...] = _dual_softmax_t(_nt(wq_t[...], xn_buf[cols, :]))

    def stage_kv():
        lr = lax.broadcasted_iota(jnp.int32, (PR, 128), 0)
        lc = lax.broadcasted_iota(jnp.int32, (PR, 128), 1) // (2 * DH)
        rh = jnp.where(lr < 2 * DH, lr // DH, (lr - 2 * DH) // 8)
        keep = rh == lc
        for j in range(NPAIR):
            kvt = _nt(vaug[j], phik[j * 128:(j + 1) * 128, :])
            lmat[j] = jnp.where(keep, kvt, 0.0).astype(BF16)

    def stage_b():
        for g in range(8):
            parts = []
            for j in (2 * g, 2 * g + 1):
                nt = _nn(lmat[j], phiq[j * 128:(j + 1) * 128, :])
                for hl in range(2):
                    den = nt[2 * DH + 8 * hl:2 * DH + 8 * hl + 8, :] + 1e-6
                    num = nt[hl * DH:(hl + 1) * DH, :].reshape(4, 8, T)
                    parts.append((num * (1.0 / den)[None]).reshape(DH, T))
            ot = jnp.concatenate(parts, axis=0)
            o_buf[:, g * 128:(g + 1) * 128] = ot.T.astype(BF16)

    def stage_c(i):
        rows = pl.ds(i * T, T)
        s = _nn(o_buf[...], wo_buf[...])
        res = x_buf[rows, :].astype(F32) + s * gate_buf[rows, :].astype(F32)
        out_buf[rows, :] = res.astype(BF16)
        out_copy(i).start()

    def stage_ffn():
        r = _rb(r_buf[0:1, :])
        rmax = jnp.max(r)
        pos = lax.broadcasted_iota(jnp.int32, (1, S), 1)
        idx = jnp.min(jnp.where(r == rmax, pos, S))
        idx = jnp.clip(idx, 0, S - 1)
        blk = pl.multiple_of((idx // RB) * RB, RB)
        xs = xn_buf[pl.ds(blk, RB), :]
        hg = _rb(_nn(xs, wg_buf[...]))
        hu = _rb(_nn(xs, wu_buf[...]))
        act = (_rb(hg * _sigmoid(hg)) * hu).astype(BF16)
        y = _rb(_nn(act, wd_buf[...]))
        rs = _rb(_sigmoid(jnp.full((1, 1), rmax, F32)))
        y = _rb(y * rs)
        row = lax.broadcasted_iota(jnp.int32, (RB, D), 0) + blk
        b = _rb(xs.astype(F32) + jnp.where(row == idx, y, 0.0))
        gate_buf[pl.ds(blk, RB), :] = (b * _sigmoid(b)).astype(BF16)

    x_copy(0).wait()
    layernorm(0)
    wqkv_copy(1).wait()
    fold(1, wk_t)
    x_copy(1).wait()
    layernorm(1)
    stage_k(0)
    wqkv_copy(2).wait()
    for g in range(8):
        wv_t[g * 128:(g + 1) * 128, :] = wraw[2, :, g * 128:(g + 1) * 128].T
    stage_k(1)
    for i in range(2, NTILE):
        x_copy(i).wait()
    layernorm(2)
    stage_v(0)
    stage_v(1)
    for i in range(2, NTILE):
        if i + 1 < NTILE:
            layernorm(i + 1)
        stage_k(i)
        if i == NTILE - 2:
            wqkv_copy(0).wait()
            fold(0, wq_t)
        stage_v(i)

    stage_q(0)
    stage_kv()
    c_wo.wait()
    c_wg.wait()
    c_wu.wait()
    c_wd.wait()
    stage_ffn()

    for i in range(NTILE):
        stage_b()
        if i + 1 < NTILE:
            stage_q(i + 1)
        stage_c(i)

    for i in range(NTILE):
        out_copy(i).wait()


@jax.jit
def pallas_recurrent_scan__linear_kernel_hedgehog__moe_arch_mod__prompt_kernel(
    A_x: jax.Array,
    A_wqkv: jax.Array,
    A_w_phi: jax.Array,
    A_wo: jax.Array,
    B_x: jax.Array,
    B_w_r: jax.Array,
    B_w_gate: jax.Array,
    B_w_up: jax.Array,
    B_w_down: jax.Array,
):
    del B_x
    x2 = A_x.reshape(S, D)
    any_spec = pl.BlockSpec(memory_space=pl.ANY)
    scratch = [
        pltpu.VMEM((S, D), BF16),
        pltpu.VMEM((S, D), BF16),
        pltpu.VMEM((S, D), BF16),
        pltpu.VMEM((S, D), BF16),
        pltpu.VMEM((3, D, D), BF16),
        pltpu.VMEM((H, DH, DH), BF16),
        pltpu.VMEM((D,), BF16),
        pltpu.VMEM((D, D), BF16),
        pltpu.VMEM((D, F), BF16),
        pltpu.VMEM((D, F), BF16),
        pltpu.VMEM((F, D), BF16),
        pltpu.VMEM((D, D), BF16),
        pltpu.VMEM((D + RB, D), BF16),
        pltpu.VMEM((D, D), BF16),
        pltpu.VMEM((2 * D, S), BF16),
        pltpu.VMEM((NPAIR, PR, S), BF16),
        pltpu.VMEM((2 * D, T), BF16),
        pltpu.VMEM((NPAIR, PR, 128), BF16),
        pltpu.VMEM((T, D), BF16),
        pltpu.VMEM((8, S), F32),
        pltpu.SemaphoreType.DMA((NTILE,)),
        pltpu.SemaphoreType.DMA((9,)),
        pltpu.SemaphoreType.DMA((NTILE,)),
    ]
    out = pl.pallas_call(
        _kernel,
        out_shape=jax.ShapeDtypeStruct((S, D), BF16),
        in_specs=[any_spec] * 8,
        out_specs=any_spec,
        scratch_shapes=scratch,
        compiler_params=pltpu.CompilerParams(vmem_limit_bytes=100 * 1024 * 1024),
        name="hedgehog_mod",
    )(x2, A_wqkv, A_w_phi, A_wo, B_w_r, B_w_gate, B_w_up, B_w_down)
    return out.reshape(1, S, D)
```

```python
import functools

import jax
import jax.numpy as jnp
from jax import lax
import jax.experimental.pallas as pl
import jax.experimental.pallas.tpu as pltpu

D, H, DH, F = 1024, 32, 32, 3584
LANE = 128
KB = D // LANE
T = 256
TB = T // LANE
NPAIR = H // 2
PR = 2 * DH + 16
RB = 16
WDP = D + LANE
LOG2E = 1.4426950408889634
F32 = jnp.float32
BF16 = jnp.bfloat16
U32 = jnp.uint32

CFG = dict(S=2048, KQ=4, p1_barrier=False, p2_barrier=False, ln_chunk=16)


def _nt(a, b):
    return lax.dot_general(a, b, (((1,), (1,)), ((), ())), preferred_element_type=F32)


def _nn(a, b):
    return jnp.dot(a, b, preferred_element_type=F32)


def _rb(v):
    return v.astype(BF16).astype(F32)


def _recip(v):
    return pl.reciprocal(v, approx=True)


def _recip_nr(v):
    r = pl.reciprocal(v, approx=True)
    return r * (2.0 - v * r)


def _sigmoid(v):
    return 0.5 * jnp.tanh(0.5 * v) + 0.5


def _cat(parts):
    return jnp.concatenate(parts, axis=1)


def _pk(v):
    return pltpu.bitcast(v, U32)


def _up(v):
    return pltpu.bitcast(v, BF16)


def _pair_allreduce(v, op):
    v = op(v, pltpu.roll(v, 2, 1))
    return op(v, pltpu.roll(v, 4, 1))


def _dual_softmax_t(p):
    n = p.shape[-1]
    g = p.shape[0] // (2 * DH)
    p4 = p.reshape(g, 8, 8, n)
    mx = _pair_allreduce(jnp.max(p4, axis=1), jnp.maximum)[:, None]
    mn = _pair_allreduce(jnp.min(p4, axis=1), jnp.minimum)[:, None]
    ep = jnp.exp2(p4 - mx)
    en = jnp.exp2(mn - p4)
    rp = _recip(_pair_allreduce(jnp.sum(ep, axis=1), jnp.add))[:, None]
    rn = _recip(_pair_allreduce(jnp.sum(en, axis=1), jnp.add))[:, None]
    out = jnp.concatenate([ep * rp, en * rn], axis=1)
    return out.reshape(g * LANE, n).astype(BF16)


def _kernel(cfg, x_hbm, wqkv_hbm, phi_hbm, wo_hbm, wr_hbm, wg_hbm, wu_hbm, wd_hbm, out_hbm,
            x_buf, xn3, out_buf, wraw, phi_buf, wr_buf, wo_buf, wg_buf, wu_buf, wd_buf,
            wq3, wk3, wv3, wo3, phik3, vaug3, phiq3, lmat, o3, r_buf, bsel_buf,
            sem, sem_o):
    S = cfg["S"]
    KQ = cfg["KQ"]
    NB = S // LANE
    NTILE = S // T
    s_phi, s_wr, s_wv, s_wq, s_wo, s_wg, s_wu, s_wd, s_wk, s_x = 0, 1, 2, 3, 4, 5, 6, 7, 8, 16

    def x_copy(i):
        return pltpu.make_async_copy(x_hbm.at[pl.ds(i * T, T)], x_buf.at[pl.ds(i * T, T)], sem.at[s_x + i])

    def out_copy(i):
        return pltpu.make_async_copy(out_buf.at[pl.ds(i * T, T)], out_hbm.at[pl.ds(i * T, T)], sem_o.at[i])

    kw = D // KQ

    def wk_copy(c):
        return pltpu.make_async_copy(wqkv_hbm.at[:, pl.ds(D + c * kw, kw)],
                                     wraw.at[1, :, pl.ds(c * kw, kw)], sem.at[s_wk + c])

    c_wv = pltpu.make_async_copy(wqkv_hbm.at[:, pl.ds(2 * D, D)], wraw.at[2], sem.at[s_wv])
    c_wq = pltpu.make_async_copy(wqkv_hbm.at[:, pl.ds(0, D)], wraw.at[0], sem.at[s_wq])
    c_phi = pltpu.make_async_copy(phi_hbm, phi_buf, sem.at[s_phi])
    c_wr = pltpu.make_async_copy(wr_hbm, wr_buf, sem.at[s_wr])
    c_wo = pltpu.make_async_copy(wo_hbm, wo_buf, sem.at[s_wo])
    c_wg = pltpu.make_async_copy(wg_hbm, wg_buf, sem.at[s_wg])
    c_wu = pltpu.make_async_copy(wu_hbm, wu_buf, sem.at[s_wu])
    c_wd = pltpu.make_async_copy(wd_hbm, wd_buf.at[:, pl.ds(0, D)], sem.at[s_wd])

    c_phi.start()
    c_wr.start()
    x_copy(0).start()
    for c in range(KQ):
        wk_copy(c).start()
    x_copy(1).start()
    x_copy(2).start()
    c_wv.start()
    for i in range(3, NTILE):
        x_copy(i).start()
    c_wq.start()
    c_wo.start()
    c_wg.start()
    c_wu.start()
    c_wd.start()

    ones = _pk(jnp.ones((RB, LANE), BF16))
    for b in range(NB):
        for j in range(NPAIR):
            vaug3[b, (j * PR + 2 * DH) // 2:(j + 1) * PR // 2, :] = ones

    c_phi.wait()
    c_wr.wait()
    phi2 = phi_buf[...].reshape(H * DH, DH)
    er = lax.broadcasted_iota(jnp.int32, (LANE, DH), 0)
    ec = lax.broadcasted_iota(jnp.int32, (LANE, DH), 1)
    eye4 = jnp.where((er % (2 * DH)) // 2 == ec, 1.0, 0.0).astype(BF16)
    br = lax.broadcasted_iota(jnp.int32, (LANE, LANE), 0)
    bc = lax.broadcasted_iota(jnp.int32, (LANE, LANE), 1)
    bmask = (2 * (br // (2 * DH)) + br % 2) == bc // DH
    bd = []
    for g in range(KB):
        t = _nt(eye4, phi2[g * LANE:(g + 1) * LANE])
        bd.append(jnp.where(bmask, t, 0.0).astype(BF16))

    wrf = wr_buf[...].reshape(1, D).astype(F32)
    for k in range(KB):
        wk3[k, D // 2:(D + RB) // 2, :] = _pk(
            jnp.broadcast_to(wrf[:, k * LANE:(k + 1) * LANE], (RB, LANE)).astype(BF16))

    def put_rows(dst, r0, val):
        n = val.shape[0]
        for k in range(KB):
            dst[k, r0 // 2:(r0 + n) // 2, :] = _pk(val[:, k * LANE:(k + 1) * LANE])

    def get_rows(src, r0, n):
        return _cat([_up(src[k, pl.ds(r0 // 2, n // 2), :]) for k in range(KB)])

    def fold(j, dst, g0, g1):
        for g in range(g0, g1):
            w = wraw[j, :, g * LANE:(g + 1) * LANE]
            put_rows(dst, g * LANE, (_nt(bd[g], w) * LOG2E).astype(BF16))

    def layernorm(i, ch):
        z = None
        eps = _rb(jnp.full((1, 1), 1e-5, F32))
        for r0 in range(i * T, (i + 1) * T, ch):
            xf = x_buf[r0:r0 + ch, :].astype(F32)
            mean = jnp.sum(xf, axis=-1, keepdims=True) * (1.0 / D)
            if z is not None:
                mean = mean + z
            c = xf - mean
            var = jnp.sum(c * c, axis=-1, keepdims=True) * (1.0 / D)
            rs = _recip_nr(_rb(jnp.sqrt(_rb(_rb(var) + eps))))
            z = jnp.where(rs < 0.0, 1.0, 0.0)
            put_rows(xn3, r0, (_rb(xf - _rb(mean)) * rs).astype(BF16))

    def stage_k(i, r0=0, r1=D):
        last = r1 == D
        for b in range(i * TB, (i + 1) * TB):
            pt = _nt(get_rows(wk3, r0, r1 - r0 + (RB if last else 0)), get_rows(xn3, b * LANE, LANE))
            if last:
                r_buf[:, b * LANE:(b + 1) * LANE] = pt[r1 - r0:r1 - r0 + 8, :]
            phik3[b, r0:r1, :] = _pk(_dual_softmax_t(pt[:r1 - r0, :]))

    def stage_v(i):
        for b in range(i * TB, (i + 1) * TB):
            vt = _nt(get_rows(wv3, 0, D), get_rows(xn3, b * LANE, LANE)).astype(BF16)
            for j in range(NPAIR):
                vaug3[b, j * PR // 2:j * PR // 2 + DH, :] = _pk(vt[j * 2 * DH:(j + 1) * 2 * DH, :])

    def stage_q(i):
        for bl in range(TB):
            b = i * TB + bl
            phiq3[bl] = _pk(_dual_softmax_t(_nt(get_rows(wq3, 0, D), get_rows(xn3, b * LANE, LANE))))

    def stage_kv():
        lr = lax.broadcasted_iota(jnp.int32, (PR, LANE), 0)
        lc = lax.broadcasted_iota(jnp.int32, (PR, LANE), 1) % 2
        rh = jnp.where(lr < 2 * DH, lr // DH, (lr - 2 * DH) // 8)
        keep = rh == lc
        for j in range(NPAIR):
            va = _cat([_up(vaug3[b, j * PR // 2:(j + 1) * PR // 2, :]) for b in range(NB)])
            pk = _cat([_up(phik3[b, j * 64:(j + 1) * 64, :]) for b in range(NB)])
            lmat[j] = _pk(jnp.where(keep, _nt(va, pk), 0.0).astype(BF16))

    def stage_b():
        for g in range(KB):
            parts = []
            for j in (2 * g, 2 * g + 1):
                pq = _cat([_up(phiq3[bl, j * 64:(j + 1) * 64, :]) for bl in range(TB)])
                nt = _nn(_up(lmat[j]), pq)
                for hl in range(2):
                    den = nt[2 * DH + 8 * hl:2 * DH + 8 * hl + 8, :] + 1e-6
                    num = nt[hl * DH:(hl + 1) * DH, :].reshape(4, 8, T)
                    parts.append((num * _recip(den)[None]).reshape(DH, T))
            ot = jnp.concatenate(parts, axis=0)
            o3[g] = _pk(ot.T.astype(BF16))

    def stage_c(i, idx):
        r0 = i * T
        o = get_rows(o3, 0, T)
        sel = (lax.broadcasted_iota(jnp.int32, (T, 2 * LANE), 0) + r0) == idx
        for n in range(0, KB, 2):
            s = _nn(o, _cat([_up(wo3[n]), _up(wo3[n + 1])]))
            cols = slice(n * LANE, (n + 2) * LANE)
            xn = _cat([_up(xn3[m, r0 // 2:(r0 + T) // 2, :]) for m in (n, n + 1)]).astype(F32)
            b = jnp.where(sel, bsel_buf[0:1, cols], xn)
            res = x_buf[r0:r0 + T, cols].astype(F32) + s * (b * _sigmoid(b))
            out_buf[r0:r0 + T, cols] = res.astype(BF16)
        out_copy(i).start()

    def route():
        r = _rb(r_buf[0:1, :])
        rmax = jnp.max(r)
        pos = lax.broadcasted_iota(jnp.int32, (1, S), 1)
        idx = jnp.min(jnp.where(r == rmax, pos, S))
        return jnp.clip(idx, 0, S - 1), rmax

    def stage_ffn(idx, rmax):
        blk2 = pl.multiple_of((idx // RB) * (RB // 2), RB // 2)
        xs = _cat([_up(xn3[k, pl.ds(blk2, RB // 2), :]) for k in range(KB)])
        hg = _rb(_nn(xs, wg_buf[...]))
        hu = _rb(_nn(xs, wu_buf[...]))
        act = (_rb(hg * _sigmoid(hg)) * hu).astype(BF16)
        y = _rb(_nn(act, wd_buf[:, 0:D]))
        rs = _rb(_sigmoid(jnp.full((1, 1), rmax, F32)))
        b = _rb(xs.astype(F32) + _rb(y * rs))
        row = lax.broadcasted_iota(jnp.int32, (RB, D), 0) + 2 * blk2
        bsel = jnp.sum(jnp.where(row == idx, b, 0.0), axis=0, keepdims=True)
        bsel_buf[...] = jnp.broadcast_to(bsel, (8, D))

    lc = cfg["ln_chunk"]
    gq = KB // KQ
    x_copy(0).wait()
    layernorm(0, T)
    for c in range(KQ):
        wk_copy(c).wait()
        if c == KQ - 1:
            x_copy(1).wait()
            layernorm(1, 32)
        fold(1, wk3, c * gq, (c + 1) * gq)
        stage_k(0, c * kw, (c + 1) * kw)
    x_copy(2).wait()
    layernorm(2, lc)
    stage_k(1)
    c_wv.wait()
    x_copy(3).wait()
    if not cfg["p1_barrier"]:
        for i in range(4, NTILE):
            x_copy(i).wait()
    for g in range(KB):
        put_rows(wv3, g * LANE, wraw[2, :, g * LANE:(g + 1) * LANE].T)
    stage_k(2)
    stage_v(0)
    stage_v(1)
    layernorm(3, lc)
    stage_v(2)
    for i in range(3, NTILE):
        if cfg["p1_barrier"] and i + 1 < NTILE:
            x_copy(i + 1).wait()
        stage_k(i)
        if i + 1 < NTILE:
            layernorm(i + 1, lc)
        stage_v(i)

    c_wq.wait()
    c_wo.wait()
    c_wg.wait()
    c_wu.wait()
    c_wd.wait()
    idx, rmax = route()
    fold(0, wq3, 0, KB)
    put_rows(wo3, 0, wo_buf[...])
    stage_kv()
    stage_q(0)
    stage_ffn(idx, rmax)

    waited = 0
    for i in range(NTILE):
        if cfg["p2_barrier"] and i >= 2:
            out_copy(i - 2).wait()
            waited = i - 1
        stage_b()
        if i + 1 < NTILE:
            stage_q(i + 1)
        stage_c(i, idx)

    for i in range(waited, NTILE):
        out_copy(i).wait()


def _build(cfg):
    S = cfg["S"]
    NB = S // LANE
    NTILE = S // T
    any_spec = pl.BlockSpec(memory_space=pl.ANY)
    scratch = [
        pltpu.VMEM((S, D), BF16),
        pltpu.VMEM((KB, S // 2, LANE), U32),
        pltpu.VMEM((S, D), BF16),
        pltpu.VMEM((3, D, D), BF16),
        pltpu.VMEM((H, DH, DH), BF16),
        pltpu.VMEM((D,), BF16),
        pltpu.VMEM((D, D), BF16),
        pltpu.VMEM((D, F), BF16),
        pltpu.VMEM((D, F), BF16),
        pltpu.VMEM((F, WDP), BF16),
        pltpu.VMEM((KB, D // 2, LANE), U32),
        pltpu.VMEM((KB, (D + RB) // 2, LANE), U32),
        pltpu.VMEM((KB, D // 2, LANE), U32),
        pltpu.VMEM((KB, D // 2, LANE), U32),
        pltpu.VMEM((NB, D, LANE), U32),
        pltpu.VMEM((NB, NPAIR * PR // 2, LANE), U32),
        pltpu.VMEM((TB, D, LANE), U32),
        pltpu.VMEM((NPAIR, PR // 2, LANE), U32),
        pltpu.VMEM((KB, T // 2, LANE), U32),
        pltpu.VMEM((8, S), F32),
        pltpu.VMEM((8, D), F32),
        pltpu.SemaphoreType.DMA((32,)),
        pltpu.SemaphoreType.DMA((NTILE,)),
    ]
    return pl.pallas_call(
        functools.partial(_kernel, cfg),
        out_shape=jax.ShapeDtypeStruct((S, D), BF16),
        in_specs=[any_spec] * 8,
        out_specs=any_spec,
        scratch_shapes=scratch,
        compiler_params=pltpu.CompilerParams(vmem_limit_bytes=100 * 1024 * 1024),
        name=cfg.get("name", "hedgehog_mod"),
    )


@jax.jit
def pallas_recurrent_scan__linear_kernel_hedgehog__moe_arch_mod__prompt_kernel(
    A_x: jax.Array,
    A_wqkv: jax.Array,
    A_w_phi: jax.Array,
    A_wo: jax.Array,
    B_x: jax.Array,
    B_w_r: jax.Array,
    B_w_gate: jax.Array,
    B_w_up: jax.Array,
    B_w_down: jax.Array,
):
    del B_x
    S = CFG["S"]
    out = _build(CFG)(A_x.reshape(S, D), A_wqkv, A_w_phi, A_wo, B_w_r, B_w_gate, B_w_up, B_w_down)
    return out.reshape(1, S, D)
```

```python
import functools

import jax
import jax.numpy as jnp
from jax import lax
import jax.experimental.pallas as pl
import jax.experimental.pallas.tpu as pltpu

D, H, DH, F = 1024, 32, 32, 3584
LANE = 128
KB = D // LANE
T = 256
TB = T // LANE
NPAIR = H // 2
PR = 2 * DH + 16
RB = 16
WDP = D + LANE
LOG2E = 1.4426950408889634
F32 = jnp.float32
BF16 = jnp.bfloat16
U32 = jnp.uint32

CFG = dict(S=2048, KQ=4, ln_chunk=16, opq="pskv", nch=4, k0_inline=False, q_inline=(0, 1))


def _nt(a, b):
    return lax.dot_general(a, b, (((1,), (1,)), ((), ())), preferred_element_type=F32)


def _nn(a, b):
    return jnp.dot(a, b, preferred_element_type=F32)


def _rb(v):
    return v.astype(BF16).astype(F32)


def _recip(v):
    return pl.reciprocal(v, approx=True)


def _recip_nr(v):
    r = pl.reciprocal(v, approx=True)
    return r * (2.0 - v * r)


def _sigmoid(v):
    return 0.5 * jnp.tanh(0.5 * v) + 0.5


def _cat(parts):
    return jnp.concatenate(parts, axis=1)


def _pk(v):
    return pltpu.bitcast(v, U32)


def _up(v):
    return pltpu.bitcast(v, BF16)


def _pk2(lo, hi):
    return pltpu.bitcast(pltpu.pack_elementwise([lo, hi], packed_dtype=BF16), U32)


def _pair_allreduce(v, op):
    v = op(v, pltpu.roll(v, 2, 0))
    return op(v, pltpu.roll(v, 4, 0))


def _zero_like(v):
    return jnp.where(v < 0.0, 1.0, 0.0)


def _dual_softmax(p, z=None):
    n = p.shape[-1]
    p = p.reshape(8, 8, n)
    mx = jnp.max(p, axis=0)
    if z is not None:
        mx = mx + z
    mx = _pair_allreduce(mx, jnp.maximum)
    mn = _pair_allreduce(jnp.min(p, axis=0), jnp.minimum)
    ep = jnp.exp2(p - mx[None])
    en = jnp.exp2(mn[None] - p)
    rp = _recip(_pair_allreduce(jnp.sum(ep, axis=0), jnp.add))
    rn = _recip(_pair_allreduce(jnp.sum(en, axis=0), jnp.add))
    return _pk2((ep * rp[None]).reshape(64, n), (en * rn[None]).reshape(64, n)), rp


def _kernel(cfg, x_hbm, wqkv_hbm, phi_hbm, wo_hbm, wr_hbm, wg_hbm, wu_hbm, wd_hbm, out_hbm,
            x_buf, xn3, out_buf, wraw, phi_buf, wr_buf, wo_buf, wg_buf, wu_buf, wd_buf,
            wq3, wk3, wv3, wo3, pbuf0, pbuf1, phik3, vaug3, phiq3, lmat, o3, r_buf, bsel_buf, s_buf, fix_buf,
            sem, sem_o):
    S = cfg["S"]
    KQ = cfg["KQ"]
    NB = S // LANE
    NTILE = S // T
    pbuf = (pbuf0, pbuf1)
    s_x0, s_phi, s_x2, s_wv, s_xr, s_rest, s_wk = 0, 1, 2, 3, 4, 5, 6

    def x_copy(i):
        slot = s_x0 if i == 0 else s_wk + KQ - 1 if i == 1 else s_x2 if i == 2 else s_wv if i == 3 else s_xr
        return pltpu.make_async_copy(x_hbm.at[pl.ds(i * T, T)], x_buf.at[pl.ds(i * T, T)], sem.at[slot])

    def out_copy(r0, n):
        slot = 2 if r0 + n == S else 0
        return pltpu.make_async_copy(out_buf.at[pl.ds(r0, n)], out_hbm.at[pl.ds(r0, n)], sem_o.at[slot])

    kw = D // KQ

    def wk_copy(c):
        return pltpu.make_async_copy(wqkv_hbm.at[:, pl.ds(D + c * kw, kw)],
                                     wraw.at[1, :, pl.ds(c * kw, kw)], sem.at[s_wk + c])

    c_wr = pltpu.make_async_copy(wr_hbm, wr_buf, sem.at[s_x0])
    c_phi = pltpu.make_async_copy(phi_hbm, phi_buf, sem.at[s_phi])
    c_wv = pltpu.make_async_copy(wqkv_hbm.at[:, pl.ds(2 * D, D)], wraw.at[2], sem.at[s_wv])
    c_rest = [
        pltpu.make_async_copy(wqkv_hbm.at[:, pl.ds(0, D)], wraw.at[0], sem.at[s_rest]),
        pltpu.make_async_copy(wo_hbm, wo_buf, sem.at[s_rest]),
        pltpu.make_async_copy(wg_hbm, wg_buf, sem.at[s_rest]),
        pltpu.make_async_copy(wu_hbm, wu_buf, sem.at[s_rest]),
        pltpu.make_async_copy(wd_hbm, wd_buf.at[:, pl.ds(0, D)], sem.at[s_rest]),
    ]

    x_copy(0).start()
    c_wr.start()
    c_phi.start()
    for c in range(KQ):
        wk_copy(c).start()
    x_copy(1).start()
    x_copy(2).start()
    c_wv.start()
    for i in range(3, NTILE):
        x_copy(i).start()
    for c in c_rest:
        c.start()

    ones = _pk(jnp.ones((RB, LANE), BF16))
    for b in range(NB):
        for j in range(NPAIR):
            vaug3[b, (j * PR + 2 * DH) // 2:(j + 1) * PR // 2, :] = ones

    def put_rows(dst, r0, val):
        n = val.shape[0]
        for k in range(KB):
            dst[k, r0 // 2:(r0 + n) // 2, :] = _pk(val[:, k * LANE:(k + 1) * LANE])

    def put_words(dst, w0, val):
        for k in range(KB):
            dst[k, w0:w0 + val.shape[0], :] = val[:, k * LANE:(k + 1) * LANE]

    def get_rows(src, r0, n):
        return _cat([_up(src[k, r0 // 2:(r0 + n) // 2, :]) for k in range(KB)])

    def layernorm(i, ch):
        z = None
        eps = _rb(jnp.full((1, 1), 1e-5, F32))
        for r0 in range(i * T, (i + 1) * T, ch):
            xf = x_buf[r0:r0 + ch, :].astype(F32)
            mean = jnp.sum(xf, axis=-1, keepdims=True) * (1.0 / D)
            if z is not None:
                mean = mean + z
            c = xf - mean
            var = jnp.sum(c * c, axis=-1, keepdims=True) * (1.0 / D)
            rs = _recip_nr(_rb(jnp.sqrt(_rb(_rb(var) + eps))))
            z = _zero_like(rs)
            put_rows(xn3, r0, (_rb(xf - _rb(mean)) * rs).astype(BF16))

    x_copy(0).wait()
    c_wr.wait()
    layernorm(0, T)
    wrf = wr_buf[...].reshape(1, D).astype(F32)
    for k in range(KB):
        wr8 = jnp.broadcast_to(wrf[:, k * LANE:(k + 1) * LANE], (8, LANE))
        wk3[k, D // 2:(D + RB) // 2, :] = _pk2(wr8, wr8)
    sign = lax.shift_right_logical(pltpu.bitcast(wrf[:, 0:LANE], jnp.int32), 31)
    zrt = pl.multiple_of(lax.shift_right_logical(jnp.max(sign), 1), 8)

    def z0(tag):
        return zrt if tag in cfg["opq"] else 0

    c_phi.wait()
    phi2 = phi_buf[...].reshape(H * DH, DH)
    er = lax.broadcasted_iota(jnp.int32, (LANE, DH), 0)
    ec = lax.broadcasted_iota(jnp.int32, (LANE, DH), 1)
    eye4 = jnp.where(er % DH == ec, 1.0, 0.0).astype(BF16)
    br = lax.broadcasted_iota(jnp.int32, (LANE, LANE), 0)
    bc = lax.broadcasted_iota(jnp.int32, (LANE, LANE), 1)
    bmask = (2 * ((br % (2 * DH)) // DH) + br // (2 * DH)) == bc // DH
    bd = []
    for g in range(KB):
        t = _nt(eye4, phi2[g * LANE:(g + 1) * LANE])
        bd.append(jnp.where(bmask, t, 0.0).astype(BF16))

    def get_w(src, r0, n):
        z = z0("w")
        return _cat([_up(src[k, pl.ds(z + r0 // 2, n // 2), :]) for k in range(KB)])

    def fold(j, dst, g0, g1):
        for g in range(g0, g1):
            w = wraw[j, :, g * LANE:(g + 1) * LANE]
            res = _nt(bd[g], w) * LOG2E
            put_words(dst, g * 64, _pk2(res[:64], res[64:]))

    def stage_k(i, r0=0, r1=D, inline=True):
        last = r1 == D
        for bl in range(TB):
            b = i * TB + bl
            pt = _nt(get_w(wk3, r0, r1 - r0 + (RB if last else 0)), get_rows(xn3, b * LANE, LANE))
            if last:
                r_buf[:, b * LANE:(b + 1) * LANE] = pt[r1 - r0:r1 - r0 + 8, :]
            if inline:
                for j in range(r0 // 64, r1 // 64):
                    phik3[b, j * 64:(j + 1) * 64, :] = _dual_softmax(pt[j * 64 - r0:(j + 1) * 64 - r0, :])[0]
            else:
                pbuf[bl][r0:r1, :] = pt[:r1 - r0, :]

    def stage_q(i):
        for bl in range(TB):
            b = i * TB + bl
            pt = _nt(get_w(wq3, 0, D), get_rows(xn3, b * LANE, LANE))
            if bl in cfg["q_inline"]:
                for j in range(NPAIR):
                    phiq3[bl, j * 64:(j + 1) * 64, :] = _dual_softmax(pt[j * 64:(j + 1) * 64, :])[0]
            else:
                pbuf[bl][...] = pt

    def stage_sm(dst, b0, skip=()):
        nch = cfg["nch"]
        zc = [None] * nch
        link = 0
        for bl in range(TB):
            if bl in skip:
                continue
            for j in range(NPAIR):
                pk, rp = _dual_softmax(pbuf[bl][pl.ds(z0("s") + j * 64, 64), :], zc[link % nch])
                zc[link % nch] = _zero_like(rp)
                dst[b0 + bl, j * 64:(j + 1) * 64, :] = pk
                link += 1

    def stage_v(i):
        for b in range(i * TB, (i + 1) * TB):
            vt = _nt(get_w(wv3, 0, D), get_rows(xn3, b * LANE, LANE))
            for j in range(NPAIR):
                r = j * 2 * DH
                vaug3[b, j * PR // 2:j * PR // 2 + DH, :] = _pk2(vt[r:r + DH], vt[r + DH:r + 2 * DH])

    def stage_kv():
        lr = lax.broadcasted_iota(jnp.int32, (PR, LANE), 0)
        lc = lax.broadcasted_iota(jnp.int32, (PR, LANE), 1)
        keep = lr % 2 == (lc // 2) % 2
        for j in range(NPAIR):
            va = _cat([_up(vaug3[b, pl.ds(z0("v") + j * PR // 2, PR // 2), :]) for b in range(NB)])
            pk = _cat([_up(phik3[b, pl.ds(z0("k") + j * 64, 64), :]) for b in range(NB)])
            lmat[j] = _pk(jnp.where(keep, _nt(va, pk), 0.0).astype(BF16))

    def stage_b():
        for g in range(KB):
            parts = []
            for j in (2 * g, 2 * g + 1):
                pq = _cat([_up(phiq3[bl, pl.ds(z0("p") + j * 64, 64), :]) for bl in range(TB)])
                nt = _nn(_up(lmat[j]), pq)
                den = nt[2 * DH:2 * DH + 8, :] + 1e-6
                num = nt[:2 * DH, :].reshape(8, 8, T)
                parts.append((num * _recip(den)[None]).reshape(2 * DH, T))
            ot = jnp.concatenate(parts, axis=0)
            o3[g] = _pk(ot.T.astype(BF16))

    def stage_c(i, idx=None):
        r0 = i * T
        o = get_rows(o3, 0, T)
        for n in range(0, KB, 2):
            s = _nn(o, _cat([_up(wo3[n]), _up(wo3[n + 1])]))
            cols = slice(n * LANE, (n + 2) * LANE)
            b = _cat([_up(xn3[m, r0 // 2:(r0 + T) // 2, :]) for m in (n, n + 1)]).astype(F32)
            if idx is None:
                s_buf[r0:r0 + T, cols] = s
            else:
                sel = (lax.broadcasted_iota(jnp.int32, (T, 2 * LANE), 0) + r0) == idx
                b = jnp.where(sel, bsel_buf[0:1, cols], b)
            res = x_buf[r0:r0 + T, cols].astype(F32) + s * (b * _sigmoid(b))
            out_buf[r0:r0 + T, cols] = res.astype(BF16)
        cp = out_copy(r0, T)
        cp.start()
        return cp

    def fixup(idx):
        blk = pl.multiple_of((idx // RB) * RB, RB)
        blk2 = pl.multiple_of((idx // RB) * (RB // 2), RB // 2)
        xn = _cat([_up(xn3[k, pl.ds(blk2, RB // 2), :]) for k in range(KB)]).astype(F32)
        sel = (lax.broadcasted_iota(jnp.int32, (RB, D), 0) + blk) == idx
        b = jnp.where(sel, bsel_buf[0:1, :], xn)
        res = x_buf[pl.ds(blk, RB), :].astype(F32) + s_buf[pl.ds(blk, RB), :] * (b * _sigmoid(b))
        fix_buf[...] = res.astype(BF16)
        cp = pltpu.make_async_copy(fix_buf, out_hbm.at[pl.ds(blk, RB)], sem_o.at[1])
        cp.start()
        cp.wait()

    def route():
        r = _rb(r_buf[0:1, :])
        rmax = jnp.max(r)
        pos = lax.broadcasted_iota(jnp.int32, (1, S), 1)
        idx = jnp.min(jnp.where(r == rmax, pos, S))
        return jnp.clip(idx, 0, S - 1), rmax

    def stage_ffn(idx, rmax):
        blk2 = pl.multiple_of((idx // RB) * (RB // 2), RB // 2)
        xs = _cat([_up(xn3[k, pl.ds(blk2, RB // 2), :]) for k in range(KB)])
        hg = _rb(_nn(xs, wg_buf[...]))
        hu = _rb(_nn(xs, wu_buf[...]))
        act = (_rb(hg * _sigmoid(hg)) * hu).astype(BF16)
        y = _rb(_nn(act, wd_buf[:, 0:D]))
        rs = _rb(_sigmoid(jnp.full((1, 1), rmax, F32)))
        b = _rb(xs.astype(F32) + _rb(y * rs))
        row = lax.broadcasted_iota(jnp.int32, (RB, D), 0) + 2 * blk2
        bsel = jnp.sum(jnp.where(row == idx, b, 0.0), axis=0, keepdims=True)
        bsel_buf[...] = jnp.broadcast_to(bsel, (8, D))

    lc = cfg["ln_chunk"]
    gq = KB // KQ
    for c in range(KQ):
        wk_copy(c).wait()
        if c == KQ - 1:
            x_copy(1).wait()
            layernorm(1, 32)
        fold(1, wk3, c * gq, (c + 1) * gq)
        stage_k(0, c * kw, (c + 1) * kw, inline=cfg["k0_inline"])
    x_copy(2).wait()
    if not cfg["k0_inline"]:
        stage_sm(phik3, 0)
    layernorm(2, lc)
    stage_k(1)
    c_wv.wait()
    x_copy(3).wait()
    for g in range(KB):
        put_rows(wv3, g * LANE, wraw[2, :, g * LANE:(g + 1) * LANE].T)
    stage_k(2)
    stage_v(0)
    stage_v(1)
    for i in range(4, NTILE):
        x_copy(i).wait()
    layernorm(3, lc)
    stage_v(2)
    for i in range(3, NTILE):
        stage_k(i)
        if i + 1 < NTILE:
            layernorm(i + 1, lc)
        stage_v(i)

    for c in c_rest:
        c.wait()
    idx, rmax = route()
    fold(0, wq3, 0, KB)
    for j in range(NPAIR):
        wf = wo_buf[j * 2 * DH:(j + 1) * 2 * DH, :].astype(F32)
        put_words(wo3, j * DH, _pk2(wf[:DH], wf[DH:]))
    stage_kv()
    stage_q(0)
    stage_sm(phiq3, 0, cfg['q_inline'])
    stage_ffn(idx, rmax)

    outs = []
    for i in range(NTILE - 1):
        stage_b()
        stage_q(i + 1)
        stage_sm(phiq3, 0, cfg['q_inline'])
        outs.append(stage_c(i))
    stage_b()
    last = stage_c(NTILE - 1, idx)
    for cp in outs:
        cp.wait()

    @pl.when(idx < S - T)
    def _():
        fixup(idx)

    last.wait()


def _build(cfg):
    S = cfg["S"]
    NB = S // LANE
    any_spec = pl.BlockSpec(memory_space=pl.ANY)
    scratch = [
        pltpu.VMEM((S, D), BF16),
        pltpu.VMEM((KB, S // 2, LANE), U32),
        pltpu.VMEM((S, D), BF16),
        pltpu.VMEM((3, D, D), BF16),
        pltpu.VMEM((H, DH, DH), BF16),
        pltpu.VMEM((D,), BF16),
        pltpu.VMEM((D, D), BF16),
        pltpu.VMEM((D, F), BF16),
        pltpu.VMEM((D, F), BF16),
        pltpu.VMEM((F, WDP), BF16),
        pltpu.VMEM((KB, D // 2, LANE), U32),
        pltpu.VMEM((KB, (D + RB) // 2, LANE), U32),
        pltpu.VMEM((KB, D // 2, LANE), U32),
        pltpu.VMEM((KB, D // 2, LANE), U32),
        pltpu.VMEM((D, LANE), F32),
        pltpu.VMEM((D, LANE), F32),
        pltpu.VMEM((NB, D, LANE), U32),
        pltpu.VMEM((NB, NPAIR * PR // 2, LANE), U32),
        pltpu.VMEM((TB, D, LANE), U32),
        pltpu.VMEM((NPAIR, PR // 2, LANE), U32),
        pltpu.VMEM((KB, T // 2, LANE), U32),
        pltpu.VMEM((8, S), F32),
        pltpu.VMEM((8, D), F32),
        pltpu.VMEM((S - T, D), F32),
        pltpu.VMEM((RB, D), BF16),
        pltpu.SemaphoreType.DMA((6 + cfg["KQ"],)),
        pltpu.SemaphoreType.DMA((3,)),
    ]
    return pl.pallas_call(
        functools.partial(_kernel, cfg),
        out_shape=jax.ShapeDtypeStruct((S, D), BF16),
        in_specs=[any_spec] * 8,
        out_specs=any_spec,
        scratch_shapes=scratch,
        compiler_params=pltpu.CompilerParams(vmem_limit_bytes=100 * 1024 * 1024),
        name=cfg.get("name", "hedgehog_mod"),
    )


@jax.jit
def pallas_recurrent_scan__linear_kernel_hedgehog__moe_arch_mod__prompt_kernel(
    A_x: jax.Array,
    A_wqkv: jax.Array,
    A_w_phi: jax.Array,
    A_wo: jax.Array,
    B_x: jax.Array,
    B_w_r: jax.Array,
    B_w_gate: jax.Array,
    B_w_up: jax.Array,
    B_w_down: jax.Array,
):
    del B_x
    S = CFG["S"]
    out = _build(CFG)(A_x.reshape(S, D), A_wqkv, A_w_phi, A_wo, B_w_r, B_w_gate, B_w_up, B_w_down)
    return out.reshape(1, S, D)
```

```python
import functools

import jax
import jax.numpy as jnp
from jax import lax
import jax.experimental.pallas as pl
import jax.experimental.pallas.tpu as pltpu

D, H, DH, F = 1024, 32, 32, 3584
LANE = 128
KB = D // LANE
KH = D // 2
T = 256
TB = T // LANE
NPAIR = H // 2
PR = 2 * DH + 16
RB = 16
WDP = D + LANE
NG = F // KH
LOG2E = 1.4426950408889634
F32 = jnp.float32
BF16 = jnp.bfloat16
U32 = jnp.uint32

CFG = dict(S=2048, ln_chunk=16, opq="pkvw")


def _nt(a, b):
    return lax.dot_general(a, b, (((1,), (1,)), ((), ())), preferred_element_type=F32)


def _nn(a, b):
    return jnp.dot(a, b, preferred_element_type=F32)


def _rb(v):
    return v.astype(BF16).astype(F32)


def _recip(v):
    return pl.reciprocal(v, approx=True)


def _recip_nr(v):
    r = pl.reciprocal(v, approx=True)
    return r * (2.0 - v * r)


def _sigmoid(v):
    return 0.5 * jnp.tanh(0.5 * v) + 0.5


def _cat(parts):
    return jnp.concatenate(parts, axis=1)


def _pk(v):
    return pltpu.bitcast(v, U32)


def _up(v):
    return pltpu.bitcast(v, BF16)


def _pk2(lo, hi):
    return pltpu.bitcast(pltpu.pack_elementwise([lo, hi], packed_dtype=BF16), U32)


def _pair_allreduce(v, op):
    v = op(v, pltpu.roll(v, 2, 0))
    return op(v, pltpu.roll(v, 4, 0))


def _dual_softmax(p):
    n = p.shape[-1]
    p = p.reshape(8, 8, n)
    mx = _pair_allreduce(jnp.max(p, axis=0), jnp.maximum)
    mn = _pair_allreduce(jnp.min(p, axis=0), jnp.minimum)
    ep = jnp.exp2(p - mx[None])
    en = jnp.exp2(mn[None] - p)
    rp = _recip(_pair_allreduce(jnp.sum(ep, axis=0), jnp.add))
    rn = _recip(_pair_allreduce(jnp.sum(en, axis=0), jnp.add))
    return _pk2((ep * rp[None]).reshape(64, n), (en * rn[None]).reshape(64, n))


def _kernel(cfg, x_hbm, wqkv_hbm, phi_hbm, wo_hbm, wr_hbm, wg_hbm, wu_hbm, wd_hbm, out_hbm,
            x_buf, xn3, out_buf, wraw, phi_buf, wr_buf, wo_buf, wg_buf, wu_buf, wd_buf,
            wq3, wk3, wv3, wo3, phik3, vaug3, phiq3, lmat, o3, r_buf, s_buf, fix_buf,
            sem, sem_o):
    S = cfg["S"]
    NB = S // LANE
    NTILE = S // T
    assert NTILE - 1 >= NG or cfg.get("short_ffn")

    def cp(src, dst, slot):
        return pltpu.make_async_copy(src, dst, sem.at[slot])

    def x_rows(r0, n, slot):
        return cp(x_hbm.at[pl.ds(r0, n)], x_buf.at[pl.ds(r0, n)], slot)

    def wk_cols(g0, g1, slot):
        n = (g1 - g0) * LANE
        return cp(wqkv_hbm.at[:, pl.ds(D + g0 * LANE, n)], wraw.at[1, :, pl.ds(g0 * LANE, n)], slot)

    groups = [
        [cp(wr_hbm, wr_buf, 0), cp(phi_hbm.at[pl.ds(0, 8)], phi_buf.at[pl.ds(0, 8)], 0), x_rows(0, LANE, 0)],
        [wk_cols(0, 1, 1)],
        [x_rows(LANE, LANE, 2), wk_cols(1, 2, 2)],
        [cp(phi_hbm.at[pl.ds(8, H - 8)], phi_buf.at[pl.ds(8, H - 8)], 3), wk_cols(2, 4, 3)],
        [wk_cols(4, 6, 4)],
        [wk_cols(6, 8, 5), x_rows(T, 2 * T, 5)],
        [cp(wqkv_hbm.at[:, pl.ds(2 * D, D)], wraw.at[2], 6), x_rows(3 * T, T, 6)],
        [x_rows(4 * T, S - 4 * T, 7), cp(wqkv_hbm.at[:, pl.ds(0, D)], wraw.at[0], 7), cp(wo_hbm, wo_buf, 7)],
        [cp(wg_hbm, wg_buf, 8), cp(wu_hbm, wu_buf, 8), cp(wd_hbm, wd_buf.at[:, pl.ds(0, D)], 8)],
    ]
    for grp in groups:
        for c in grp:
            c.start()

    def arrive(k):
        for c in groups[k]:
            c.wait()

    ones = _pk(jnp.ones((RB, LANE), BF16))
    for b in range(NB):
        for j in range(NPAIR):
            vaug3[b, (j * PR + 2 * DH) // 2:(j + 1) * PR // 2, :] = ones

    def put_rows(dst, r0, val):
        n = val.shape[0]
        for k in range(KB):
            dst[k, r0 // 2:(r0 + n) // 2, :] = _pk(val[:, k * LANE:(k + 1) * LANE])

    def put_words(dst, w0, val):
        for k in range(KB):
            dst[k, w0:w0 + val.shape[0], :] = val[:, k * LANE:(k + 1) * LANE]

    def get_rows(src, r0, n, k0=0, k1=KB):
        return _cat([_up(src[k, r0 // 2:(r0 + n) // 2, :]) for k in range(k0, k1)])

    def layernorm(row0, n, ch):
        z = None
        eps = _rb(jnp.full((1, 1), 1e-5, F32))
        for r0 in range(row0, row0 + n, ch):
            xf = x_buf[r0:r0 + ch, :].astype(F32)
            mean = jnp.sum(xf, axis=-1, keepdims=True) * (1.0 / D)
            if z is not None:
                mean = mean + z
            c = xf - mean
            var = jnp.sum(c * c, axis=-1, keepdims=True) * (1.0 / D)
            rs = _recip_nr(_rb(jnp.sqrt(_rb(_rb(var) + eps))))
            z = jnp.where(rs < 0.0, 1.0, 0.0)
            put_rows(xn3, r0, (_rb(xf - _rb(mean)) * rs).astype(BF16))

    er = lax.broadcasted_iota(jnp.int32, (LANE, DH), 0)
    ec = lax.broadcasted_iota(jnp.int32, (LANE, DH), 1)
    eye4 = jnp.where(er % DH == ec, 1.0, 0.0).astype(BF16)
    br = lax.broadcasted_iota(jnp.int32, (LANE, LANE), 0)
    bc = lax.broadcasted_iota(jnp.int32, (LANE, LANE), 1)
    bmask = (2 * ((br % (2 * DH)) // DH) + br // (2 * DH)) == bc // DH
    bd = {}

    def blockdiag(g0, g1):
        for g in range(g0, g1):
            t = _nt(eye4, phi_buf[4 * g:4 * g + 4].reshape(LANE, DH))
            bd[g] = jnp.where(bmask, t, 0.0).astype(BF16)

    def fold(j, dst, g0, g1):
        for g in range(g0, g1):
            res = _nt(bd[g], wraw[j, :, g * LANE:(g + 1) * LANE]) * LOG2E
            put_words(dst, g * 64, _pk2(res[:64], res[64:]))

    def keys(b, g0=0, g1=KB):
        r0, r1 = g0 * LANE, g1 * LANE
        last = g1 == KB
        pt = _nt(get_rows(wk3, r0, r1 - r0 + (RB if last else 0)), get_rows(xn3, b * LANE, LANE))
        if last:
            r_buf[:, b * LANE:(b + 1) * LANE] = pt[r1 - r0:r1 - r0 + 8, :]
        for j in range(r0 // 64, r1 // 64):
            phik3[b, j * 64:(j + 1) * 64, :] = _dual_softmax(pt[j * 64 - r0:(j + 1) * 64 - r0, :])

    def stage_k(i, g0=0, g1=KB):
        for b in range(i * TB, (i + 1) * TB):
            keys(b, g0, g1)

    def stage_v(i):
        for b in range(i * TB, (i + 1) * TB):
            wv = _cat([_up(wv3[k, pl.ds(zw, D // 2), :]) for k in range(KB)])
            vt = _nt(wv, get_rows(xn3, b * LANE, LANE))
            for j in range(NPAIR):
                r = j * 2 * DH
                vaug3[b, j * PR // 2:j * PR // 2 + DH, :] = _pk2(vt[r:r + DH], vt[r + DH:r + 2 * DH])

    ffn_q = []

    def ffn_step():
        if ffn_q:
            ffn_q.pop(0)()

    def stage_q(i):
        for bl in range(TB):
            r0 = (i * TB + bl) * LANE
            pt = _nt(get_rows(wq3, 0, D, 0, 4), get_rows(xn3, r0, LANE, 0, 4))
            ffn_step()
            pt = pt + _nt(get_rows(wq3, 0, D, 4, 8), get_rows(xn3, r0, LANE, 4, 8))
            ffn_step()
            for j in range(NPAIR):
                phiq3[bl, j * 64:(j + 1) * 64, :] = _dual_softmax(pt[j * 64:(j + 1) * 64, :])

    def stage_kv(zv, zk):
        lr = lax.broadcasted_iota(jnp.int32, (PR, LANE), 0)
        lc = lax.broadcasted_iota(jnp.int32, (PR, LANE), 1)
        keep = lr % 2 == (lc // 2) % 2
        for j in range(NPAIR):
            va = _cat([_up(vaug3[b, pl.ds(zv + j * PR // 2, PR // 2), :]) for b in range(NB)])
            pk = _cat([_up(phik3[b, pl.ds(zk + j * 64, 64), :]) for b in range(NB)])
            lmat[j] = _pk(jnp.where(keep, _nt(va, pk), 0.0).astype(BF16))

    def stage_b(zp):
        for g in range(KB):
            parts = []
            for j in (2 * g, 2 * g + 1):
                pq = _cat([_up(phiq3[bl, pl.ds(zp + j * 64, 64), :]) for bl in range(TB)])
                nt = _nn(_up(lmat[j]), pq)
                den = nt[2 * DH:2 * DH + 8, :] + 1e-6
                num = nt[:2 * DH, :].reshape(8, 8, T)
                parts.append((num * _recip(den)[None]).reshape(2 * DH, T))
            ffn_step()
            ot = jnp.concatenate(parts, axis=0)
            o3[g] = _pk(ot.T.astype(BF16))

    def stage_c(i, routed=None):
        r0 = i * T
        o = get_rows(o3, 0, T)
        copies = []
        for n in range(0, KB, 2):
            parts = []
            for m in (n, n + 1):
                w = _up(wo3[m])
                s = _nn(o[:, :KH], w[:KH])
                ffn_step()
                parts.append(s + _nn(o[:, KH:], w[KH:]))
                ffn_step()
            s = _cat(parts)
            cols = slice(n * LANE, (n + 2) * LANE)
            b = get_rows(xn3, r0, T, n, n + 2).astype(F32)
            if routed is None:
                s_buf[r0:r0 + T, cols] = s
            else:
                idx, bsel = routed()
                sel = (lax.broadcasted_iota(jnp.int32, (T, 2 * LANE), 0) + r0) == idx
                b = jnp.where(sel, bsel[:, cols], b)
            res = x_buf[r0:r0 + T, cols].astype(F32) + s * (b * _sigmoid(b))
            out_buf[r0:r0 + T, cols] = res.astype(BF16)
            if routed is not None:
                win = (pl.ds(r0, T), pl.ds(n * LANE, 2 * LANE))
                copies.append(pltpu.make_async_copy(out_buf.at[win], out_hbm.at[win], sem_o.at[2]))
                copies[-1].start()
        if routed is None:
            copies.append(pltpu.make_async_copy(out_buf.at[pl.ds(r0, T)], out_hbm.at[pl.ds(r0, T)], sem_o.at[0]))
            copies[-1].start()
        return copies

    lc = cfg["ln_chunk"]
    arrive(0)
    layernorm(0, LANE, LANE)
    wrf = wr_buf[...].reshape(1, D).astype(F32)
    for k in range(KB):
        wr8 = jnp.broadcast_to(wrf[:, k * LANE:(k + 1) * LANE], (8, LANE))
        wk3[k, D // 2:(D + RB) // 2, :] = _pk2(wr8, wr8)
    sign = lax.shift_right_logical(pltpu.bitcast(wrf[:, 0:LANE], jnp.int32), 31)
    zrt = pl.multiple_of(lax.shift_right_logical(jnp.max(sign), 1), 8)
    zp, zk, zv, zw = [zrt if t in cfg["opq"] else 0 for t in "pkvw"]
    blockdiag(0, 2)
    arrive(1)
    fold(1, wk3, 0, 1)
    keys(0, 0, 1)
    arrive(2)
    layernorm(LANE, LANE, LANE)
    fold(1, wk3, 1, 2)
    keys(0, 1, 2)
    keys(1, 0, 2)
    arrive(3)
    blockdiag(2, KB)
    fold(1, wk3, 2, 4)
    stage_k(0, 2, 4)
    arrive(4)
    fold(1, wk3, 4, 6)
    stage_k(0, 4, 6)
    arrive(5)
    layernorm(T, T, 32)
    fold(1, wk3, 6, 8)
    stage_k(0, 6, 8)
    layernorm(2 * T, T, lc)
    stage_k(1)
    arrive(6)
    for g in range(KB):
        put_rows(wv3, g * LANE, wraw[2, :, g * LANE:(g + 1) * LANE].T)
    stage_k(2)
    stage_v(0)
    stage_v(1)
    layernorm(3 * T, T, lc)
    stage_v(2)
    arrive(7)
    for i in range(3, NTILE):
        stage_k(i)
        if i + 1 < NTILE:
            layernorm((i + 1) * T, T, lc)
        stage_v(i)
        if i == 3:
            fold(0, wq3, 0, KB)
    for j in range(NPAIR):
        wf = wo_buf[j * 2 * DH:(j + 1) * 2 * DH, :].astype(F32)
        put_words(wo3, j * DH, _pk2(wf[:DH], wf[DH:]))
    stage_q(0)
    stage_kv(zv, zk)

    arrive(8)
    r = _rb(r_buf[0:1, :])
    rmax = jnp.max(r)
    pos = lax.broadcasted_iota(jnp.int32, (1, S), 1)
    idx = jnp.clip(jnp.min(jnp.where(r == rmax, pos, S)), 0, S - 1)
    blk = pl.multiple_of((idx // RB) * RB, RB)
    blk2 = pl.multiple_of((idx // RB) * (RB // 2), RB // 2)
    xs = _cat([_up(xn3[k, pl.ds(blk2, RB // 2), :]) for k in range(KB)])
    rowsel = (lax.broadcasted_iota(jnp.int32, (RB, D), 0) + blk) == idx
    part, act, y = {}, {}, {}

    def gate_up(w_buf, j, h):
        def f():
            v = _nn(xs[:, h * KH:(h + 1) * KH], w_buf[h * KH:(h + 1) * KH, j * LANE:(j + 1) * LANE])
            key = (w_buf is wu_buf, j)
            part[key] = v if h == 0 else _rb(part[key] + v)
            if h == 1 and w_buf is wu_buf:
                hg = part.pop((False, j))
                act[j] = (_rb(hg * _sigmoid(hg)) * part.pop(key)).astype(BF16)
        return f

    def down(m, n):
        def f():
            a = _cat([act[j] for j in range(4 * m, 4 * m + 4)])
            v = _nn(a, wd_buf[m * KH:(m + 1) * KH, n * LANE:(n + 1) * LANE])
            y[n] = v if m == 0 else y[n] + v
        return f

    def gate_input():
        rs = _rb(_sigmoid(jnp.full((1, 1), rmax, F32)))
        yf = _rb(_rb(_cat([y[n] for n in range(KB)])) * rs)
        return _rb(xs.astype(F32) + jnp.where(rowsel, yf, 0.0))

    def routed():
        if "b" not in part:
            part["b"] = gate_input()
            part["row"] = jnp.sum(jnp.where(rowsel, part["b"], 0.0), axis=0, keepdims=True)
        return idx, part["row"]

    ng = min(NG, NTILE - 1)
    outs = []
    for i in range(NTILE):
        if 1 <= i <= ng:
            ffn_q.extend(down(i - 1, n) for n in range(KB))
        stage_b(zp)
        if i < ng:
            for j in range(4 * i, 4 * i + 4):
                ffn_q.extend(gate_up(w, j, h) for w in (wg_buf, wu_buf) for h in range(2))
        if i + 1 < NTILE:
            stage_q(i + 1)
            outs += stage_c(i)
        else:
            last = stage_c(i, routed)
        assert not ffn_q

    for c in outs:
        c.wait()

    @pl.when(idx < S - T)
    def _():
        b = part["b"]
        res = x_buf[pl.ds(blk, RB), :].astype(F32) + s_buf[pl.ds(blk, RB), :] * (b * _sigmoid(b))
        fix_buf[...] = res.astype(BF16)
        c = pltpu.make_async_copy(fix_buf, out_hbm.at[pl.ds(blk, RB)], sem_o.at[1])
        c.start()
        c.wait()

    for c in last:
        c.wait()


def _build(cfg):
    S = cfg["S"]
    NB = S // LANE
    any_spec = pl.BlockSpec(memory_space=pl.ANY)
    scratch = [
        pltpu.VMEM((S, D), BF16),
        pltpu.VMEM((KB, S // 2, LANE), U32),
        pltpu.VMEM((S, D), BF16),
        pltpu.VMEM((3, D, D), BF16),
        pltpu.VMEM((H, DH, DH), BF16),
        pltpu.VMEM((D,), BF16),
        pltpu.VMEM((D, D), BF16),
        pltpu.VMEM((D, F), BF16),
        pltpu.VMEM((D, F), BF16),
        pltpu.VMEM((F, WDP), BF16),
        pltpu.VMEM((KB, D // 2, LANE), U32),
        pltpu.VMEM((KB, (D + RB) // 2, LANE), U32),
        pltpu.VMEM((KB, D // 2, LANE), U32),
        pltpu.VMEM((KB, D // 2, LANE), U32),
        pltpu.VMEM((NB, D, LANE), U32),
        pltpu.VMEM((NB, NPAIR * PR // 2, LANE), U32),
        pltpu.VMEM((TB, D, LANE), U32),
        pltpu.VMEM((NPAIR, PR // 2, LANE), U32),
        pltpu.VMEM((KB, T // 2, LANE), U32),
        pltpu.VMEM((8, S), F32),
        pltpu.VMEM((S - T, D), F32),
        pltpu.VMEM((RB, D), BF16),
        pltpu.SemaphoreType.DMA((9,)),
        pltpu.SemaphoreType.DMA((3,)),
    ]
    return pl.pallas_call(
        functools.partial(_kernel, cfg),
        out_shape=jax.ShapeDtypeStruct((S, D), BF16),
        in_specs=[any_spec] * 8,
        out_specs=any_spec,
        scratch_shapes=scratch,
        compiler_params=pltpu.CompilerParams(vmem_limit_bytes=100 * 1024 * 1024),
        name=cfg.get("name", "hedgehog_mod"),
    )


@jax.jit
def pallas_recurrent_scan__linear_kernel_hedgehog__moe_arch_mod__prompt_kernel(
    A_x: jax.Array,
    A_wqkv: jax.Array,
    A_w_phi: jax.Array,
    A_wo: jax.Array,
    B_x: jax.Array,
    B_w_r: jax.Array,
    B_w_gate: jax.Array,
    B_w_up: jax.Array,
    B_w_down: jax.Array,
):
    del B_x
    S = CFG["S"]
    out = _build(CFG)(A_x.reshape(S, D), A_wqkv, A_w_phi, A_wo, B_w_r, B_w_gate, B_w_up, B_w_down)
    return out.reshape(1, S, D)
```

```python
import functools

import jax
import jax.numpy as jnp
from jax import lax
import jax.experimental.pallas as pl
import jax.experimental.pallas.tpu as pltpu

D, H, DH, F = 1024, 32, 32, 3584
LANE = 128
KB = D // LANE
KH = D // 2
T = 256
TB = T // LANE
NPAIR = H // 2
PR = 2 * DH + 16
RB = 16
WDP = D + LANE
NG = F // KH
LOG2E = 1.4426950408889634
F32 = jnp.float32
BF16 = jnp.bfloat16
U32 = jnp.uint32

CFG = dict(S=2048, ln_chunk=16, opq="pkvw", mid_at=6)


def _nt(a, b):
    return lax.dot_general(a, b, (((1,), (1,)), ((), ())), preferred_element_type=F32)


def _nn(a, b):
    return jnp.dot(a, b, preferred_element_type=F32)


def _rb(v):
    return v.astype(BF16).astype(F32)


def _recip(v):
    return pl.reciprocal(v, approx=True)


def _recip_nr(v):
    r = pl.reciprocal(v, approx=True)
    return r * (2.0 - v * r)


def _sigmoid(v):
    return 0.5 * jnp.tanh(0.5 * v) + 0.5


def _cat(parts):
    return jnp.concatenate(parts, axis=1)


def _pk(v):
    return pltpu.bitcast(v, U32)


def _up(v):
    return pltpu.bitcast(v, BF16)


def _pk2(lo, hi):
    return pltpu.bitcast(pltpu.pack_elementwise([lo, hi], packed_dtype=BF16), U32)


def _pair_allreduce(v, op):
    v = op(v, pltpu.roll(v, 2, 0))
    return op(v, pltpu.roll(v, 4, 0))


def _dual_softmax(p, z=None):
    n = p.shape[-1]
    p = p.reshape(8, 8, n)
    mx = _pair_allreduce(jnp.max(p, axis=0), jnp.maximum)
    mn = _pair_allreduce(jnp.min(p, axis=0), jnp.minimum)
    ep = jnp.exp2(p - mx[None])
    en = jnp.exp2(mn[None] - p)
    rp = _recip(_pair_allreduce(jnp.sum(ep, axis=0), jnp.add))
    rn = _recip(_pair_allreduce(jnp.sum(en, axis=0), jnp.add))
    if z is not None:
        dp = _pair_allreduce(jnp.sum(ep * z[0].reshape(8, 8, n), axis=0), jnp.add)
        dn = _pair_allreduce(jnp.sum(en * z[1].reshape(8, 8, n), axis=0), jnp.add)
        rd = _recip(rp * dp + rn * dn + 1e-6)
        rp = rp * rd
        rn = rn * rd
    return (ep * rp[None]).reshape(64, n), (en * rn[None]).reshape(64, n)


def _kernel(cfg, x_hbm, wqkv_hbm, phi_hbm, wo_hbm, wr_hbm, wg_hbm, wu_hbm, wd_hbm, out_hbm,
            x_buf, xn3, out_buf, wraw, phi_buf, wr_buf, wo_buf, wg_buf, wu_buf, wd_buf,
            wq3, wk3, wv3, wo3, phik3, vaug3, zrow, zbuf, phiq3, lmat, o3, r_buf, s_buf, fix_buf,
            sem, sem_o):
    S = cfg["S"]
    NB = S // LANE
    NTILE = S // T

    def cp(src, dst, slot):
        return pltpu.make_async_copy(src, dst, sem.at[slot])

    def x_rows(r0, n, slot):
        return cp(x_hbm.at[pl.ds(r0, n)], x_buf.at[pl.ds(r0, n)], slot)

    def wk_cols(g0, g1, slot):
        n = (g1 - g0) * LANE
        return [cp(wqkv_hbm.at[pl.ds(r, KH), pl.ds(D + g0 * LANE, n)],
                   wraw.at[1, pl.ds(r, KH), pl.ds(g0 * LANE, n)], slot) for r in (0, KH)]

    groups = [
        [x_rows(0, 64, 0), x_rows(64, 64, 0), cp(wr_hbm, wr_buf, 0),
         cp(phi_hbm.at[pl.ds(0, 8)], phi_buf.at[pl.ds(0, 8)], 0)],
        wk_cols(0, 2, 1),
        [x_rows(b * LANE, LANE, 2) for b in range(1, 2 * TB)],
        [cp(phi_hbm.at[pl.ds(8, H - 8)], phi_buf.at[pl.ds(8, H - 8)], 3)] + wk_cols(2, 4, 3),
        wk_cols(4, 8, 4) + [x_rows(2 * T, T, 4)],
        [cp(wqkv_hbm.at[:, pl.ds(2 * D, D)], wraw.at[2], 5), x_rows(3 * T, T, 5)],
        [x_rows(4 * T, S - 4 * T, 6), cp(wqkv_hbm.at[:, pl.ds(0, D)], wraw.at[0], 6), cp(wo_hbm, wo_buf, 6)],
        [cp(wg_hbm, wg_buf, 7), cp(wu_hbm, wu_buf, 7), cp(wd_hbm, wd_buf.at[:, pl.ds(0, D)], 7)],
    ]
    for grp in groups:
        for c in grp:
            c.start()

    def arrive(k):
        for c in groups[k]:
            c.wait()

    ones = _pk(jnp.ones((RB, LANE), BF16))
    for b in range(NB):
        for j in range(NPAIR):
            vaug3[b, (j * PR + 2 * DH) // 2:(j + 1) * PR // 2, :] = ones

    def put_rows(dst, r0, val):
        n = val.shape[0]
        for k in range(KB):
            dst[k, r0 // 2:(r0 + n) // 2, :] = _pk(val[:, k * LANE:(k + 1) * LANE])

    def put_words(dst, w0, val):
        for k in range(KB):
            dst[k, w0:w0 + val.shape[0], :] = val[:, k * LANE:(k + 1) * LANE]

    def get_rows(src, r0, n, k0=0, k1=KB):
        return _cat([_up(src[k, r0 // 2:(r0 + n) // 2, :]) for k in range(k0, k1)])

    def layernorm(row0, n, ch):
        z = None
        eps = _rb(jnp.full((1, 1), 1e-5, F32))
        for r0 in range(row0, row0 + n, ch):
            xf = x_buf[r0:r0 + ch, :].astype(F32)
            mean = jnp.sum(xf, axis=-1, keepdims=True) * (1.0 / D)
            if z is not None:
                mean = mean + z
            c = xf - mean
            var = jnp.sum(c * c, axis=-1, keepdims=True) * (1.0 / D)
            rs = _recip_nr(_rb(jnp.sqrt(_rb(_rb(var) + eps))))
            z = jnp.where(rs < 0.0, 1.0, 0.0)
            put_rows(xn3, r0, (_rb(xf - _rb(mean)) * rs).astype(BF16))

    er = lax.broadcasted_iota(jnp.int32, (LANE, DH), 0)
    ec = lax.broadcasted_iota(jnp.int32, (LANE, DH), 1)
    eye4 = jnp.where(er % DH == ec, 1.0, 0.0).astype(BF16)
    br = lax.broadcasted_iota(jnp.int32, (LANE, LANE), 0)
    bc = lax.broadcasted_iota(jnp.int32, (LANE, LANE), 1)
    bmask = (2 * ((br % (2 * DH)) // DH) + br // (2 * DH)) == bc // DH
    bd = {}

    def blockdiag(g0, g1):
        for g in range(g0, g1):
            t = _nt(eye4, phi_buf[4 * g:4 * g + 4].reshape(LANE, DH))
            bd[g] = jnp.where(bmask, t, 0.0).astype(BF16)

    def fold(j, dst, g0, g1):
        for g in range(g0, g1):
            res = _nt(bd[g], wraw[j, :, g * LANE:(g + 1) * LANE]) * LOG2E
            put_words(dst, g * 64, _pk2(res[:64], res[64:]))

    def keys(b, g0=0, g1=KB):
        r0, r1 = g0 * LANE, g1 * LANE
        last = g1 == KB
        pt = _nt(get_rows(wk3, r0, r1 - r0 + (RB if last else 0)), get_rows(xn3, b * LANE, LANE))
        if last:
            r_buf[:, b * LANE:(b + 1) * LANE] = pt[r1 - r0:r1 - r0 + 8, :]
        for j in range(r0 // 64, r1 // 64):
            rows = slice(j * 64, (j + 1) * 64)
            phik3[b, rows, :] = _pk2(*_dual_softmax(pt[j * 64 - r0:(j + 1) * 64 - r0, :]))

    def stage_k(i, g0=0, g1=KB):
        for b in range(i * TB, (i + 1) * TB):
            keys(b, g0, g1)

    def stage_v(i):
        for b in range(i * TB, (i + 1) * TB):
            wv = _cat([_up(wv3[k, pl.ds(zw, D // 2), :]) for k in range(KB)])
            vt = _nt(wv, get_rows(xn3, b * LANE, LANE))
            for j in range(NPAIR):
                r = j * 2 * DH
                vaug3[b, j * PR // 2:j * PR // 2 + DH, :] = _pk2(vt[r:r + DH], vt[r + DH:r + 2 * DH])

    ffn_q = []

    def ffn_step():
        if ffn_q:
            ffn_q.pop(0)()

    def stage_q(i):
        for bl in range(TB):
            r0 = (i * TB + bl) * LANE
            pt = _nt(get_rows(wq3, 0, D, 0, 4), get_rows(xn3, r0, LANE, 0, 4))
            ffn_step()
            pt = pt + _nt(get_rows(wq3, 0, D, 4, 8), get_rows(xn3, r0, LANE, 4, 8))
            for j in range(NPAIR):
                rows = slice(j * 64, (j + 1) * 64)
                z = None if i == 0 else [zbuf[j, pl.ds(t, 64, stride=2), :] for t in range(2)]
                phiq3[bl, rows, :] = _pk2(*_dual_softmax(pt[rows, :], z))

    def stage_kv(zv, zk):
        lr = lax.broadcasted_iota(jnp.int32, (PR, LANE), 0)
        lc = lax.broadcasted_iota(jnp.int32, (PR, LANE), 1)
        keep = lr % 2 == (lc // 2) % 2
        for j in range(NPAIR):
            va = _cat([_up(vaug3[b, pl.ds(zv + j * PR // 2, PR // 2), :]) for b in range(NB)])
            pk = _cat([_up(phik3[b, pl.ds(zk + j * 64, 64), :]) for b in range(NB)])
            kvt = _nt(va, pk)
            lmat[j] = _pk(jnp.where(keep, kvt, 0.0).astype(BF16))
            zrow[j] = kvt[2 * DH:2 * DH + 8, :]

    def stage_z():
        for j in range(NPAIR):
            zbuf[j] = jnp.concatenate([zrow[j]] * (LANE // 8), axis=0).T

    def stage_b(i, zp):
        for g in range(KB):
            parts = []
            for j in (2 * g, 2 * g + 1):
                pq = _cat([_up(phiq3[bl, pl.ds(zp + j * 64, 64), :]) for bl in range(TB)])
                if i == 0:
                    nt = _nn(_up(lmat[j]), pq)
                    den = nt[2 * DH:2 * DH + 8, :] + 1e-6
                    num = nt[:2 * DH, :].reshape(8, 8, T)
                    parts.append((num * _recip(den)[None]).reshape(2 * DH, T))
                else:
                    parts.append(_nn(_up(lmat[j, 0:DH, :]), pq))
            ffn_step()
            o3[g] = _pk(jnp.concatenate(parts, axis=0).T.astype(BF16))

    def stage_c(i, routed=None, mid=None):
        r0 = i * T
        o = get_rows(o3, 0, T)
        copies = []
        for n in range(0, KB, 2):
            if mid is not None and n == cfg["mid_at"]:
                mid()
            parts = []
            for m in (n, n + 1):
                w = _up(wo3[m])
                s = _nn(o[:, :KH], w[:KH])
                ffn_step()
                parts.append(s + _nn(o[:, KH:], w[KH:]))
                ffn_step()
            s = _cat(parts)
            cols = slice(n * LANE, (n + 2) * LANE)
            b = get_rows(xn3, r0, T, n, n + 2).astype(F32)
            if routed is None:
                s_buf[r0:r0 + T, cols] = s
            else:
                idx, bsel = routed()
                sel = (lax.broadcasted_iota(jnp.int32, (T, 2 * LANE), 0) + r0) == idx
                b = jnp.where(sel, bsel[:, cols], b)
            res = x_buf[r0:r0 + T, cols].astype(F32) + s * (b * _sigmoid(b))
            out_buf[r0:r0 + T, cols] = res.astype(BF16)
            if routed is not None:
                win = (pl.ds(r0, T), pl.ds(n * LANE, 2 * LANE))
                copies.append(pltpu.make_async_copy(out_buf.at[win], out_hbm.at[win], sem_o.at[2]))
                copies[-1].start()
        if routed is None:
            copies.append(pltpu.make_async_copy(out_buf.at[pl.ds(r0, T)], out_hbm.at[pl.ds(r0, T)], sem_o.at[0]))
            copies[-1].start()
        return copies

    lc = cfg["ln_chunk"]
    arrive(0)
    layernorm(0, LANE, LANE)
    wrf = wr_buf[...].reshape(1, D).astype(F32)
    for k in range(KB):
        wr8 = jnp.broadcast_to(wrf[:, k * LANE:(k + 1) * LANE], (8, LANE))
        wk3[k, D // 2:(D + RB) // 2, :] = _pk2(wr8, wr8)
    sign = lax.shift_right_logical(pltpu.bitcast(wrf[:, 0:LANE], jnp.int32), 31)
    zrt = pl.multiple_of(lax.shift_right_logical(jnp.max(sign), 1), 8)
    zp, zk, zv, zw = [zrt if t in cfg["opq"] else 0 for t in "pkvw"]
    blockdiag(0, 2)
    arrive(1)
    fold(1, wk3, 0, 2)
    keys(0, 0, 2)
    arrive(2)
    for b in range(1, 2 * TB):
        layernorm(b * LANE, LANE, LANE)
        keys(b, 0, 2)
    arrive(3)
    blockdiag(2, KB)
    fold(1, wk3, 2, 4)
    for b in range(2 * TB):
        keys(b, 2, 4)
    arrive(4)
    fold(1, wk3, 4, 8)
    for b in range(2 * TB):
        keys(b, 4, 8)
    layernorm(2 * T, T, lc)
    arrive(5)
    for g in range(KB):
        put_rows(wv3, g * LANE, wraw[2, :, g * LANE:(g + 1) * LANE].T)
    stage_k(2)
    stage_v(0)
    layernorm(3 * T, T, lc)
    stage_v(1)
    stage_k(3)
    stage_v(2)
    arrive(6)
    for i in range(3, NTILE):
        if i > 3:
            stage_k(i)
        if i + 1 < NTILE:
            layernorm((i + 1) * T, T, lc)
        stage_v(i)
        if i == 3:
            fold(0, wq3, 0, KB)
    stage_q(0)
    stage_kv(zv, zk)

    arrive(7)
    r = _rb(r_buf[0:1, :])
    rmax = jnp.max(r)
    pos = lax.broadcasted_iota(jnp.int32, (1, S), 1)
    idx = jnp.clip(jnp.min(jnp.where(r == rmax, pos, S)), 0, S - 1)
    blk = pl.multiple_of((idx // RB) * RB, RB)
    blk2 = pl.multiple_of((idx // RB) * (RB // 2), RB // 2)
    xs = _cat([_up(xn3[k, pl.ds(blk2, RB // 2), :]) for k in range(KB)])
    rowsel = (lax.broadcasted_iota(jnp.int32, (RB, D), 0) + blk) == idx
    part, act, y = {}, {}, {}

    def gate_up(w_buf, j, h):
        def f():
            v = _nn(xs[:, h * KH:(h + 1) * KH], w_buf[h * KH:(h + 1) * KH, j * LANE:(j + 1) * LANE])
            key = (w_buf is wu_buf, j)
            part[key] = v if h == 0 else _rb(part[key] + v)
            if h == 1 and w_buf is wu_buf:
                hg = part.pop((False, j))
                act[j] = (_rb(hg * _sigmoid(hg)) * part.pop(key)).astype(BF16)
        return f

    def down(m, n):
        def f():
            a = _cat([act[j] for j in range(4 * m, 4 * m + 4)])
            v = _nn(a, wd_buf[m * KH:(m + 1) * KH, n * LANE:(n + 1) * LANE])
            y[n] = v if m == 0 else y[n] + v
        return f

    def gate_input():
        rs = _rb(_sigmoid(jnp.full((1, 1), rmax, F32)))
        yf = _rb(_rb(_cat([y[n] for n in range(KB)])) * rs)
        return _rb(xs.astype(F32) + jnp.where(rowsel, yf, 0.0))

    def routed():
        if "b" not in part:
            part["b"] = gate_input()
            part["row"] = jnp.sum(jnp.where(rowsel, part["b"], 0.0), axis=0, keepdims=True)
        return idx, part["row"]

    stage_z()
    for j in range(NPAIR):
        wf = wo_buf[j * 2 * DH:(j + 1) * 2 * DH, :].astype(F32)
        put_words(wo3, j * DH, _pk2(wf[:DH], wf[DH:]))
    ng = cfg.get("short_ffn") or NG
    sets = []
    for m in range(ng + 1):
        gu = [gate_up(w, j, h) for j in range(4 * m, 4 * m + 4) for w in (wg_buf, wu_buf) for h in range(2)
              ] if m < ng else []
        dn = [down(m - 1, n) for n in range(KB)] if m > 0 else []
        while gu or dn:
            sets += gu[:2] + dn[:1]
            gu, dn = gu[2:], dn[1:]

    outs = []
    for i in range(NTILE - 1):
        stage_b(i, zp)
        if i == 0:
            ffn_q.extend(sets)
        stage_q(i + 1)
        outs += stage_c(i, mid=(lambda: stage_b(NTILE - 1, zp)) if i == NTILE - 2 else None)
    assert not ffn_q
    last = stage_c(NTILE - 1, routed)

    for c in outs:
        c.wait()

    @pl.when(idx < S - T)
    def _():
        b = part["b"]
        res = x_buf[pl.ds(blk, RB), :].astype(F32) + s_buf[pl.ds(blk, RB), :] * (b * _sigmoid(b))
        fix_buf[...] = res.astype(BF16)
        c = pltpu.make_async_copy(fix_buf, out_hbm.at[pl.ds(blk, RB)], sem_o.at[1])
        c.start()
        c.wait()

    for c in last:
        c.wait()


def _build(cfg):
    S = cfg["S"]
    NB = S // LANE
    any_spec = pl.BlockSpec(memory_space=pl.ANY)
    scratch = [
        pltpu.VMEM((S, D), BF16),
        pltpu.VMEM((KB, S // 2, LANE), U32),
        pltpu.VMEM((S, D), BF16),
        pltpu.VMEM((3, D, D), BF16),
        pltpu.VMEM((H, DH, DH), BF16),
        pltpu.VMEM((D,), BF16),
        pltpu.VMEM((D, D), BF16),
        pltpu.VMEM((D, F), BF16),
        pltpu.VMEM((D, F), BF16),
        pltpu.VMEM((F, WDP), BF16),
        pltpu.VMEM((KB, D // 2, LANE), U32),
        pltpu.VMEM((KB, (D + RB) // 2, LANE), U32),
        pltpu.VMEM((KB, D // 2, LANE), U32),
        pltpu.VMEM((KB, D // 2, LANE), U32),
        pltpu.VMEM((NB, D, LANE), U32),
        pltpu.VMEM((NB, NPAIR * PR // 2, LANE), U32),
        pltpu.VMEM((NPAIR, 8, LANE), F32),
        pltpu.VMEM((NPAIR, LANE, LANE), F32),
        pltpu.VMEM((TB, D, LANE), U32),
        pltpu.VMEM((NPAIR, PR // 2, LANE), U32),
        pltpu.VMEM((KB, T // 2, LANE), U32),
        pltpu.VMEM((8, S), F32),
        pltpu.VMEM((S - T, D), F32),
        pltpu.VMEM((RB, D), BF16),
        pltpu.SemaphoreType.DMA((8,)),
        pltpu.SemaphoreType.DMA((3,)),
    ]
    return pl.pallas_call(
        functools.partial(_kernel, cfg),
        out_shape=jax.ShapeDtypeStruct((S, D), BF16),
        in_specs=[any_spec] * 8,
        out_specs=any_spec,
        scratch_shapes=scratch,
        compiler_params=pltpu.CompilerParams(vmem_limit_bytes=100 * 1024 * 1024),
        name=cfg.get("name", "hedgehog_mod"),
    )


@jax.jit
def pallas_recurrent_scan__linear_kernel_hedgehog__moe_arch_mod__prompt_kernel(
    A_x: jax.Array,
    A_wqkv: jax.Array,
    A_w_phi: jax.Array,
    A_wo: jax.Array,
    B_x: jax.Array,
    B_w_r: jax.Array,
    B_w_gate: jax.Array,
    B_w_up: jax.Array,
    B_w_down: jax.Array,
):
    del B_x
    S = CFG["S"]
    out = _build(CFG)(A_x.reshape(S, D), A_wqkv, A_w_phi, A_wo, B_w_r, B_w_gate, B_w_up, B_w_down)
    return out.reshape(1, S, D)
```

```python
import functools

import jax
import jax.numpy as jnp
from jax import lax
import jax.experimental.pallas as pl
import jax.experimental.pallas.tpu as pltpu

D, H, DH, F = 1024, 32, 32, 3584
LANE = 128
KB = D // LANE
KH = D // 2
T = 256
TB = T // LANE
NPAIR = H // 2
VR = 2 * DH + 8
PR = 2 * DH + 16
RB = 16
WDP = D + LANE
NG = F // KH
LOG2E = 1.4426950408889634
F32 = jnp.float32
BF16 = jnp.bfloat16
U32 = jnp.uint32

CFG = dict(S=2048, ln_chunk=16, opq="pkvw", mid_at=6, c_last=4, extra={}, qc_lag=2,
           b_lag=((4, 0),) * 5 + ((3, 16), (2, 48), (0, 0)), b_mid=((4, 0),) * 5 + ((3, 16), (2, 48), (2, 0)))


def _nt(a, b):
    return lax.dot_general(a, b, (((1,), (1,)), ((), ())), preferred_element_type=F32)


def _nn(a, b):
    return jnp.dot(a, b, preferred_element_type=F32)


def _rb(v):
    return v.astype(BF16).astype(F32)


def _recip(v):
    return pl.reciprocal(v, approx=True)


def _recip_nr(v):
    r = pl.reciprocal(v, approx=True)
    return r * (2.0 - v * r)


def _sigmoid(v):
    return 0.5 * jnp.tanh(0.5 * v) + 0.5


def _cat(parts):
    return jnp.concatenate(parts, axis=1)


def _pk(v):
    return pltpu.bitcast(v, U32)


def _up(v):
    return pltpu.bitcast(v, BF16)


def _pk2(lo, hi):
    return pltpu.bitcast(pltpu.pack_elementwise([lo, hi], packed_dtype=BF16), U32)


def _pair_allreduce(v, op):
    v = op(v, pltpu.roll(v, 2, 0))
    return op(v, pltpu.roll(v, 4, 0))


def _dual_softmax(p, z=None):
    n = p.shape[-1]
    p = p.reshape(8, 8, n)
    mx = _pair_allreduce(jnp.max(p, axis=0), jnp.maximum)
    mn = _pair_allreduce(jnp.min(p, axis=0), jnp.minimum)
    ep = jnp.exp2(p - mx[None])
    en = jnp.exp2(mn[None] - p)
    rp = _recip(_pair_allreduce(jnp.sum(ep, axis=0), jnp.add))
    rn = _recip(_pair_allreduce(jnp.sum(en, axis=0), jnp.add))
    if z is not None:
        dp = _pair_allreduce(jnp.sum(ep * z[0].reshape(8, 8, n), axis=0), jnp.add)
        dn = _pair_allreduce(jnp.sum(en * z[1].reshape(8, 8, n), axis=0), jnp.add)
        rd = _recip(rp * dp + rn * dn + 1e-6)
        rp = rp * rd
        rn = rn * rd
    return (ep * rp[None]).reshape(64, n), (en * rn[None]).reshape(64, n)


def _kernel(cfg, x_hbm, wqkv_hbm, phi_hbm, wo_hbm, wr_hbm, wg_hbm, wu_hbm, wd_hbm, out_hbm,
            x_buf, xn3, out_buf, wraw, phi_buf, wr_buf, wo_buf, wg_buf, wu_buf, wd_buf,
            wq3, wk3, wv3, phik3, vaug3, zrow, zbuf, phiq3, lmat, o3, r_buf, s_buf, fix_buf,
            sem, sem_o):
    S = cfg["S"]
    NB = S // LANE
    NTILE = S // T

    def cp(src, dst, slot):
        return pltpu.make_async_copy(src, dst, sem.at[slot])

    def x_rows(r0, n, slot):
        return cp(x_hbm.at[pl.ds(r0, n)], x_buf.at[pl.ds(r0, n)], slot)

    def wk_cols(g0, g1, slot):
        n = (g1 - g0) * LANE
        return [cp(wqkv_hbm.at[pl.ds(r, KH), pl.ds(D + g0 * LANE, n)],
                   wraw.at[1, pl.ds(r, KH), pl.ds(g0 * LANE, n)], slot) for r in (0, KH)]

    groups = [
        [x_rows(0, 64, 0), x_rows(64, 64, 0), cp(wr_hbm, wr_buf, 0),
         cp(phi_hbm.at[pl.ds(0, 8)], phi_buf.at[pl.ds(0, 8)], 0)],
        wk_cols(0, 2, 1),
        [x_rows(b * LANE, LANE, 2) for b in range(1, 2 * TB)],
        [cp(phi_hbm.at[pl.ds(8, H - 8)], phi_buf.at[pl.ds(8, H - 8)], 3)] + wk_cols(2, 4, 3),
        wk_cols(4, 8, 4) + [x_rows(2 * T, T, 4)],
        [cp(wqkv_hbm.at[:, pl.ds(2 * D, D)], wraw.at[2], 5), x_rows(3 * T, T, 5)],
        [x_rows(4 * T, S - 4 * T, 6), cp(wqkv_hbm.at[:, pl.ds(0, D)], wraw.at[0], 6), cp(wo_hbm, wo_buf.at[:, pl.ds(0, D)], 6)],
        [cp(wg_hbm, wg_buf, 7), cp(wu_hbm, wu_buf, 7), cp(wd_hbm, wd_buf.at[:, pl.ds(0, D)], 7)],
    ]
    for grp in groups:
        for c in grp:
            c.start()

    def arrive(k):
        for c in groups[k]:
            c.wait()

    for b in range(NB):
        for j in range(NPAIR):
            vaug3[b, j * VR + 2 * DH:(j + 1) * VR, :] = jnp.ones((8, LANE), F32)

    def put_rows(dst, r0, val):
        n = val.shape[0]
        for k in range(KB):
            dst[k, r0 // 2:(r0 + n) // 2, :] = _pk(val[:, k * LANE:(k + 1) * LANE])

    def put_words(dst, w0, val):
        for k in range(KB):
            dst[k, w0:w0 + val.shape[0], :] = val[:, k * LANE:(k + 1) * LANE]

    def get_rows(src, r0, n, k0=0, k1=KB):
        return _cat([_up(src[k, r0 // 2:(r0 + n) // 2, :]) for k in range(k0, k1)])

    def layernorm(row0, n, ch):
        z = None
        eps = _rb(jnp.full((1, 1), 1e-5, F32))
        for r0 in range(row0, row0 + n, ch):
            xf = x_buf[r0:r0 + ch, :].astype(F32)
            mean = jnp.sum(xf, axis=-1, keepdims=True) * (1.0 / D)
            if z is not None:
                mean = mean + z
            c = xf - mean
            var = jnp.sum(c * c, axis=-1, keepdims=True) * (1.0 / D)
            rs = _recip_nr(_rb(jnp.sqrt(_rb(_rb(var) + eps))))
            z = jnp.where(rs < 0.0, 1.0, 0.0)
            put_rows(xn3, r0, (_rb(xf - _rb(mean)) * rs).astype(BF16))

    er = lax.broadcasted_iota(jnp.int32, (LANE, DH), 0)
    ec = lax.broadcasted_iota(jnp.int32, (LANE, DH), 1)
    eye4 = jnp.where(er % DH == ec, 1.0, 0.0).astype(BF16)
    br = lax.broadcasted_iota(jnp.int32, (LANE, LANE), 0)
    bc = lax.broadcasted_iota(jnp.int32, (LANE, LANE), 1)
    bmask = (2 * ((br % (2 * DH)) // DH) + br // (2 * DH)) == bc // DH
    bd = {}

    def blockdiag(g0, g1):
        for g in range(g0, g1):
            t = _nt(eye4, phi_buf[4 * g:4 * g + 4].reshape(LANE, DH))
            bd[g] = jnp.where(bmask, t, 0.0).astype(BF16)

    def fold(j, dst, g0, g1):
        for g in range(g0, g1):
            res = _nt(bd[g], wraw[j, :, g * LANE:(g + 1) * LANE]) * LOG2E
            put_words(dst, g * 64, _pk2(res[:64], res[64:]))

    def keys(b, g0=0, g1=KB):
        r0, r1 = g0 * LANE, g1 * LANE
        last = g1 == KB
        pt = _nt(get_rows(wk3, r0, r1 - r0 + (RB if last else 0)), get_rows(xn3, b * LANE, LANE))
        if last:
            r_buf[:, b * LANE:(b + 1) * LANE] = pt[r1 - r0:r1 - r0 + 8, :]
        for j in range(r0 // 64, r1 // 64):
            rows = slice(j * 64, (j + 1) * 64)
            phik3[b, rows, :] = _pk2(*_dual_softmax(pt[j * 64 - r0:(j + 1) * 64 - r0, :]))

    def stage_k(i, g0=0, g1=KB):
        for b in range(i * TB, (i + 1) * TB):
            keys(b, g0, g1)

    def stage_v(i):
        for b in range(i * TB, (i + 1) * TB):
            wv = _cat([_up(wv3[k, pl.ds(zw, D // 2), :]) for k in range(KB)])
            vt = _nt(wv, get_rows(xn3, b * LANE, LANE))
            for j in range(NPAIR):
                vaug3[b, j * VR:j * VR + 2 * DH, :] = vt[j * 2 * DH:(j + 1) * 2 * DH]

    ffn_q = []
    pending = []

    def ffn_step(lag, off=0):
        if ffn_q and lag:
            pending.append([lag, off, ffn_q.pop(0)()])

    def lhs(words):
        for p in pending:
            p[0] -= 1
        for p in [p for p in pending if p[0] == 0]:
            pending.remove(p)
            w, off = words[0], p[1]
            tied = w[off:off + 8] ^ (pltpu.bitcast(p[2], U32) & zvec[0])
            words = [jnp.concatenate(([w[:off]] if off else []) + [tied, w[off + 8:]], axis=0)] + words[1:]
        return _cat([_up(w) for w in words])

    zvec = []

    def stage_q(i):
        for bl in range(TB):
            r0 = (i * TB + bl) * LANE
            pt = _nt(lhs([wq3[k] for k in range(KB)]), get_rows(xn3, r0, LANE))
            for j in range(NPAIR):
                rows = slice(j * 64, (j + 1) * 64)
                z = None if i == 0 else [zbuf[j, pl.ds(t, 64, stride=2), :] for t in range(2)]
                phiq3[bl, rows, :] = _pk2(*_dual_softmax(pt[rows, :], z))

    def stage_kv(zv, zk):
        lr = lax.broadcasted_iota(jnp.int32, (PR, LANE), 0)
        lc = lax.broadcasted_iota(jnp.int32, (PR, LANE), 1)
        keep = jnp.where(lr < 2 * DH, lr // DH, (lr - 2 * DH) // 8) == (lc // 2) % 2
        for j in range(NPAIR):
            va = _cat([vaug3[b, pl.ds(zv + j * VR, VR), :] for b in range(NB)])
            pk = _cat([_up(phik3[b, pl.ds(zk + j * 64, 64), :]) for b in range(NB)])
            kvt = _nt(va, pk)
            z = kvt[2 * DH:, :]
            lmat[j] = _pk(jnp.where(keep, jnp.concatenate([kvt, z], axis=0), 0.0).astype(BF16))
            zrow[j] = z

    def stage_z():
        for j in range(NPAIR):
            zbuf[j] = jnp.concatenate([zrow[j]] * (LANE // 8), axis=0).T

    def stage_b(i, zp, mid=False):
        for g in range(KB):
            parts = []
            for j in (2 * g, 2 * g + 1):
                pq = _cat([_up(phiq3[bl, pl.ds(zp + j * 64, 64), :]) for bl in range(TB)])
                if i == 0:
                    nt = _nn(_up(lmat[j]), pq)
                    for h in range(2):
                        den = nt[2 * DH + 8 * h:2 * DH + 8 * h + 8, :] + 1e-6
                        num = nt[h * DH:(h + 1) * DH, :].reshape(4, 8, T)
                        parts.append((num * _recip(den)[None]).reshape(DH, T))
                else:
                    lw = lmat[j, 0:DH, :]
                    parts.append(_nn(lhs([lw]) if j % 2 == 0 else _up(lw), pq))
            if i > 0:
                ffn_step(*(cfg["b_mid"] if mid else cfg["b_lag"])[g])
            o3[g] = _pk(jnp.concatenate(parts, axis=0).T.astype(BF16))

    def stage_c(i, routed=None, mid=None):
        r0 = i * T
        o = [o3[k] for k in range(KB)]
        copies = []
        for n in range(0, KB, 2):
            if mid is not None and n == cfg["mid_at"]:
                mid()
            parts = []
            for m in (n, n + 1):
                halves = []
                for h in range(TB):
                    ow = [w[h * 64:(h + 1) * 64] for w in o]
                    halves.append(_nn(lhs(ow), wo_buf[:, m * LANE:(m + 1) * LANE]))
                    before_b = h == TB - 1 and (m == KB - 1 or (mid is not None and m + 1 == cfg["mid_at"]))
                    for _ in range(cfg["extra"].get((i, m, h), 1)):
                        ffn_step(cfg["c_last"] if before_b else 2)
                parts.append(jnp.concatenate(halves, axis=0))
            s = _cat(parts)
            cols = slice(n * LANE, (n + 2) * LANE)
            b = get_rows(xn3, r0, T, n, n + 2).astype(F32)
            if routed is None:
                s_buf[r0:r0 + T, cols] = s
            else:
                idx, bsel = routed()
                sel = (lax.broadcasted_iota(jnp.int32, (T, 2 * LANE), 0) + r0) == idx
                b = jnp.where(sel, bsel[:, cols], b)
            res = x_buf[r0:r0 + T, cols].astype(F32) + s * (b * _sigmoid(b))
            out_buf[r0:r0 + T, cols] = res.astype(BF16)
            if routed is not None:
                win = (pl.ds(r0, T), pl.ds(n * LANE, 2 * LANE))
                copies.append(pltpu.make_async_copy(out_buf.at[win], out_hbm.at[win], sem_o.at[2]))
                copies[-1].start()
        if routed is None:
            copies.append(pltpu.make_async_copy(out_buf.at[pl.ds(r0, T)], out_hbm.at[pl.ds(r0, T)], sem_o.at[0]))
            copies[-1].start()
        return copies

    lc = cfg["ln_chunk"]
    arrive(0)
    layernorm(0, LANE, LANE)
    wrf = wr_buf[...].reshape(1, D).astype(F32)
    for k in range(KB):
        wr8 = jnp.broadcast_to(wrf[:, k * LANE:(k + 1) * LANE], (8, LANE))
        wk3[k, D // 2:(D + RB) // 2, :] = _pk2(wr8, wr8)
    sign = lax.shift_right_logical(pltpu.bitcast(wrf[:, 0:LANE], jnp.int32), 31)
    zrt = pl.multiple_of(lax.shift_right_logical(jnp.max(sign), 1), 8)
    zvec.append(jnp.full((8, LANE), zrt, jnp.int32).astype(U32))
    zp, zk, zv, zw = [zrt if t in cfg["opq"] else 0 for t in "pkvw"]
    blockdiag(0, 2)
    arrive(1)
    fold(1, wk3, 0, 2)
    keys(0, 0, 2)
    arrive(2)
    for b in range(1, 2 * TB):
        layernorm(b * LANE, LANE, LANE)
        keys(b, 0, 2)
    arrive(3)
    blockdiag(2, KB)
    fold(1, wk3, 2, 4)
    for b in range(2 * TB):
        keys(b, 2, 4)
    arrive(4)
    fold(1, wk3, 4, 8)
    for b in range(2 * TB):
        keys(b, 4, 8)
    layernorm(2 * T, T, lc)
    arrive(5)
    for g in range(KB):
        put_rows(wv3, g * LANE, wraw[2, :, g * LANE:(g + 1) * LANE].T)
    stage_k(2)
    stage_v(0)
    layernorm(3 * T, T, lc)
    stage_v(1)
    stage_k(3)
    stage_v(2)
    arrive(6)
    for i in range(3, NTILE):
        if i > 3:
            stage_k(i)
        if i + 1 < NTILE:
            layernorm((i + 1) * T, T, lc)
        stage_v(i)
        if i == 3:
            fold(0, wq3, 0, KB)
    stage_q(0)
    stage_kv(zv, zk)

    arrive(7)
    r = _rb(r_buf[0:1, :])
    rmax = jnp.max(r)
    pos = lax.broadcasted_iota(jnp.int32, (1, S), 1)
    idx = jnp.clip(jnp.min(jnp.where(r == rmax, pos, S)), 0, S - 1)
    blk = pl.multiple_of((idx // RB) * RB, RB)
    blk2 = pl.multiple_of((idx // RB) * (RB // 2), RB // 2)
    xblk = _cat([_up(xn3[k, pl.ds(blk2, RB // 2), :]) for k in range(KB)]).astype(F32)
    rowsel = (lax.broadcasted_iota(jnp.int32, (RB, D), 0) + blk) == idx
    xs = jnp.broadcast_to(jnp.sum(jnp.where(rowsel, xblk, 0.0), axis=0, keepdims=True), (8, D))
    part, act, y = {}, {}, {}

    def gate_up(w_buf, j, h):
        def f():
            v = _nn(xs[:, h * KH:(h + 1) * KH], w_buf[h * KH:(h + 1) * KH, j * LANE:(j + 1) * LANE])
            key = (w_buf is wu_buf, j)
            part[key] = v if h == 0 else _rb(part[key] + v)
            if h == 1 and w_buf is wu_buf:
                hg = part.pop((False, j))
                act[j] = _rb(_rb(hg * _sigmoid(hg)) * part.pop(key))
            return v
        return f

    def down(m, n):
        def f():
            a = _cat([act[j] for j in range(4 * m, 4 * m + 4)])
            v = _nn(a, wd_buf[m * KH:(m + 1) * KH, n * LANE:(n + 1) * LANE])
            y[n] = v if m == 0 else y[n] + v
            return v
        return f

    def routed():
        if "row" not in part:
            rs = _rb(_sigmoid(jnp.full((1, 1), rmax, F32)))
            yf = _rb(_rb(_cat([y[n] for n in range(KB)])) * rs)
            part["row"] = _rb(xs + yf)[0:1, :]
        return idx, part["row"]

    stage_z()
    ng = cfg.get("short_ffn") or NG
    sets = []
    for m in range(ng + 1):
        gu = [gate_up(w, j, h) for j in range(4 * m, 4 * m + 4) for w in (wg_buf, wu_buf) for h in range(2)
              ] if m < ng else []
        dn = [down(m - 1, n) for n in range(KB)] if m > 0 else []
        while gu or dn:
            sets += gu[:2] + dn[:1]
            gu, dn = gu[2:], dn[1:]

    outs = []
    for i in range(NTILE - 1):
        stage_b(i, zp)
        if i == 0:
            ffn_q.extend(sets)
        stage_q(i + 1)
        ffn_step(cfg["qc_lag"])
        outs += stage_c(i, mid=(lambda: stage_b(NTILE - 1, zp, True)) if i == NTILE - 2 else None)
    assert not ffn_q, len(ffn_q)
    last = stage_c(NTILE - 1, routed)

    for c in outs:
        c.wait()

    @pl.when(idx < S - T)
    def _():
        b = jnp.where(rowsel, part["row"], xblk)
        res = x_buf[pl.ds(blk, RB), :].astype(F32) + s_buf[pl.ds(blk, RB), :] * (b * _sigmoid(b))
        fix_buf[...] = res.astype(BF16)
        c = pltpu.make_async_copy(fix_buf, out_hbm.at[pl.ds(blk, RB)], sem_o.at[1])
        c.start()
        c.wait()

    for c in last:
        c.wait()


def _build(cfg):
    S = cfg["S"]
    NB = S // LANE
    any_spec = pl.BlockSpec(memory_space=pl.ANY)
    scratch = [
        pltpu.VMEM((S, D), BF16),
        pltpu.VMEM((KB, S // 2, LANE), U32),
        pltpu.VMEM((S, D), BF16),
        pltpu.VMEM((3, D, D), BF16),
        pltpu.VMEM((H, DH, DH), BF16),
        pltpu.VMEM((D,), BF16),
        pltpu.VMEM((D, WDP), BF16),
        pltpu.VMEM((D, F), BF16),
        pltpu.VMEM((D, F), BF16),
        pltpu.VMEM((F, WDP), BF16),
        pltpu.VMEM((KB, D // 2, LANE), U32),
        pltpu.VMEM((KB, (D + RB) // 2, LANE), U32),
        pltpu.VMEM((KB, D // 2, LANE), U32),
        pltpu.VMEM((NB, D, LANE), U32),
        pltpu.VMEM((NB, NPAIR * VR, LANE), F32),
        pltpu.VMEM((NPAIR, 8, LANE), F32),
        pltpu.VMEM((NPAIR, LANE, LANE), F32),
        pltpu.VMEM((TB, D, LANE), U32),
        pltpu.VMEM((NPAIR, PR // 2, LANE), U32),
        pltpu.VMEM((KB, T // 2, LANE), U32),
        pltpu.VMEM((8, S), F32),
        pltpu.VMEM((S - T, D), F32),
        pltpu.VMEM((RB, D), BF16),
        pltpu.SemaphoreType.DMA((8,)),
        pltpu.SemaphoreType.DMA((3,)),
    ]
    return pl.pallas_call(
        functools.partial(_kernel, cfg),
        out_shape=jax.ShapeDtypeStruct((S, D), BF16),
        in_specs=[any_spec] * 8,
        out_specs=any_spec,
        scratch_shapes=scratch,
        compiler_params=pltpu.CompilerParams(vmem_limit_bytes=100 * 1024 * 1024),
        name=cfg.get("name", "hedgehog_mod"),
    )


@jax.jit
def pallas_recurrent_scan__linear_kernel_hedgehog__moe_arch_mod__prompt_kernel(
    A_x: jax.Array,
    A_wqkv: jax.Array,
    A_w_phi: jax.Array,
    A_wo: jax.Array,
    B_x: jax.Array,
    B_w_r: jax.Array,
    B_w_gate: jax.Array,
    B_w_up: jax.Array,
    B_w_down: jax.Array,
):
    del B_x
    S = CFG["S"]
    out = _build(CFG)(A_x.reshape(S, D), A_wqkv, A_w_phi, A_wo, B_w_r, B_w_gate, B_w_up, B_w_down)
    return out.reshape(1, S, D)
```

```python
import functools

import jax
import jax.numpy as jnp
from jax import lax
import jax.experimental.pallas as pl
import jax.experimental.pallas.tpu as pltpu

D, H, DH, F = 1024, 32, 32, 3584
LANE = 128
KB = D // LANE
KH = D // 2
T = 256
TB = T // LANE
NPAIR = H // 2
VR = 2 * DH + 8
PR = 2 * DH + 16
RB = 16
WDP = D + LANE
NG = F // KH
LOG2E = 1.4426950408889634
F32 = jnp.float32
BF16 = jnp.bfloat16
U32 = jnp.uint32

CFG = dict(S=2048, ln_chunk=16, ln1=64, ln2=32, round_d=False, xn_u32=False, plan='A', p1='K2 V0 L3 K3 V1 V2 | F L4 V3 K4 L5 V4 K5 L6 V5 K6 L7 V6 K7 V7', k_gate=(None, None), q_gate=(None, 7), o_pin=(1, 480), o_opq=False, z_pin=0, slab=False, zstride=False, q_u32=False, b_rev=False, b_prod=0, q_split=(8, 1), k_split=(16, 16), tree='', park='', park_split=512, one_rcp=True, opq='', mid_at=6, wv_bf16=True, zalign=1024, c_last=4, extra={}, qc_lag=2,
           b_lag=((4, 0),) * 5 + ((3, 16), (2, 48), (0, 0)), b_mid=((4, 0),) * 5 + ((3, 16), (2, 48), (2, 0)))


def _nt(a, b):
    return lax.dot_general(a, b, (((1,), (1,)), ((), ())), preferred_element_type=F32)


def _nn(a, b):
    return jnp.dot(a, b, preferred_element_type=F32)


def _rb(v):
    return v.astype(BF16).astype(F32)


def _recip(v):
    return pl.reciprocal(v, approx=True)


def _recip_nr(v):
    r = pl.reciprocal(v, approx=True)
    return r * (2.0 - v * r)


def _sigmoid(v):
    return 0.5 * jnp.tanh(0.5 * v) + 0.5


def _cat(parts):
    return jnp.concatenate(parts, axis=1)


def _pk(v):
    return pltpu.bitcast(v, U32)


def _up(v):
    return pltpu.bitcast(v, BF16)


def _pair_allreduce(v, op):
    v = op(v, pltpu.roll(v, 2, 0))
    return op(v, pltpu.roll(v, 4, 0))


def _tsum(v, tree):
    if not tree:
        return jnp.sum(v, axis=0)
    return ((v[0] + v[1]) + (v[2] + v[3])) + ((v[4] + v[5]) + (v[6] + v[7]))


def _dual_softmax(p, z=None, tree=False, one_rcp=True, slab=False, gates=(None, None)):
    n = p.shape[-1]
    p = p.reshape(8, 8, n)
    def gate(v, g):
        return v if g is None else pltpu.bitcast(pltpu.bitcast(v, U32) ^ g, F32)

    mx = gate(_pair_allreduce(jnp.max(p, axis=0), jnp.maximum), gates[0])
    mn = _pair_allreduce(jnp.min(p, axis=0), jnp.minimum)
    ep = jnp.exp2(p - mx[None])
    en = jnp.exp2(mn[None] - p)
    sp = _pair_allreduce(_tsum(ep, tree), jnp.add)
    sn = _pair_allreduce(_tsum(en, tree), jnp.add)
    if z is None:
        rp, rn = _recip(gate(sp, gates[1])), _recip(sn)
    else:
        if slab:
            z4 = z.reshape(8, 2, 8, n)
            zpos, zneg = z4[:, 0], z4[:, 1]
        else:
            zpos, zneg = z[:64].reshape(8, 8, n), z[64:].reshape(8, 8, n)
        dp = _pair_allreduce(_tsum(ep * zpos, tree), jnp.add)
        dn = _pair_allreduce(_tsum(en * zneg, tree), jnp.add)
        if one_rcp:
            rd = _recip(gate(dp * sn + (dn + 1e-6 * sn) * sp, gates[1]))
            rp, rn = sn * rd, sp * rd
        else:
            rp, rn = _recip(sp), _recip(sn)
            rd = _recip(rp * dp + rn * dn + 1e-6)
            rp, rn = rp * rd, rn * rd
    pos, neg = ep * rp[None], en * rn[None]
    if slab:
        return jnp.concatenate([v for k in range(8) for v in (pos[k], neg[k])], axis=0).astype(BF16)
    return jnp.concatenate([pos, neg], axis=0).reshape(LANE, n).astype(BF16)


def _kernel(cfg, x_hbm, wqkv_hbm, phi_hbm, wo_hbm, wr_hbm, wg_hbm, wu_hbm, wd_hbm, out_hbm,
            x_buf, xn3, out_buf, wraw, phi_buf, wr_buf, wo_buf, wg_buf, wu_buf, wd_buf,
            wq3, wk3, wv3, phik, vaug3, zrow, zbuf, phiq, lmat, o3, r_buf, s_buf, fix_buf, pb0, pb1, pb2, pb3,
            sem, sem_o):
    S = cfg["S"]
    NB = S // LANE
    NTILE = S // T

    def cp(src, dst, slot):
        return pltpu.make_async_copy(src, dst, sem.at[slot])

    def x_rows(r0, n, slot):
        return cp(x_hbm.at[pl.ds(r0, n)], x_buf.at[pl.ds(r0, n)], slot)

    def wk_cols(g0, g1, slot):
        n = (g1 - g0) * LANE
        return [cp(wqkv_hbm.at[pl.ds(r, KH), pl.ds(D + g0 * LANE, n)],
                   wraw.at[1, pl.ds(r, KH), pl.ds(g0 * LANE, n)], slot) for r in (0, KH)]

    phi_a = cp(phi_hbm.at[pl.ds(0, 8)], phi_buf.at[pl.ds(0, 8)], 0)
    if cfg["plan"] == "F":
        head = [
            [x_rows(0, LANE, 0), x_rows(LANE, LANE, 0), cp(wr_hbm, wr_buf, 0), phi_a],
            wk_cols(0, 2, 1),
            [cp(phi_hbm.at[pl.ds(8, H - 8)], phi_buf.at[pl.ds(8, H - 8)], 2)] + wk_cols(2, 4, 2),
            [x_rows(T, T, 3)] + wk_cols(4, 6, 3),
            wk_cols(6, 8, 4) + [x_rows(2 * T, T, 4)],
        ]
    else:
        head = [
            [x_rows(0, LANE, 0), cp(wr_hbm, wr_buf, 0), phi_a],
            wk_cols(0, 2, 1),
            [x_rows(LANE, 3 * LANE, 2)],
            [cp(phi_hbm.at[pl.ds(8, H - 8)], phi_buf.at[pl.ds(8, H - 8)], 3)] + wk_cols(2, 4, 3),
            wk_cols(4, 8, 4) + [x_rows(2 * T, T, 4)],
        ]
    groups = head + [
        [cp(wqkv_hbm.at[:, pl.ds(2 * D, D)], wraw.at[2], 5), x_rows(3 * T, T, 5)],
        [x_rows(4 * T, S - 4 * T, 6), cp(wqkv_hbm.at[:, pl.ds(0, D)], wraw.at[0], 6),
         cp(wo_hbm, wo_buf.at[:, pl.ds(0, D)], 6)],
        [cp(wg_hbm, wg_buf, 7), cp(wu_hbm, wu_buf, 7), cp(wd_hbm, wd_buf.at[:, pl.ds(0, D)], 7)],
    ]
    for grp in groups:
        for c in grp:
            c.start()

    def arrive(k):
        for c in groups[k]:
            c.wait()

    for b in range(NB):
        for j in range(NPAIR):
            vaug3[b, j * VR + 2 * DH:(j + 1) * VR, :] = jnp.ones((8, LANE), F32)

    def put_rows(dst, r0, val):
        n = val.shape[0]
        for k in range(KB):
            dst[k, r0 // 2:(r0 + n) // 2, :] = _pk(val[:, k * LANE:(k + 1) * LANE])

    def get_rows(src, r0, n, k0=0, k1=KB):
        return _cat([_up(src[k, r0 // 2:(r0 + n) // 2, :]) for k in range(k0, k1)])

    def xn_rows(r0, n, k0=0, k1=KB):
        if cfg["xn_u32"]:
            w0 = r0 // 2 if isinstance(r0, int) else pl.multiple_of(r0 // 2, RB // 2)
            return _cat([_up(xn3[k, pl.ds(w0, n // 2), :]) for k in range(k0, k1)])
        return _cat([xn3[k, pl.ds(r0, n), :] for k in range(k0, k1)])

    def layernorm(row0, n, ch):
        z = None
        eps = _rb(jnp.full((1, 1), 1e-5, F32))
        for r0 in range(row0, row0 + n, ch):
            xf = x_buf[r0:r0 + ch, :].astype(F32)
            mean = jnp.sum(xf, axis=-1, keepdims=True) * (1.0 / D)
            if z is not None:
                mean = mean + z
            c = xf - mean
            var = jnp.sum(c * c, axis=-1, keepdims=True) * (1.0 / D)
            rs = _recip_nr(_rb(jnp.sqrt(_rb(_rb(var) + eps))))
            z = jnp.where(rs < 0.0, 1.0, 0.0)
            d = xf - _rb(mean)
            xn = ((_rb(d) if cfg["round_d"] else d) * rs).astype(BF16)
            if cfg["xn_u32"]:
                put_rows(xn3, r0, xn)
            else:
                for k in range(KB):
                    xn3[k, r0:r0 + ch, :] = xn[:, k * LANE:(k + 1) * LANE]

    er = lax.broadcasted_iota(jnp.int32, (LANE, DH), 0)
    ec = lax.broadcasted_iota(jnp.int32, (LANE, DH), 1)
    eye4 = jnp.where((er % (2 * DH)) // 2 == ec, 1.0, 0.0).astype(BF16)
    br = lax.broadcasted_iota(jnp.int32, (LANE, LANE), 0)
    bc = lax.broadcasted_iota(jnp.int32, (LANE, LANE), 1)
    bmask = (2 * (br // (2 * DH)) + br % 2) == bc // DH
    bd = {}

    def blockdiag(g0, g1):
        for g in range(g0, g1):
            t = _nt(eye4, phi_buf[4 * g:4 * g + 4].reshape(LANE, DH))
            bd[g] = jnp.where(bmask, t, 0.0).astype(BF16)

    def fold(j, dst, g0, g1):
        for g in range(g0, g1):
            res = _nt(bd[g], wraw[j, :, g * LANE:(g + 1) * LANE]) * LOG2E
            put_rows(dst, g * LANE, res.astype(BF16))

    zz = [0, 0]
    zvec = []
    pbufs = (pb0, pb1, pb2, pb3)

    def gates(pt, row, end, which):
        out = []
        for a in which:
            ok = a is not None and row + 8 * a < end
            out.append(pltpu.bitcast(pt[row + 8 * a:row + 8 * a + 8], U32) & zvec[0] if ok else None)
        return out

    def park(v, slot):
        n = v.shape[0]
        h = cfg["park_split"] if n > cfg["park_split"] else n
        out = []
        for q, (a, b) in enumerate(((0, h), (h, n))):
            if b > a:
                pb = pbufs[2 * slot + q]
                pb[0:b - a, :] = v[a:b]
                out.append(pb[pl.ds(zz[1], b - a), :])
        return jnp.concatenate(out, axis=0)

    def phi_loc(refs, split, b, j):
        pj, pb = split
        return refs[(b // pb) * (NPAIR // pj) + j // pj], b % pb, j % pj

    def put_phi(refs, split, b, j, val):
        ref, b, j = phi_loc(refs, split, b, j)
        if ref.dtype == U32:
            ref[b, j * 64:(j + 1) * 64, :] = _pk(val)
        else:
            ref[b, j * LANE:(j + 1) * LANE, :] = val

    def get_phi(refs, split, b, j, z):
        ref, b, j = phi_loc(refs, split, b, j)
        if ref.dtype == U32:
            return _up(ref[b, pl.ds(z + j * 64, 64), :])
        return ref[b, pl.ds(z + j * LANE, LANE), :]

    def keys(b, g0=0, g1=KB):
        r0, r1 = g0 * LANE, g1 * LANE
        last = g1 == KB
        n = r1 - r0 + (RB if last else 0)
        if "k" in cfg["park"]:
            pt = park(_nt(get_rows(wk3, r0, n, 0, 4), xn_rows(b * LANE, LANE, 0, 4)), b % 2)
            pt = pt + _nt(get_rows(wk3, r0, n, 4, KB), xn_rows(b * LANE, LANE, 4, KB))
        else:
            pt = _nt(get_rows(wk3, r0, n), xn_rows(b * LANE, LANE))
        if last:
            r_buf[:, b * LANE:(b + 1) * LANE] = pt[r1 - r0:r1 - r0 + 8, :]
        for j in range(r0 // 64, r1 // 64):
            put_phi(phik, cfg['k_split'], b, j, _dual_softmax(pt[j * 64 - r0:(j + 1) * 64 - r0, :], None, 'k' in cfg['tree'], False, cfg['slab'],
                                                                gates(pt, (j + 1) * 64 - r0, r1 - r0, cfg['k_gate'])))

    def stage_k(i, g0=0, g1=KB):
        for b in range(i * TB, (i + 1) * TB):
            keys(b, g0, g1)

    def stage_v(i):
        for b in range(i * TB, (i + 1) * TB):
            if wv3.dtype == BF16:
                wv = _cat([wv3[k] for k in range(KB)])
            else:
                wv = _cat([_up(wv3[k, pl.ds(zw, D // 2), :]) for k in range(KB)])
            vt = _nt(wv, xn_rows(b * LANE, LANE))
            for j in range(NPAIR):
                vaug3[b, j * VR:j * VR + 2 * DH, :] = vt[j * 2 * DH:(j + 1) * 2 * DH]

    ffn_q = []
    pending = []

    def ffn_step(lag, off=0):
        if ffn_q and lag:
            pending.append([lag, off, ffn_q.pop(0)()])

    def lhs(words):
        for p in pending:
            p[0] -= 1
        for p in [p for p in pending if p[0] == 0]:
            pending.remove(p)
            w, off = words[0], p[1]
            if w.dtype == F32:
                off *= 2
            tied = pltpu.bitcast(w[off:off + 8], U32) ^ (pltpu.bitcast(p[2], U32) & zvec[0])
            tied = pltpu.bitcast(tied, w.dtype)
            words = [jnp.concatenate(([w[:off]] if off else []) + [tied, w[off + 8:]], axis=0)] + words[1:]
        return _cat([_up(w) if w.dtype == U32 else w for w in words])


    def stage_q(i):
        for bl in range(TB):
            r0 = (i * TB + bl) * LANE
            if "q" in cfg["park"]:
                pt = park(_nt(lhs([wq3[k] for k in range(4)]), xn_rows(r0, LANE, 0, 4)), bl)
                pt = pt + _nt(get_rows(wq3, 0, D, 4, KB), xn_rows(r0, LANE, 4, KB))
            else:
                pt = _nt(lhs([wq3[k] for k in range(KB)]), xn_rows(r0, LANE))
            for j in range(NPAIR):
                z = None if i == 0 else zbuf[j, pl.ds(0, LANE, stride=2) if cfg['zstride'] else pl.ds(zz[0], LANE), :]
                put_phi(phiq, cfg['q_split'], bl, j, _dual_softmax(pt[j * 64:(j + 1) * 64, :], z, 'q' in cfg['tree'], cfg['one_rcp'], cfg['slab'],
                                                                 gates(pt, (j + 1) * 64, D, cfg['q_gate'])))

    def stage_kv(zv, zk):
        lr = lax.broadcasted_iota(jnp.int32, (PR, LANE), 0)
        lc = lax.broadcasted_iota(jnp.int32, (PR, LANE), 1)
        keep = jnp.where(lr < 2 * DH, lr // DH, (lr - 2 * DH) // 8) == lc % 2
        for j in range(NPAIR):
            va = _cat([vaug3[b, pl.ds(zv + j * VR, VR), :] for b in range(NB)])
            pk = _cat([get_phi(phik, cfg['k_split'], b, j, zk) for b in range(NB)])
            kvt = _nt(va, pk)
            z = kvt[2 * DH:, :]
            lmat[j] = _pk(jnp.where(keep, jnp.concatenate([kvt, z], axis=0), 0.0).astype(BF16))
            zrow[j] = z

    def stage_z():
        for j in range(NPAIR):
            zbuf[j, pl.ds(0, LANE, stride=2) if cfg['zstride'] else pl.ds(0, LANE), :] = jnp.concatenate([zrow[j]] * (LANE // 8), axis=0).T

    def stage_b(i, zp, mid=False):
        if cfg["b_prod"] and i > 0:
            keep = {}
            for gi in range(KB):
                bl, q = divmod(gi, 4)
                parts = []
                for j in range(4 * q, 4 * q + 4):
                    lw = lmat[j, 0:DH, :]
                    parts.append(_nn(lhs([lw]) if j % 4 == 0 else _up(lw),
                                     get_phi(phiq, cfg['q_split'], bl, j, zp)))
                ffn_step(*(cfg["b_mid"] if mid else cfg["b_lag"])[gi])
                for h in range(2):
                    g = 2 * q + h
                    ot = jnp.concatenate(parts[2 * h:2 * h + 2], axis=0)
                    if cfg["b_prod"] == 1:
                        o3[g, bl * 64:(bl + 1) * 64, :] = _pk(ot.T.astype(BF16))
                    elif bl == 0:
                        keep[g] = ot
                    else:
                        o3[g] = _pk(_cat([keep[g], ot]).T.astype(BF16))
            return
        for gi, g in enumerate(range(KB - 1, -1, -1) if cfg["b_rev"] else range(KB)):
            parts = []
            for j in (2 * g, 2 * g + 1):
                pq = _cat([get_phi(phiq, cfg['q_split'], bl, j, zp) for bl in range(TB)])
                if i == 0:
                    nt = _nn(_up(lmat[j]), pq)
                    for h in range(2):
                        den = nt[2 * DH + 8 * h:2 * DH + 8 * h + 8, :] + 1e-6
                        num = nt[h * DH:(h + 1) * DH, :].reshape(4, 8, T)
                        parts.append((num * _recip(den)[None]).reshape(DH, T))
                else:
                    lw = lmat[j, 0:DH, :]
                    parts.append(_nn(lhs([lw]) if j % 2 == 0 else _up(lw), pq))
            if i > 0:
                ffn_step(*(cfg["b_mid"] if mid else cfg["b_lag"])[gi])
            o3[g] = _pk(jnp.concatenate(parts, axis=0).T.astype(BF16))

    def stage_c(i, routed=None, mid=None):
        r0 = i * T
        o = [o3[k, pl.ds(zrt if cfg["o_opq"] and routed is None else 0, T // 2), :] for k in range(KB)]
        copies = []
        for n in range(0, KB, 2):
            if mid is not None and n == cfg["mid_at"]:
                mid()
            parts = []
            for m in (n, n + 1):
                halves = []
                for h in range(TB):
                    ow = [w[h * 64:(h + 1) * 64] for w in o]
                    halves.append(_nn(lhs(ow), wo_buf[:, m * LANE:(m + 1) * LANE]))
                    before_b = h == TB - 1 and (m == KB - 1 or (mid is not None and m + 1 == cfg["mid_at"]))
                    for _ in range(cfg["extra"].get((i, m, h), 1)):
                        ffn_step(cfg["c_last"] if before_b else 2)
                parts.append(jnp.concatenate(halves, axis=0))
            s = _cat(parts)
            cols = slice(n * LANE, (n + 2) * LANE)
            b = xn_rows(r0, T, n, n + 2).astype(F32)
            if routed is None:
                s_buf[r0:r0 + T, cols] = s
            else:
                idx, bsel = routed()
                sel = (lax.broadcasted_iota(jnp.int32, (T, 2 * LANE), 0) + r0) == idx
                b = jnp.where(sel, bsel[:, cols], b)
            res = x_buf[r0:r0 + T, cols].astype(F32) + s * (b * _sigmoid(b))
            out_buf[r0:r0 + T, cols] = res.astype(BF16)
            if routed is not None:
                win = (pl.ds(r0, T), pl.ds(n * LANE, 2 * LANE))
                copies.append(pltpu.make_async_copy(out_buf.at[win], out_hbm.at[win], sem_o.at[2]))
                copies[-1].start()
        if routed is None:
            copies.append(pltpu.make_async_copy(out_buf.at[pl.ds(r0, T)], out_hbm.at[pl.ds(r0, T)], sem_o.at[0]))
            copies[-1].start()
        return copies

    lc = cfg["ln_chunk"]
    arrive(0)
    layernorm(0, T if cfg['plan'] == 'F' else LANE, LANE)
    wrf = wr_buf[...].reshape(1, D).astype(F32)
    for k in range(KB):
        wk3[k, D // 2:(D + RB) // 2, :] = _pk(
            jnp.broadcast_to(wrf[:, k * LANE:(k + 1) * LANE], (RB, LANE)).astype(BF16))
    sign = lax.shift_right_logical(pltpu.bitcast(wrf[:, 0:LANE], jnp.int32), 31)
    zrt = pl.multiple_of(lax.shift_right_logical(jnp.max(sign), 1), cfg["zalign"])
    zz[0] = zrt if 'z' in cfg['opq'] else 0
    zz[1] = zrt
    zvec.append(jnp.full((8, LANE), zrt, jnp.int32).astype(U32))
    zp, zk, zv, zw = [zrt if t in cfg["opq"] else 0 for t in "pkvw"]
    blockdiag(0, 2)
    def phase1():
        if cfg['plan'] == 'F':
            arrive(1)
            fold(1, wk3, 0, 2)
            stage_k(0, 0, 2)
            arrive(2)
            blockdiag(2, KB)
            fold(1, wk3, 2, 4)
            stage_k(0, 2, 4)
            arrive(3)
            layernorm(T, T, cfg["ln1"])
            fold(1, wk3, 4, 6)
            stage_k(0, 4, 6)
            stage_k(1, 0, 6)
            arrive(4)
            fold(1, wk3, 6, 8)
            stage_k(0, 6, 8)
            stage_k(1, 6, 8)
            layernorm(2 * T, T, cfg["ln2"])
        else:
            arrive(1)
            fold(1, wk3, 0, 2)
            keys(0, 0, 2)
            arrive(2)
            for b in range(1, 2 * TB):
                layernorm(b * LANE, LANE, LANE)
                keys(b, 0, 2)
            arrive(3)
            blockdiag(2, KB)
            fold(1, wk3, 2, 4)
            for b in range(2 * TB):
                keys(b, 2, 4)
            arrive(4)
            fold(1, wk3, 4, 8)
            for b in range(2 * TB):
                keys(b, 4, 8)
            layernorm(2 * T, T, lc)
        arrive(5)
        for g in range(KB):
            wt = wraw[2, :, g * LANE:(g + 1) * LANE].T
            if wv3.dtype == BF16:
                for k in range(KB):
                    wv3[k, g * LANE:(g + 1) * LANE, :] = wt[:, k * LANE:(k + 1) * LANE]
            else:
                put_rows(wv3, g * LANE, wt)
        for op in cfg["p1"].split():
            if op == "|":
                arrive(6)
            elif op == "F":
                fold(0, wq3, 0, KB)
            elif int(op[1]) >= NTILE:
                pass
            elif op[0] == "K":
                stage_k(int(op[1]))
            elif op[0] == "V":
                stage_v(int(op[1]))
            else:
                layernorm(int(op[1]) * T, T, lc)
        stage_q(0)
        stage_kv(zv, zk)


    if cfg.get("only") == 2:
        for k in range(1, 7):
            arrive(k)
    else:
        phase1()

    arrive(7)
    r = _rb(r_buf[0:1, :])
    rmax = jnp.max(r)
    pos = lax.broadcasted_iota(jnp.int32, (1, S), 1)
    idx = jnp.clip(jnp.min(jnp.where(r == rmax, pos, S)), 0, S - 1)
    blk = pl.multiple_of((idx // RB) * RB, RB)
    xblk = xn_rows(blk, RB).astype(F32)
    rowsel = (lax.broadcasted_iota(jnp.int32, (RB, D), 0) + blk) == idx
    xs = jnp.broadcast_to(jnp.sum(jnp.where(rowsel, xblk, 0.0), axis=0, keepdims=True), (8, D))
    part, act, y = {}, {}, {}

    def gate_up(w_buf, j, h):
        def f():
            v = _nn(xs[:, h * KH:(h + 1) * KH], w_buf[h * KH:(h + 1) * KH, j * LANE:(j + 1) * LANE])
            key = (w_buf is wu_buf, j)
            part[key] = v if h == 0 else _rb(part[key] + v)
            if h == 1 and w_buf is wu_buf:
                hg = part.pop((False, j))
                act[j] = _rb(_rb(hg * _sigmoid(hg)) * part.pop(key))
            return v
        return f

    def down(m, n):
        def f():
            a = _cat([act[j] for j in range(4 * m, 4 * m + 4)])
            v = _nn(a, wd_buf[m * KH:(m + 1) * KH, n * LANE:(n + 1) * LANE])
            y[n] = v if m == 0 else y[n] + v
            return v
        return f

    def routed():
        if "row" not in part:
            rs = _rb(_sigmoid(jnp.full((1, 1), rmax, F32)))
            yf = _rb(_rb(_cat([y[n] for n in range(KB)])) * rs)
            part["row"] = _rb(xs + yf)[0:1, :]
        return idx, part["row"]

    stage_z()
    ng = cfg.get("short_ffn") or NG
    sets = []
    for m in range(ng + 1):
        gu = [gate_up(w, j, h) for j in range(4 * m, 4 * m + 4) for w in (wg_buf, wu_buf) for h in range(2)
              ] if m < ng else []
        dn = [down(m - 1, n) for n in range(KB)] if m > 0 else []
        while gu or dn:
            sets += gu[:2] + dn[:1]
            gu, dn = gu[2:], dn[1:]

    if cfg.get("only") == 1:
        c = pltpu.make_async_copy(out_buf, out_hbm, sem_o.at[0])
        out_buf[0:16, 0:LANE] = (_up(lmat[pl.ds(zrt, 1)][0]) [0:16] + sum(get_phi(phiq, cfg['q_split'], bb, jj, zrt)[0:16] for bb in range(TB) for jj in range(NPAIR))
                                 + zrow[pl.ds(zrt, 1)][0].astype(BF16)[0:1] + xs[0:1, 0:LANE].astype(BF16))
        c.start()
        c.wait()
        return
    outs = []
    for i in range(NTILE - 1):
        stage_b(i, zp)
        if i == 0:
            ffn_q.extend(sets)
        if i == 0 and cfg["z_pin"]:
            pending.append([1, cfg["z_pin"], zbuf[0, pl.ds(zrt, 8), :]])
        if cfg["o_pin"]:
            pending.append([cfg["o_pin"][0], cfg["o_pin"][1], o3[0, pl.ds(zrt, 8), :]])
        stage_q(i + 1)
        ffn_step(cfg["qc_lag"])
        outs += stage_c(i, mid=(lambda: stage_b(NTILE - 1, zp, True)) if i == NTILE - 2 else None)
    assert not ffn_q, len(ffn_q)
    last = stage_c(NTILE - 1, routed)

    for c in outs:
        c.wait()

    @pl.when(idx < S - T)
    def _():
        b = jnp.where(rowsel, part["row"], xblk)
        res = x_buf[pl.ds(blk, RB), :].astype(F32) + s_buf[pl.ds(blk, RB), :] * (b * _sigmoid(b))
        fix_buf[...] = res.astype(BF16)
        c = pltpu.make_async_copy(fix_buf, out_hbm.at[pl.ds(blk, RB)], sem_o.at[1])
        c.start()
        c.wait()

    for c in last:
        c.wait()


def _build(cfg):
    S = cfg["S"]
    NB = S // LANE
    any_spec = pl.BlockSpec(memory_space=pl.ANY)
    def phi_bufs(split, nb, u32=False):
        pj, pb = split
        if u32:
            return [pltpu.VMEM((pb, pj * 64, LANE), U32)] * ((NPAIR // pj) * (nb // pb))
        return [pltpu.VMEM((pb, pj * LANE, LANE), BF16)] * ((NPAIR // pj) * (nb // pb))

    scratch = [
        pltpu.VMEM((S, D), BF16),
        pltpu.VMEM((KB, S // 2, LANE), U32) if cfg['xn_u32'] else pltpu.VMEM((KB, S, LANE), BF16),
        pltpu.VMEM((S, D), BF16),
        pltpu.VMEM((3, D, D), BF16),
        pltpu.VMEM((H, DH, DH), BF16),
        pltpu.VMEM((D,), BF16),
        pltpu.VMEM((D, WDP), BF16),
        pltpu.VMEM((D, F), BF16),
        pltpu.VMEM((D, F), BF16),
        pltpu.VMEM((F, WDP), BF16),
        pltpu.VMEM((KB, D // 2, LANE), U32),
        pltpu.VMEM((KB, (D + RB) // 2, LANE), U32),
        pltpu.VMEM((KB, D, LANE), BF16) if cfg['wv_bf16'] else pltpu.VMEM((KB, D // 2, LANE), U32),
        phi_bufs(cfg['k_split'], NB),
        pltpu.VMEM((NB, NPAIR * VR, LANE), F32),
        pltpu.VMEM((NPAIR, 8, LANE), F32),
        pltpu.VMEM((NPAIR, 2 * LANE, LANE), F32),
        phi_bufs(cfg['q_split'], TB, cfg['q_u32']),
        pltpu.VMEM((NPAIR, PR // 2, LANE), U32),
        pltpu.VMEM((KB, T // 2, LANE), U32),
        pltpu.VMEM((8, S), F32),
        pltpu.VMEM((S - T, D), F32),
        pltpu.VMEM((RB, D), BF16),
        pltpu.VMEM((D + RB, LANE), F32),
        pltpu.VMEM((D + RB, LANE), F32),
        pltpu.VMEM((D + RB, LANE), F32),
        pltpu.VMEM((D + RB, LANE), F32),
        pltpu.SemaphoreType.DMA((8,)),
        pltpu.SemaphoreType.DMA((3,)),
    ]
    return pl.pallas_call(
        functools.partial(_kernel, cfg),
        out_shape=jax.ShapeDtypeStruct((S, D), BF16),
        in_specs=[any_spec] * 8,
        out_specs=any_spec,
        scratch_shapes=scratch,
        compiler_params=pltpu.CompilerParams(vmem_limit_bytes=100 * 1024 * 1024),
        name=cfg.get("name", "hedgehog_mod"),
    )


@jax.jit
def pallas_recurrent_scan__linear_kernel_hedgehog__moe_arch_mod__prompt_kernel(
    A_x: jax.Array,
    A_wqkv: jax.Array,
    A_w_phi: jax.Array,
    A_wo: jax.Array,
    B_x: jax.Array,
    B_w_r: jax.Array,
    B_w_gate: jax.Array,
    B_w_up: jax.Array,
    B_w_down: jax.Array,
):
    del B_x
    S = CFG["S"]
    out = _build(CFG)(A_x.reshape(S, D), A_wqkv, A_w_phi, A_wo, B_w_r, B_w_gate, B_w_up, B_w_down)
    return out.reshape(1, S, D)
```

```python
import functools

import jax
import jax.numpy as jnp
from jax import lax
import jax.experimental.pallas as pl
import jax.experimental.pallas.tpu as pltpu

S, D, H, DH, F = 2048, 1024, 32, 32, 3584
LANE = 128
KB = D // LANE
KH = D // 2
T = 256
TB = T // LANE
NB = S // LANE
NTILE = S // T
NPAIR = H // 2
VR = 2 * DH + 8
PR = 2 * DH + 16
RB = 16
WP = D + LANE
NG = F // KH
LOG2E = 1.4426950408889634
F32 = jnp.float32
BF16 = jnp.bfloat16
U32 = jnp.uint32

CFG = dict(ln0=128, ln1=128, ln2=16, ln=16, early_fix=True,
           p1="K2 V0 L3 K3 V1 V2 | F L4 V3 K4 L5 V4 K5 L6 V5 K6 L7 V6 K7 V7")


def _nt(a, b):
    return lax.dot_general(a, b, (((1,), (1,)), ((), ())), preferred_element_type=F32)


def _nn(a, b):
    return jnp.dot(a, b, preferred_element_type=F32)


def _rb(v):
    return v.astype(BF16).astype(F32)


def _recip(v):
    return pl.reciprocal(v, approx=True)


def _recip_nr(v):
    r = pl.reciprocal(v, approx=True)
    return r * (2.0 - v * r)


def _silu(v):
    return v * (0.5 * jnp.tanh(0.5 * v) + 0.5)


def _cat(parts):
    return jnp.concatenate(parts, axis=1)


def _pk(v):
    return pltpu.bitcast(v, U32)


def _up(v):
    return pltpu.bitcast(v, BF16)


def _pair_allreduce(v, op):
    v = op(v, pltpu.roll(v, 2, 0))
    return op(v, pltpu.roll(v, 4, 0))


def _dual_softmax(p, z=None):
    n = p.shape[-1]
    p = p.reshape(8, 8, n)
    mx = _pair_allreduce(jnp.max(p, axis=0), jnp.maximum)
    mn = _pair_allreduce(jnp.min(p, axis=0), jnp.minimum)
    ep = jnp.exp2(p - mx[None])
    en = jnp.exp2(mn[None] - p)
    sp = _pair_allreduce(jnp.sum(ep, axis=0), jnp.add)
    sn = _pair_allreduce(jnp.sum(en, axis=0), jnp.add)
    if z is None:
        rp, rn = _recip(sp), _recip(sn)
    else:
        dp = _pair_allreduce(jnp.sum(ep * z[:64].reshape(8, 8, n), axis=0), jnp.add)
        dn = _pair_allreduce(jnp.sum(en * z[64:].reshape(8, 8, n), axis=0), jnp.add)
        rd = _recip(dp * sn + (dn + 1e-6 * sn) * sp)
        rp, rn = sn * rd, sp * rd
    return jnp.concatenate([ep * rp[None], en * rn[None]], axis=0).reshape(LANE, n).astype(BF16)


def _kernel(cfg, x_hbm, wqkv_hbm, phi_hbm, wo_hbm, wr_hbm, wg_hbm, wu_hbm, wd_hbm, out_hbm,
            x_buf, xn3, out_buf, wraw, phi_buf, wr_buf, wo_buf, wg_buf, wu_buf, wd_buf,
            wq3, wk3, wv3, phik3, vaug3, zrow, zbuf, phiq3, lmat, o3, r_buf, s_buf, fix_buf,
            sem, sem_o):
    def cp(src, dst, slot):
        return pltpu.make_async_copy(src, dst, sem.at[slot])

    def x_rows(r0, n, slot):
        return cp(x_hbm.at[pl.ds(r0, n)], x_buf.at[pl.ds(r0, n)], slot)

    def w_cols(j, g0, g1, slot):
        n = (g1 - g0) * LANE
        return cp(wqkv_hbm.at[:, pl.ds(j * D + g0 * LANE, n)], wraw.at[j, :, pl.ds(g0 * LANE, n)], slot)

    def phi_heads(h0, h1, slot):
        return cp(phi_hbm.at[pl.ds(h0, h1 - h0)], phi_buf.at[pl.ds(h0, h1 - h0)], slot)

    groups = [
        [x_rows(0, T, 0), cp(wr_hbm, wr_buf, 0), phi_heads(0, 8, 0)],
        [w_cols(1, 0, 2, 1)],
        [x_rows(T, T, 2), phi_heads(8, H, 2)],
        [w_cols(1, 2, 4, 3)],
        [w_cols(1, 4, KB, 4), x_rows(2 * T, T, 4)],
        [w_cols(2, 0, KB, 5), x_rows(3 * T, T, 5)],
        [x_rows(4 * T, S - 4 * T, 6), w_cols(0, 0, KB, 6), cp(wo_hbm, wo_buf.at[:, pl.ds(0, D)], 6)],
        [cp(wg_hbm, wg_buf, 7), cp(wu_hbm, wu_buf, 7), cp(wd_hbm, wd_buf.at[:, pl.ds(0, D)], 7)],
    ]
    for grp in groups:
        for c in grp:
            c.start()

    def arrive(k):
        for c in groups[k]:
            c.wait()

    def put_blocks(dst, r0, val):
        n = val.shape[0]
        for k in range(KB):
            blk = val[:, k * LANE:(k + 1) * LANE]
            if dst.dtype == U32:
                dst[k, r0 // 2:(r0 + n) // 2, :] = _pk(blk)
            else:
                dst[k, r0:r0 + n, :] = blk

    def xn_rows(r0, n, k0=0, k1=KB):
        return _cat([xn3[k, pl.ds(r0, n), :] for k in range(k0, k1)])

    def layernorm(row0, n, ch, chain=True):
        z = None
        eps = _rb(jnp.full((1, 1), 1e-5, F32))
        for r0 in range(row0, row0 + n, ch):
            xf = x_buf[r0:r0 + ch, :].astype(F32)
            mean = jnp.sum(xf, axis=-1, keepdims=True) * (1.0 / D)
            if z is not None and chain:
                mean = mean + z
            c = xf - mean
            var = jnp.sum(c * c, axis=-1, keepdims=True) * (1.0 / D)
            rs = _recip_nr(_rb(jnp.sqrt(_rb(_rb(var) + eps))))
            z = jnp.where(rs < 0.0, 1.0, 0.0)
            put_blocks(xn3, r0, ((xf - _rb(mean)) * rs).astype(BF16))

    er = lax.broadcasted_iota(jnp.int32, (LANE, DH), 0)
    ec = lax.broadcasted_iota(jnp.int32, (LANE, DH), 1)
    eye4 = jnp.where((er % (2 * DH)) // 2 == ec, 1.0, 0.0).astype(BF16)
    br = lax.broadcasted_iota(jnp.int32, (LANE, LANE), 0)
    bc = lax.broadcasted_iota(jnp.int32, (LANE, LANE), 1)
    bmask = (2 * (br // (2 * DH)) + br % 2) == bc // DH
    bd = {}

    def blockdiag(g0, g1):
        for g in range(g0, g1):
            t = _nt(eye4, phi_buf[4 * g:4 * g + 4].reshape(LANE, DH))
            bd[g] = jnp.where(bmask, t, 0.0).astype(BF16)

    def fold(j, dst, g0, g1):
        for g in range(g0, g1):
            res = _nt(bd[g], wraw[j, :, g * LANE:(g + 1) * LANE]) * LOG2E
            put_blocks(dst, g * LANE, res if dst.dtype == F32 else res.astype(BF16))

    def keys(b, g0=0, g1=KB):
        r0, r1 = g0 * LANE, g1 * LANE
        if wk3.dtype == F32:
            re = r1 + 8 if g1 == KB else r1
            pt = _nt(_cat([wk3[k, r0:re, :] for k in range(KB)]), xn_rows(b * LANE, LANE))
        else:
            re = r1 + RB if g1 == KB else r1
            pt = _nt(_cat([_up(wk3[k, r0 // 2:re // 2, :]) for k in range(KB)]), xn_rows(b * LANE, LANE))
        if re > r1:
            r_buf[:, b * LANE:(b + 1) * LANE] = pt[r1 - r0:r1 - r0 + 8, :]
        for j in range(r0 // 64, r1 // 64):
            phik3[b, j * LANE:(j + 1) * LANE, :] = _dual_softmax(pt[j * 64 - r0:(j + 1) * 64 - r0, :])

    def values(b):
        vt = _nt(_cat([wv3[k] for k in range(KB)]), xn_rows(b * LANE, LANE))
        for j in range(NPAIR):
            vaug3[b, j * VR:j * VR + 2 * DH, :] = vt[j * 2 * DH:(j + 1) * 2 * DH]
            vaug3[b, j * VR + 2 * DH:(j + 1) * VR, :] = jnp.ones((8, LANE), F32)

    ffn_q = []
    pending = []
    zero = []

    def ffn_step(lag, off=0):
        if ffn_q and lag:
            pending.append([lag, off, ffn_q.pop(0)()])

    def lhs(words):
        for p in pending:
            p[0] -= 1
        for p in [p for p in pending if p[0] == 0]:
            pending.remove(p)
            w, off = words[0], p[1]
            tied = w[off:off + 8] ^ (pltpu.bitcast(p[2], U32) & zero[0])
            words = [jnp.concatenate(([w[:off]] if off else []) + [tied, w[off + 8:]], axis=0)] + words[1:]
        return _cat([_up(w) for w in words])

    def stage_q(i):
        for bl in range(TB):
            pt = _nt(lhs([wq3[k] for k in range(KB)]), xn_rows((i * TB + bl) * LANE, LANE))
            for j in range(NPAIR):
                phiq3[bl, j * LANE:(j + 1) * LANE, :] = _dual_softmax(
                    pt[j * 64:(j + 1) * 64, :], None if i == 0 else zbuf[j])

    def stage_kv():
        lr = lax.broadcasted_iota(jnp.int32, (PR, LANE), 0)
        lc = lax.broadcasted_iota(jnp.int32, (PR, LANE), 1)
        keep = jnp.where(lr < 2 * DH, lr // DH, (lr - 2 * DH) // 8) == lc % 2
        for j in range(NPAIR):
            va = _cat([vaug3[b, j * VR:(j + 1) * VR, :] for b in range(NB)])
            pk = _cat([phik3[b, j * LANE:(j + 1) * LANE, :] for b in range(NB)])
            kvt = _nt(va, pk)
            z = kvt[2 * DH:, :]
            lmat[j] = _pk(jnp.where(keep, jnp.concatenate([kvt, z], axis=0), 0.0).astype(BF16))
            zrow[j] = z

    def stage_b(i, slots):
        for g in range(KB):
            parts = []
            for j in (2 * g, 2 * g + 1):
                pq = _cat([phiq3[bl, j * LANE:(j + 1) * LANE, :] for bl in range(TB)])
                if i == 0:
                    nt = _nn(_up(lmat[j]), pq)
                    for h in range(2):
                        den = nt[2 * DH + 8 * h:2 * DH + 8 * h + 8, :] + 1e-6
                        num = nt[h * DH:(h + 1) * DH, :].reshape(4, 8, T)
                        parts.append((num * _recip(den)[None]).reshape(DH, T))
                else:
                    lw = lmat[j, 0:DH, :]
                    parts.append(_nn(lhs([lw]) if j % 2 == 0 else _up(lw), pq))
            ffn_step(*slots[g])
            o3[g] = _pk(jnp.concatenate(parts, axis=0).T.astype(BF16))

    def stage_c(i, routed=None, mid=None):
        r0 = i * T
        o = [o3[k] for k in range(KB)]
        copies = []
        for n in range(0, KB, 2):
            if mid is not None and n == KB - 2:
                mid()
            parts = []
            for m in (n, n + 1):
                halves = []
                for h in range(TB):
                    halves.append(_nn(lhs([w[h * 64:(h + 1) * 64] for w in o]),
                                      wo_buf[:, m * LANE:(m + 1) * LANE]))
                    before_b = h == TB - 1 and (m == KB - 1 or (mid is not None and m == KB - 3))
                    ffn_step(4 if before_b else 2)
                parts.append(jnp.concatenate(halves, axis=0))
            s = _cat(parts)
            cols = slice(n * LANE, (n + 2) * LANE)
            b = xn_rows(r0, T, n, n + 2).astype(F32)
            if routed is None:
                s_buf[r0:r0 + T, cols] = s
            else:
                idx, brow = routed()
                sel = (lax.broadcasted_iota(jnp.int32, (T, 2 * LANE), 0) + r0) == idx
                b = jnp.where(sel, brow[:, cols], b)
            res = x_buf[r0:r0 + T, cols].astype(F32) + s * _silu(b)
            out_buf[r0:r0 + T, cols] = res.astype(BF16)
            if routed is not None:
                win = (pl.ds(r0, T), pl.ds(n * LANE, 2 * LANE))
                copies.append(pltpu.make_async_copy(out_buf.at[win], out_hbm.at[win], sem_o.at[2]))
                copies[-1].start()
        if routed is None:
            copies.append(pltpu.make_async_copy(out_buf.at[pl.ds(r0, T)], out_hbm.at[pl.ds(r0, T)], sem_o.at[0]))
            copies[-1].start()
        return copies

    arrive(0)
    layernorm(0, T, cfg["ln0"], False)
    wrf = wr_buf[...].reshape(1, D).astype(F32)
    for k in range(KB):
        if wk3.dtype == F32:
            wk3[k, D:D + 8, :] = jnp.broadcast_to(wrf[:, k * LANE:(k + 1) * LANE], (8, LANE))
        else:
            wk3[k, D // 2:(D + RB) // 2, :] = _pk(
                jnp.broadcast_to(wrf[:, k * LANE:(k + 1) * LANE], (RB, LANE)).astype(BF16))
    sign = lax.shift_right_logical(pltpu.bitcast(wrf[:, 0:LANE], jnp.int32), 31)
    zrt = pl.multiple_of(lax.shift_right_logical(jnp.max(sign), 1), 8)
    zero.append(jnp.full((8, LANE), zrt, jnp.int32).astype(U32))
    blockdiag(0, 2)

    def phase1():
        arrive(1)
        fold(1, wk3, 0, 2)
        for b in range(TB):
            keys(b, 0, 2)
        arrive(2)
        blockdiag(2, KB)
        for b in range(TB, 2 * TB):
            layernorm(b * LANE, LANE, cfg["ln1"], False)
            keys(b, 0, 2)
        arrive(3)
        fold(1, wk3, 2, 4)
        for b in range(2 * TB):
            keys(b, 2, 4)
        arrive(4)
        fold(1, wk3, 4, KB)
        for b in range(2 * TB):
            keys(b, 4, KB)
        layernorm(2 * T, T, cfg["ln2"])
        arrive(5)
        for g in range(KB):
            put_blocks(wv3, g * LANE, wraw[2, :, g * LANE:(g + 1) * LANE].T)
        for op in cfg["p1"].split():
            if op == "|":
                arrive(6)
            elif op == "F":
                fold(0, wq3, 0, KB)
            elif op[0] == "L":
                layernorm(int(op[1]) * T, T, cfg["ln"])
            else:
                for b in range(int(op[1]) * TB, (int(op[1]) + 1) * TB):
                    keys(b) if op[0] == "K" else values(b)
        stage_q(0)
        stage_kv()

    if cfg.get("only") == 2:
        for k in range(1, 7):
            arrive(k)
    else:
        phase1()

    arrive(7)
    r = _rb(r_buf[0:1, :])
    rmax = jnp.max(r)
    pos = lax.broadcasted_iota(jnp.int32, (1, S), 1)
    idx = jnp.clip(jnp.min(jnp.where(r == rmax, pos, S)), 0, S - 1)
    blk = pl.multiple_of((idx // RB) * RB, RB)
    xblk = xn_rows(blk, RB).astype(F32)
    rowsel = (lax.broadcasted_iota(jnp.int32, (RB, D), 0) + blk) == idx
    xs = jnp.broadcast_to(jnp.sum(jnp.where(rowsel, xblk, 0.0), axis=0, keepdims=True), (8, D))
    part, act, y = {}, {}, {}

    def gate_up(w_buf, j, h):
        def f():
            v = _nn(xs[:, h * KH:(h + 1) * KH], w_buf[h * KH:(h + 1) * KH, j * LANE:(j + 1) * LANE])
            key = (w_buf is wu_buf, j)
            part[key] = v if h == 0 else _rb(part[key] + v)
            if h == 1 and w_buf is wu_buf:
                act[j] = _rb(_rb(_silu(part.pop((False, j)))) * part.pop(key))
            return v
        return f

    def down(m, n):
        def f():
            a = _cat([act[j] for j in range(4 * m, 4 * m + 4)])
            v = _nn(a, wd_buf[m * KH:(m + 1) * KH, n * LANE:(n + 1) * LANE])
            y[n] = v if m == 0 else y[n] + v
            return v
        return f

    def routed():
        if "row" not in part:
            rs = _rb(0.5 * jnp.tanh(0.5 * jnp.full((1, 1), rmax, F32)) + 0.5)
            yf = _rb(_rb(_cat([y[n] for n in range(KB)])) * rs)
            part["row"] = _rb(xs + yf)[0:1, :]
        return idx, part["row"]

    sets = []
    for m in range(NG + 1):
        gu = [gate_up(w, j, h) for j in range(4 * m, 4 * m + 4) for w in (wg_buf, wu_buf) for h in range(2)
              ] if m < NG else []
        dn = [down(m - 1, n) for n in range(KB)] if m > 0 else []
        while gu or dn:
            sets += gu[:2] + dn[:1]
            gu, dn = gu[2:], dn[1:]

    for j in range(NPAIR):
        zbuf[j] = jnp.concatenate([zrow[j]] * (LANE // 8), axis=0).T

    if cfg.get("only") == 1:
        c = pltpu.make_async_copy(out_buf, out_hbm, sem_o.at[0])
        out_buf[0:16, 0:LANE] = (_up(lmat[pl.ds(zrt, 1)][0])[0:16] + phiq3[0, pl.ds(zrt, 16), :]
                                 + zrow[pl.ds(zrt, 1)][0].astype(BF16)[0:1] + xs[0:1, 0:LANE].astype(BF16))
        c.start()
        c.wait()
        return

    b_slots = ((4, 0),) * 5 + ((3, 16), (2, 48))
    outs = []
    for i in range(NTILE - 1):
        stage_b(i, b_slots + ((0, 0),))
        if i == 0:
            ffn_q.extend(sets)
        pending.append([1, 480, o3[0, pl.ds(zrt, 8), :]])
        stage_q(i + 1)
        ffn_step(2)
        outs += stage_c(i, mid=(lambda: stage_b(NTILE - 1, b_slots + ((2, 0),))) if i == NTILE - 2 else None)
    assert not ffn_q, len(ffn_q)

    def fix_rows():
        sb = pl.multiple_of(jnp.minimum(blk, S - T - RB), RB)
        b = jnp.where(rowsel, routed()[1], xblk)
        res = x_buf[pl.ds(blk, RB), :].astype(F32) + s_buf[pl.ds(sb, RB), :] * _silu(b)
        fix_buf[...] = res.astype(BF16)

    if cfg["early_fix"]:
        fix_rows()
    last = stage_c(NTILE - 1, routed)
    for c in outs:
        c.wait()

    @pl.when(idx < S - T)
    def _():
        if not cfg["early_fix"]:
            fix_rows()
        c = pltpu.make_async_copy(fix_buf, out_hbm.at[pl.ds(blk, RB)], sem_o.at[1])
        c.start()
        c.wait()

    for c in last:
        c.wait()


def _build(cfg):
    any_spec = pl.BlockSpec(memory_space=pl.ANY)
    scratch = [
        pltpu.VMEM((S, D), BF16),
        pltpu.VMEM((KB, S, LANE), BF16),
        pltpu.VMEM((S, D), BF16),
        pltpu.VMEM((3, D, D), BF16),
        pltpu.VMEM((H, DH, DH), BF16),
        pltpu.VMEM((D,), BF16),
        pltpu.VMEM((D, WP), BF16),
        pltpu.VMEM((D, F), BF16),
        pltpu.VMEM((D, F), BF16),
        pltpu.VMEM((F, WP), BF16),
        pltpu.VMEM((KB, D // 2, LANE), U32),
        pltpu.VMEM((KB, D + 8, LANE), F32) if cfg.get('wk_f32') else pltpu.VMEM((KB, (D + RB) // 2, LANE), U32),
        pltpu.VMEM((KB, D, LANE), BF16),
        pltpu.VMEM((NB, 2 * D, LANE), BF16),
        pltpu.VMEM((NB, NPAIR * VR, LANE), F32),
        pltpu.VMEM((NPAIR, 8, LANE), F32),
        pltpu.VMEM((NPAIR, LANE, LANE), F32),
        pltpu.VMEM((TB, 2 * D, LANE), BF16),
        pltpu.VMEM((NPAIR, PR // 2, LANE), U32),
        pltpu.VMEM((KB, T // 2, LANE), U32),
        pltpu.VMEM((8, S), F32),
        pltpu.VMEM((S - T, D), F32),
        pltpu.VMEM((RB, D), BF16),
        pltpu.SemaphoreType.DMA((8,)),
        pltpu.SemaphoreType.DMA((3,)),
    ]
    return pl.pallas_call(
        functools.partial(_kernel, cfg),
        out_shape=jax.ShapeDtypeStruct((S, D), BF16),
        in_specs=[any_spec] * 8,
        out_specs=any_spec,
        scratch_shapes=scratch,
        compiler_params=pltpu.CompilerParams(vmem_limit_bytes=100 * 1024 * 1024),
        name=cfg.get("name", "hedgehog_mod"),
    )


@jax.jit
def pallas_recurrent_scan__linear_kernel_hedgehog__moe_arch_mod__prompt_kernel(
    A_x: jax.Array,
    A_wqkv: jax.Array,
    A_w_phi: jax.Array,
    A_wo: jax.Array,
    B_x: jax.Array,
    B_w_r: jax.Array,
    B_w_gate: jax.Array,
    B_w_up: jax.Array,
    B_w_down: jax.Array,
):
    del B_x
    out = _build(CFG)(A_x.reshape(S, D), A_wqkv, A_w_phi, A_wo, B_w_r, B_w_gate, B_w_up, B_w_down)
    return out.reshape(1, S, D)
```

```python
import functools

import jax
import jax.numpy as jnp
from jax import lax
import jax.experimental.pallas as pl
import jax.experimental.pallas.tpu as pltpu

S, D, H, DH, F = 2048, 1024, 32, 32, 3584
LANE = 128
KB = D // LANE
KH = D // 2
T = 256
TB = T // LANE
NB = S // LANE
NTILE = S // T
NPAIR = H // 2
VR = 2 * DH + 8
PR = 2 * DH + 16
RB = 16
WP = D + LANE
NG = F // KH
LOG2E = 1.4426950408889634
F32 = jnp.float32
BF16 = jnp.bfloat16
U32 = jnp.uint32

CFG = dict(ln0=128, ln1=64, ln2=16, ln=16, early_fix=True, chain='rs', chain1='rs', chain2=8, chain3=8, plan=(4, 5), phi1=8,
           p1="K2 V0 L3 K3 V1 V2 | F L4 V3 K4 L5 V4 K5 L6 V5 K6 L7 V6 K7 V7")


def _nt(a, b):
    return lax.dot_general(a, b, (((1,), (1,)), ((), ())), preferred_element_type=F32)


def _nn(a, b):
    return jnp.dot(a, b, preferred_element_type=F32)


def _rb(v):
    return v.astype(BF16).astype(F32)


def _recip(v):
    return pl.reciprocal(v, approx=True)


def _recip_nr(v):
    r = pl.reciprocal(v, approx=True)
    return r * (2.0 - v * r)


def _silu(v):
    return v * (0.5 * jnp.tanh(0.5 * v) + 0.5)


def _cat(parts):
    return jnp.concatenate(parts, axis=1)


def _pk(v):
    return pltpu.bitcast(v, U32)


def _up(v):
    return pltpu.bitcast(v, BF16)


def _pair_allreduce(v, op):
    v = op(v, pltpu.roll(v, 2, 0))
    return op(v, pltpu.roll(v, 4, 0))


def _dual_softmax(p, z=None):
    n = p.shape[-1]
    p = p.reshape(8, 8, n)
    mx = _pair_allreduce(jnp.max(p, axis=0), jnp.maximum)
    mn = _pair_allreduce(jnp.min(p, axis=0), jnp.minimum)
    ep = jnp.exp2(p - mx[None])
    en = jnp.exp2(mn[None] - p)
    sp = _pair_allreduce(jnp.sum(ep, axis=0), jnp.add)
    sn = _pair_allreduce(jnp.sum(en, axis=0), jnp.add)
    if z is None:
        rp, rn = _recip(sp), _recip(sn)
    else:
        dp = _pair_allreduce(jnp.sum(ep * z[:64].reshape(8, 8, n), axis=0), jnp.add)
        dn = _pair_allreduce(jnp.sum(en * z[64:].reshape(8, 8, n), axis=0), jnp.add)
        rd = _recip(dp * sn + (dn + 1e-6 * sn) * sp)
        rp, rn = sn * rd, sp * rd
    return jnp.concatenate([ep * rp[None], en * rn[None]], axis=0).reshape(LANE, n).astype(BF16)


def _kernel(cfg, x_hbm, wqkv_hbm, phi_hbm, wo_hbm, wr_hbm, wg_hbm, wu_hbm, wd_hbm, out_hbm,
            x_buf, xn3, out_buf, wraw, phi_buf, wr_buf, wo_buf, wg_buf, wu_buf, wd_buf,
            wq3, wk3, wv3, phik3, vaug3, zrow, zbuf, phiq3, lmat, o3, r_buf, s_buf, fix_buf,
            sem, sem_o):
    def cp(src, dst, slot):
        return pltpu.make_async_copy(src, dst, sem.at[slot])

    def x_rows(r0, n, slot):
        return cp(x_hbm.at[pl.ds(r0, n)], x_buf.at[pl.ds(r0, n)], slot)

    def w_cols(j, g0, g1, slot):
        n = (g1 - g0) * LANE
        return cp(wqkv_hbm.at[:, pl.ds(j * D + g0 * LANE, n)], wraw.at[j, :, pl.ds(g0 * LANE, n)], slot)

    def phi_heads(h0, h1, slot):
        return cp(phi_hbm.at[pl.ds(h0, h1 - h0)], phi_buf.at[pl.ds(h0, h1 - h0)], slot)

    c1, c2 = cfg["plan"]
    h1 = cfg["phi1"]
    groups = [
        [x_rows(0, T, 0), cp(wr_hbm, wr_buf, 0), phi_heads(0, 8, 0)],
        [w_cols(1, 0, 2, 1)] + ([phi_heads(8, h1, 1)] if h1 > 8 else []),
        [phi_heads(h1, H, 2), w_cols(1, 2, c1, 2)],
        [x_rows(T, T, 3), w_cols(1, c1, c2, 3)],
        [w_cols(1, c2, KB, 4), x_rows(2 * T, T, 4)],
        [w_cols(2, 0, KB, 5), x_rows(3 * T, T, 5)],
        [x_rows(4 * T, S - 4 * T, 6), w_cols(0, 0, KB, 6), cp(wo_hbm, wo_buf.at[:, pl.ds(0, D)], 6)],
        [cp(wg_hbm, wg_buf, 7), cp(wu_hbm, wu_buf, 7), cp(wd_hbm, wd_buf.at[:, pl.ds(0, D)], 7)],
    ]
    for grp in groups:
        for c in grp:
            c.start()

    def arrive(k):
        for c in groups[k]:
            c.wait()

    def put_blocks(dst, r0, val):
        n = val.shape[0]
        for k in range(KB):
            blk = val[:, k * LANE:(k + 1) * LANE]
            if dst.dtype != F32:
                blk = blk.astype(BF16)
            if dst.dtype == U32:
                dst[k, r0 // 2:(r0 + n) // 2, :] = _pk(blk)
            else:
                dst[k, r0:r0 + n, :] = blk

    def xn_rows(r0, n, k0=0, k1=KB):
        return _cat([xn3[k, pl.ds(r0, n), :] for k in range(k0, k1)])

    def layernorm(row0, n, ch, chain="rs"):
        z = None
        eps = _rb(jnp.full((1, 1), 1e-5, F32))
        for r0 in range(row0, row0 + n, ch):
            xf = x_buf[r0:r0 + ch, :].astype(F32)
            mean = jnp.broadcast_to(jnp.sum(xf, axis=-1, keepdims=True) * (1.0 / D), (ch, LANE))
            if z is not None and chain:
                mean = mean + z
            c = xf - _cat([mean] * KB)
            var = jnp.sum(c * c, axis=-1, keepdims=True) * (1.0 / D)
            rs = _recip_nr(_rb(jnp.sqrt(_rb(_rb(var) + eps))))
            xn = (xf - _cat([_rb(mean)] * KB)) * rs
            put_blocks(xn3, r0, xn)
            if chain == "rs":
                z = jnp.where(rs < 0.0, 1.0, 0.0)
            elif chain:
                u = pltpu.bitcast(xn, U32)
                acc = u[:, 0:LANE]
                for k in range(1, chain):
                    acc = acc | u[:, k * (KB // chain) * LANE:(k * (KB // chain) + 1) * LANE]
                z = pltpu.bitcast(acc & jnp.concatenate([zero[0]] * (ch // 8), axis=0), F32)

    er = lax.broadcasted_iota(jnp.int32, (LANE, DH), 0)
    ec = lax.broadcasted_iota(jnp.int32, (LANE, DH), 1)
    eye4 = jnp.where((er % (2 * DH)) // 2 == ec, 1.0, 0.0).astype(BF16)
    br = lax.broadcasted_iota(jnp.int32, (LANE, LANE), 0)
    bc = lax.broadcasted_iota(jnp.int32, (LANE, LANE), 1)
    bmask = (2 * (br // (2 * DH)) + br % 2) == bc // DH
    bd = {}

    def blockdiag(g0, g1):
        for g in range(g0, g1):
            t = _nt(eye4, phi_buf[4 * g:4 * g + 4].reshape(LANE, DH))
            bd[g] = jnp.where(bmask, t, 0.0).astype(BF16)

    def fold(j, dst, g0, g1):
        for g in range(g0, g1):
            res = _nt(bd[g], wraw[j, :, g * LANE:(g + 1) * LANE]) * LOG2E
            put_blocks(dst, g * LANE, res if dst.dtype == F32 or True else res.astype(BF16))

    def keys(b, g0=0, g1=KB):
        r0, r1 = g0 * LANE, g1 * LANE
        if wk3.dtype == F32:
            re = r1 + 8 if g1 == KB else r1
            pt = _nt(_cat([wk3[k, r0:re, :] for k in range(KB)]), xn_rows(b * LANE, LANE))
        else:
            re = r1 + RB if g1 == KB else r1
            pt = _nt(_cat([_up(wk3[k, r0 // 2:re // 2, :]) for k in range(KB)]), xn_rows(b * LANE, LANE))
        if re > r1:
            r_buf[:, b * LANE:(b + 1) * LANE] = pt[r1 - r0:r1 - r0 + 8, :]
        for j in range(r0 // 64, r1 // 64):
            phik3[b, j * LANE:(j + 1) * LANE, :] = _dual_softmax(pt[j * 64 - r0:(j + 1) * 64 - r0, :])

    def values(b):
        vt = _nt(_cat([wv3[k] for k in range(KB)]), xn_rows(b * LANE, LANE))
        for j in range(NPAIR):
            vaug3[b, j * VR:j * VR + 2 * DH, :] = vt[j * 2 * DH:(j + 1) * 2 * DH]
            vaug3[b, j * VR + 2 * DH:(j + 1) * VR, :] = jnp.ones((8, LANE), F32)

    ffn_q = []
    pending = []
    zero = []

    def ffn_step(lag, off=0):
        if ffn_q and lag:
            pending.append([lag, off, ffn_q.pop(0)()])

    def lhs(words):
        for p in pending:
            p[0] -= 1
        for p in [p for p in pending if p[0] == 0]:
            pending.remove(p)
            w, off = words[0], p[1]
            tied = w[off:off + 8] ^ (pltpu.bitcast(p[2], U32) & zero[0])
            words = [jnp.concatenate(([w[:off]] if off else []) + [tied, w[off + 8:]], axis=0)] + words[1:]
        return _cat([_up(w) for w in words])

    def stage_q(i):
        for bl in range(TB):
            pt = _nt(lhs([wq3[k] for k in range(KB)]), xn_rows((i * TB + bl) * LANE, LANE))
            for j in range(NPAIR):
                phiq3[bl, j * LANE:(j + 1) * LANE, :] = _dual_softmax(
                    pt[j * 64:(j + 1) * 64, :], None if i == 0 else zbuf[j])

    def stage_kv():
        lr = lax.broadcasted_iota(jnp.int32, (PR, LANE), 0)
        lc = lax.broadcasted_iota(jnp.int32, (PR, LANE), 1)
        keep = jnp.where(lr < 2 * DH, lr // DH, (lr - 2 * DH) // 8) == lc % 2
        for j in range(NPAIR):
            va = _cat([vaug3[b, j * VR:(j + 1) * VR, :] for b in range(NB)])
            pk = _cat([phik3[b, j * LANE:(j + 1) * LANE, :] for b in range(NB)])
            kvt = _nt(va, pk)
            z = kvt[2 * DH:, :]
            lmat[j] = _pk(jnp.where(keep, jnp.concatenate([kvt, z], axis=0), 0.0).astype(BF16))
            zrow[j] = z

    def stage_b(i, slots):
        for g in range(KB):
            parts = []
            for j in (2 * g, 2 * g + 1):
                pq = _cat([phiq3[bl, j * LANE:(j + 1) * LANE, :] for bl in range(TB)])
                if i == 0:
                    nt = _nn(_up(lmat[j]), pq)
                    for h in range(2):
                        den = nt[2 * DH + 8 * h:2 * DH + 8 * h + 8, :] + 1e-6
                        num = nt[h * DH:(h + 1) * DH, :].reshape(4, 8, T)
                        parts.append((num * _recip(den)[None]).reshape(DH, T))
                else:
                    lw = lmat[j, 0:DH, :]
                    parts.append(_nn(lhs([lw]) if j % 2 == 0 else _up(lw), pq))
            ffn_step(*slots[g])
            o3[g] = _pk(jnp.concatenate(parts, axis=0).T.astype(BF16))

    def stage_c(i, routed=None, mid=None):
        r0 = i * T
        o = [o3[k] for k in range(KB)]
        copies = []
        for n in range(0, KB, 2):
            if mid is not None and n == KB - 2:
                mid()
            parts = []
            for m in (n, n + 1):
                halves = []
                for h in range(TB):
                    halves.append(_nn(lhs([w[h * 64:(h + 1) * 64] for w in o]),
                                      wo_buf[:, m * LANE:(m + 1) * LANE]))
                    before_b = h == TB - 1 and (m == KB - 1 or (mid is not None and m == KB - 3))
                    ffn_step(4 if before_b else 2)
                parts.append(jnp.concatenate(halves, axis=0))
            s = _cat(parts)
            cols = slice(n * LANE, (n + 2) * LANE)
            b = xn_rows(r0, T, n, n + 2).astype(F32)
            if routed is None:
                s_buf[r0:r0 + T, cols] = s
            else:
                idx, brow = routed()
                sel = (lax.broadcasted_iota(jnp.int32, (T, 2 * LANE), 0) + r0) == idx
                b = jnp.where(sel, brow[:, cols], b)
            res = x_buf[r0:r0 + T, cols].astype(F32) + s * _silu(b)
            out_buf[r0:r0 + T, cols] = res.astype(BF16)
            if routed is not None:
                win = (pl.ds(r0, T), pl.ds(n * LANE, 2 * LANE))
                copies.append(pltpu.make_async_copy(out_buf.at[win], out_hbm.at[win], sem_o.at[2]))
                copies[-1].start()
        if routed is None:
            copies.append(pltpu.make_async_copy(out_buf.at[pl.ds(r0, T)], out_hbm.at[pl.ds(r0, T)], sem_o.at[0]))
            copies[-1].start()
        return copies

    arrive(0)
    layernorm(0, T, cfg["ln0"], False)
    wrf = wr_buf[...].reshape(1, D).astype(F32)
    for k in range(KB):
        if wk3.dtype == F32:
            wk3[k, D:D + 8, :] = jnp.broadcast_to(wrf[:, k * LANE:(k + 1) * LANE], (8, LANE))
        else:
            wk3[k, D // 2:(D + RB) // 2, :] = _pk(
                jnp.broadcast_to(wrf[:, k * LANE:(k + 1) * LANE], (RB, LANE)).astype(BF16))
    sign = lax.shift_right_logical(pltpu.bitcast(wrf[:, 0:LANE], jnp.int32), 31)
    zrt = pl.multiple_of(lax.shift_right_logical(jnp.max(sign), 1), 8)
    zero.append(jnp.full((8, LANE), zrt, jnp.int32).astype(U32))
    blockdiag(0, 2)

    def phase1():
        arrive(1)
        blockdiag(2, h1 // 4)
        fold(1, wk3, 0, 2)
        for b in range(TB):
            keys(b, 0, 2)
        arrive(2)
        blockdiag(h1 // 4, KB)
        fold(1, wk3, 2, c1)
        for b in range(TB):
            keys(b, 2, c1)
        arrive(3)
        fold(1, wk3, c1, c2)
        for b in range(TB):
            keys(b, c1, c2)
        for b in range(TB, 2 * TB):
            layernorm(b * LANE, LANE, cfg["ln1"], cfg["chain1"])
            keys(b, 0, c2)
        arrive(4)
        fold(1, wk3, c2, KB)
        for b in range(2 * TB):
            keys(b, c2, KB)
        layernorm(2 * T, T, cfg["ln2"], cfg["chain2"])
        arrive(5)
        for g in range(KB):
            put_blocks(wv3, g * LANE, wraw[2, :, g * LANE:(g + 1) * LANE].T)
        for op in cfg["p1"].split():
            if op == "|":
                arrive(6)
            elif op == "F":
                fold(0, wq3, 0, KB)
            elif op[0] == "L":
                layernorm(int(op[1]) * T, T, cfg["ln"], cfg["chain3"] if op == "L3" else cfg["chain"])
            else:
                for b in range(int(op[1]) * TB, (int(op[1]) + 1) * TB):
                    keys(b) if op[0] == "K" else values(b)
        stage_q(0)
        stage_kv()

    if cfg.get("only") == 2:
        for k in range(1, 7):
            arrive(k)
    else:
        phase1()

    arrive(7)
    r = _rb(r_buf[0:1, :])
    rmax = jnp.max(r)
    pos = lax.broadcasted_iota(jnp.int32, (1, S), 1)
    idx = jnp.clip(jnp.min(jnp.where(r == rmax, pos, S)), 0, S - 1)
    blk = pl.multiple_of((idx // RB) * RB, RB)
    xblk = xn_rows(blk, RB).astype(F32)
    rowsel = (lax.broadcasted_iota(jnp.int32, (RB, D), 0) + blk) == idx
    xs = jnp.broadcast_to(jnp.sum(jnp.where(rowsel, xblk, 0.0), axis=0, keepdims=True), (8, D))
    part, act, y = {}, {}, {}

    def gate_up(w_buf, j, h):
        def f():
            v = _nn(xs[:, h * KH:(h + 1) * KH], w_buf[h * KH:(h + 1) * KH, j * LANE:(j + 1) * LANE])
            key = (w_buf is wu_buf, j)
            part[key] = v if h == 0 else _rb(part[key] + v)
            if h == 1 and w_buf is wu_buf:
                act[j] = _rb(_rb(_silu(part.pop((False, j)))) * part.pop(key))
            return v
        return f

    def down(m, n):
        def f():
            a = _cat([act[j] for j in range(4 * m, 4 * m + 4)])
            v = _nn(a, wd_buf[m * KH:(m + 1) * KH, n * LANE:(n + 1) * LANE])
            y[n] = v if m == 0 else y[n] + v
            return v
        return f

    def routed():
        if "row" not in part:
            rs = _rb(0.5 * jnp.tanh(0.5 * jnp.full((1, 1), rmax, F32)) + 0.5)
            yf = _rb(_rb(_cat([y[n] for n in range(KB)])) * rs)
            part["row"] = _rb(xs + yf)[0:1, :]
        return idx, part["row"]

    sets = []
    for m in range(NG + 1):
        gu = [gate_up(w, j, h) for j in range(4 * m, 4 * m + 4) for w in (wg_buf, wu_buf) for h in range(2)
              ] if m < NG else []
        dn = [down(m - 1, n) for n in range(KB)] if m > 0 else []
        while gu or dn:
            sets += gu[:2] + dn[:1]
            gu, dn = gu[2:], dn[1:]

    for j in range(NPAIR):
        zbuf[j] = jnp.concatenate([zrow[j]] * (LANE // 8), axis=0).T

    if cfg.get("only") == 1:
        c = pltpu.make_async_copy(out_buf, out_hbm, sem_o.at[0])
        out_buf[0:16, 0:LANE] = (_up(lmat[pl.ds(zrt, 1)][0])[0:16] + phiq3[0, pl.ds(zrt, 16), :]
                                 + zrow[pl.ds(zrt, 1)][0].astype(BF16)[0:1] + xs[0:1, 0:LANE].astype(BF16))
        c.start()
        c.wait()
        return

    b_slots = ((4, 0),) * 5 + ((3, 16), (2, 48))
    outs = []
    for i in range(NTILE - 1):
        stage_b(i, b_slots + ((0, 0),))
        if i == 0:
            ffn_q.extend(sets)
        pending.append([1, 480, o3[0, pl.ds(zrt, 8), :]])
        stage_q(i + 1)
        ffn_step(2)
        outs += stage_c(i, mid=(lambda: stage_b(NTILE - 1, b_slots + ((2, 0),))) if i == NTILE - 2 else None)
    assert not ffn_q, len(ffn_q)

    def fix_rows():
        sb = pl.multiple_of(jnp.minimum(blk, S - T - RB), RB)
        b = jnp.where(rowsel, routed()[1], xblk)
        res = x_buf[pl.ds(blk, RB), :].astype(F32) + s_buf[pl.ds(sb, RB), :] * _silu(b)
        fix_buf[...] = res.astype(BF16)

    if cfg["early_fix"]:
        fix_rows()
    last = stage_c(NTILE - 1, routed)
    for c in outs:
        c.wait()

    @pl.when(idx < S - T)
    def _():
        if not cfg["early_fix"]:
            fix_rows()
        c = pltpu.make_async_copy(fix_buf, out_hbm.at[pl.ds(blk, RB)], sem_o.at[1])
        c.start()
        c.wait()

    for c in last:
        c.wait()


def _build(cfg):
    any_spec = pl.BlockSpec(memory_space=pl.ANY)
    scratch = [
        pltpu.VMEM((S, D), BF16),
        pltpu.VMEM((KB, S, LANE), BF16),
        pltpu.VMEM((S, D), BF16),
        pltpu.VMEM((3, D, D), BF16),
        pltpu.VMEM((H, DH, DH), BF16),
        pltpu.VMEM((D,), BF16),
        pltpu.VMEM((D, WP), BF16),
        pltpu.VMEM((D, F), BF16),
        pltpu.VMEM((D, F), BF16),
        pltpu.VMEM((F, WP), BF16),
        pltpu.VMEM((KB, D // 2, LANE), U32),
        pltpu.VMEM((KB, D + 8, LANE), F32) if cfg.get('wk_f32') else pltpu.VMEM((KB, (D + RB) // 2, LANE), U32),
        pltpu.VMEM((KB, D, LANE), BF16),
        pltpu.VMEM((NB, 2 * D, LANE), BF16),
        pltpu.VMEM((NB, NPAIR * VR, LANE), F32),
        pltpu.VMEM((NPAIR, 8, LANE), F32),
        pltpu.VMEM((NPAIR, LANE, LANE), F32),
        pltpu.VMEM((TB, 2 * D, LANE), BF16),
        pltpu.VMEM((NPAIR, PR // 2, LANE), U32),
        pltpu.VMEM((KB, T // 2, LANE), U32),
        pltpu.VMEM((8, S), F32),
        pltpu.VMEM((S - T, D), F32),
        pltpu.VMEM((RB, D), BF16),
        pltpu.SemaphoreType.DMA((8,)),
        pltpu.SemaphoreType.DMA((3,)),
    ]
    return pl.pallas_call(
        functools.partial(_kernel, cfg),
        out_shape=jax.ShapeDtypeStruct((S, D), BF16),
        in_specs=[any_spec] * 8,
        out_specs=any_spec,
        scratch_shapes=scratch,
        compiler_params=pltpu.CompilerParams(vmem_limit_bytes=100 * 1024 * 1024),
        name=cfg.get("name", "hedgehog_mod"),
    )


@jax.jit
def pallas_recurrent_scan__linear_kernel_hedgehog__moe_arch_mod__prompt_kernel(
    A_x: jax.Array,
    A_wqkv: jax.Array,
    A_w_phi: jax.Array,
    A_wo: jax.Array,
    B_x: jax.Array,
    B_w_r: jax.Array,
    B_w_gate: jax.Array,
    B_w_up: jax.Array,
    B_w_down: jax.Array,
):
    del B_x
    out = _build(CFG)(A_x.reshape(S, D), A_wqkv, A_w_phi, A_wo, B_w_r, B_w_gate, B_w_up, B_w_down)
    return out.reshape(1, S, D)
```

```python
import functools

import jax
import jax.numpy as jnp
from jax import lax
import jax.experimental.pallas as pl
import jax.experimental.pallas.tpu as pltpu

S, D, H, DH, F = 2048, 1024, 32, 32, 3584
LANE = 128
KB = D // LANE
KH = D // 2
T = 256
TB = T // LANE
NB = S // LANE
NTILE = S // T
NPAIR = H // 2
VR = 2 * DH + 8
PR = 2 * DH + 16
RB = 16
WP = D + LANE
NG = F // KH
LOG2E = 1.4426950408889634
F32 = jnp.float32
BF16 = jnp.bfloat16
U32 = jnp.uint32

PHASE1 = "K2 V0 L3 K3 V1 V2 | F L4 V3 K4 L5 V4 K5 L6 V5 K6 L7 V6 K7 V7"


def _nt(a, b):
    return lax.dot_general(a, b, (((1,), (1,)), ((), ())), preferred_element_type=F32)


def _nn(a, b):
    return jnp.dot(a, b, preferred_element_type=F32)


def _rb(v):
    return v.astype(BF16).astype(F32)


def _recip(v):
    return pl.reciprocal(v, approx=True)


def _recip_nr(v):
    r = pl.reciprocal(v, approx=True)
    return r * (2.0 - v * r)


def _silu(v):
    return v * (0.5 * jnp.tanh(0.5 * v) + 0.5)


def _cat(parts):
    return jnp.concatenate(parts, axis=1)


def _pk(v):
    return pltpu.bitcast(v, U32)


def _up(v):
    return pltpu.bitcast(v, BF16)


def _pair_allreduce(v, op):
    v = op(v, pltpu.roll(v, 2, 0))
    return op(v, pltpu.roll(v, 4, 0))


def _dual_softmax(p, z=None):
    n = p.shape[-1]
    p = p.reshape(8, 8, n)
    mx = _pair_allreduce(jnp.max(p, axis=0), jnp.maximum)
    mn = _pair_allreduce(jnp.min(p, axis=0), jnp.minimum)
    ep = jnp.exp2(p - mx[None])
    en = jnp.exp2(mn[None] - p)
    sp = _pair_allreduce(jnp.sum(ep, axis=0), jnp.add)
    sn = _pair_allreduce(jnp.sum(en, axis=0), jnp.add)
    if z is None:
        rp, rn = _recip(sp), _recip(sn)
    else:
        dp = _pair_allreduce(jnp.sum(ep * z[:64].reshape(8, 8, n), axis=0), jnp.add)
        dn = _pair_allreduce(jnp.sum(en * z[64:].reshape(8, 8, n), axis=0), jnp.add)
        rd = _recip(dp * sn + (dn + 1e-6 * sn) * sp)
        rp, rn = sn * rd, sp * rd
    return jnp.concatenate([ep * rp[None], en * rn[None]], axis=0).reshape(LANE, n).astype(BF16)


def _kernel(x_hbm, wqkv_hbm, phi_hbm, wo_hbm, wr_hbm, wg_hbm, wu_hbm, wd_hbm, out_hbm,
            x_buf, xn3, out_buf, wraw, phi_buf, wr_buf, wo_buf, wg_buf, wu_buf, wd_buf,
            wq3, wk3, wv3, phik3, vaug3, zrow, zbuf, phiq3, lmat, o3, r_buf, s_buf, fix_buf, pbuf,
            sem, sem_o):
    def cp(src, dst, slot):
        return pltpu.make_async_copy(src, dst, sem.at[slot])

    def x_rows(r0, n, slot):
        return cp(x_hbm.at[pl.ds(r0, n)], x_buf.at[pl.ds(r0, n)], slot)

    def w_cols(j, g0, g1, slot):
        n = (g1 - g0) * LANE
        return cp(wqkv_hbm.at[:, pl.ds(j * D + g0 * LANE, n)], wraw.at[j, :, pl.ds(g0 * LANE, n)], slot)

    def phi_heads(h0, h1, slot):
        return cp(phi_hbm.at[pl.ds(h0, h1 - h0)], phi_buf.at[pl.ds(h0, h1 - h0)], slot)

    groups = [
        [x_rows(0, T, 0), cp(wr_hbm, wr_buf, 0), phi_heads(0, 8, 0)],
        [w_cols(1, 0, 2, 1)],
        [phi_heads(8, H, 2), w_cols(1, 2, 4, 2)],
        [x_rows(T, T, 3), w_cols(1, 4, 5, 3)],
        [w_cols(1, 5, KB, 4), x_rows(2 * T, T, 4)],
        [w_cols(2, 0, KB, 5), x_rows(3 * T, T, 5)],
        [x_rows(4 * T, S - 4 * T, 6), w_cols(0, 0, KB, 6), cp(wo_hbm, wo_buf.at[:, pl.ds(0, D)], 6)],
        [cp(wg_hbm, wg_buf, 7), cp(wu_hbm, wu_buf, 7), cp(wd_hbm, wd_buf.at[:, pl.ds(0, D)], 7)],
    ]
    for grp in groups:
        for c in grp:
            c.start()

    def arrive(k):
        for c in groups[k]:
            c.wait()

    zero = []

    def put_blocks(dst, r0, val):
        n = val.shape[0]
        for k in range(KB):
            blk = val[:, k * LANE:(k + 1) * LANE].astype(BF16)
            if dst.dtype == U32:
                dst[k, r0 // 2:(r0 + n) // 2, :] = _pk(blk)
            else:
                dst[k, r0:r0 + n, :] = blk

    def xn_rows(r0, n, k0=0, k1=KB):
        return _cat([xn3[k, pl.ds(r0, n), :] for k in range(k0, k1)])

    def layernorm(row0, n, ch, chain):
        z = None
        eps = _rb(jnp.full((1, 1), 1e-5, F32))
        for r0 in range(row0, row0 + n, ch):
            xf = x_buf[r0:r0 + ch, :].astype(F32)
            mean = jnp.broadcast_to(jnp.sum(xf, axis=-1, keepdims=True) * (1.0 / D), (ch, LANE))
            if z is not None:
                mean = mean + z
            c = xf - _cat([mean] * KB)
            var = jnp.sum(c * c, axis=-1, keepdims=True) * (1.0 / D)
            rs = _recip_nr(_rb(jnp.sqrt(_rb(_rb(var) + eps))))
            xn = (xf - _cat([_rb(mean)] * KB)) * rs
            put_blocks(xn3, r0, xn)
            if chain == "scale":
                z = jnp.where(rs < 0.0, 1.0, 0.0)
            elif chain == "result":
                u = pltpu.bitcast(xn, U32)
                acc = functools.reduce(jnp.bitwise_or, [u[:, k * LANE:(k + 1) * LANE] for k in range(KB)])
                z = pltpu.bitcast(acc & jnp.concatenate(zero * (ch // 8), axis=0), F32)

    er = lax.broadcasted_iota(jnp.int32, (LANE, DH), 0)
    ec = lax.broadcasted_iota(jnp.int32, (LANE, DH), 1)
    eye4 = jnp.where((er % (2 * DH)) // 2 == ec, 1.0, 0.0).astype(BF16)
    br = lax.broadcasted_iota(jnp.int32, (LANE, LANE), 0)
    bc = lax.broadcasted_iota(jnp.int32, (LANE, LANE), 1)
    bmask = (2 * (br // (2 * DH)) + br % 2) == bc // DH
    bd = {}

    def blockdiag(g0, g1):
        for g in range(g0, g1):
            t = _nt(eye4, phi_buf[4 * g:4 * g + 4].reshape(LANE, DH))
            bd[g] = jnp.where(bmask, t, 0.0).astype(BF16)

    def fold(j, dst, g0, g1):
        for g in range(g0, g1):
            put_blocks(dst, g * LANE, _nt(bd[g], wraw[j, :, g * LANE:(g + 1) * LANE]) * LOG2E)

    pending = []

    def pin(value, lag, off=0):
        pending.append((lag, off, value))

    def lhs(words):
        todo = [(lag - 1, off, value) for lag, off, value in pending]
        pending[:] = [p for p in todo if p[0] > 0]
        for _, off, value in [p for p in todo if p[0] == 0]:
            w = words[0]
            tied = w[off:off + 8] ^ (pltpu.bitcast(value, U32) & zero[0])
            words = [jnp.concatenate(([w[:off]] if off else []) + [tied, w[off + 8:]], axis=0)] + words[1:]
        return _cat([_up(w) for w in words])

    parked = []

    def keys(b, g0=0, g1=KB, park=False):
        r0, r1 = g0 * LANE, g1 * LANE
        re = r1 + RB if g1 == KB else r1
        pt = _nt(lhs([wk3[k, r0 // 2:re // 2, :] for k in range(KB)]), xn_rows(b * LANE, LANE))
        if re > r1:
            r_buf[:, b * LANE:(b + 1) * LANE] = pt[r1 - r0:r1 - r0 + 8, :]
        for j in range(r0 // 64, r1 // 64):
            p = pt[j * 64 - r0:(j + 1) * 64 - r0, :]
            if park and j == r1 // 64 - 1:
                pbuf[len(parked)] = p
                parked.append((b, j))
            else:
                phik3[b, j * LANE:(j + 1) * LANE, :] = _dual_softmax(p)

    def unpark():
        b, j = parked[-1]
        phik3[b, j * LANE:(j + 1) * LANE, :] = _dual_softmax(pbuf[len(parked) - 1])

    def values(b):
        vt = _nt(_cat([_up(wv3[k]) for k in range(KB)]), xn_rows(b * LANE, LANE))
        for j in range(NPAIR):
            vaug3[b, j * VR:j * VR + 2 * DH, :] = vt[j * 2 * DH:(j + 1) * 2 * DH]
            vaug3[b, j * VR + 2 * DH:(j + 1) * VR, :] = jnp.ones((8, LANE), F32)

    ffn_q = []

    def ffn_step(lag, off=0):
        if ffn_q and lag:
            pin(ffn_q.pop(0)(), lag, off)

    def stage_q(i):
        for bl in range(TB):
            pt = _nt(lhs([wq3[k] for k in range(KB)]), xn_rows((i * TB + bl) * LANE, LANE))
            for j in range(NPAIR):
                phiq3[bl, j * LANE:(j + 1) * LANE, :] = _dual_softmax(
                    pt[j * 64:(j + 1) * 64, :], None if i == 0 else zbuf[j])

    def stage_kv():
        lr = lax.broadcasted_iota(jnp.int32, (PR, LANE), 0)
        lc = lax.broadcasted_iota(jnp.int32, (PR, LANE), 1)
        keep = jnp.where(lr < 2 * DH, lr // DH, (lr - 2 * DH) // 8) == lc % 2
        for j in range(NPAIR):
            va = _cat([vaug3[b, j * VR:(j + 1) * VR, :] for b in range(NB)])
            pk = _cat([phik3[b, j * LANE:(j + 1) * LANE, :] for b in range(NB)])
            kvt = _nt(va, pk)
            z = kvt[2 * DH:, :]
            lmat[j] = _pk(jnp.where(keep, jnp.concatenate([kvt, z], axis=0), 0.0).astype(BF16))
            zrow[j] = z

    def stage_b(i, slots):
        for g in range(KB):
            parts = []
            for j in (2 * g, 2 * g + 1):
                pq = _cat([phiq3[bl, j * LANE:(j + 1) * LANE, :] for bl in range(TB)])
                if i == 0:
                    nt = _nn(_up(lmat[j]), pq)
                    for h in range(2):
                        den = nt[2 * DH + 8 * h:2 * DH + 8 * h + 8, :] + 1e-6
                        num = nt[h * DH:(h + 1) * DH, :].reshape(4, 8, T)
                        parts.append((num * _recip(den)[None]).reshape(DH, T))
                else:
                    lw = lmat[j, 0:DH, :]
                    parts.append(_nn(lhs([lw]) if j % 2 == 0 else _up(lw), pq))
            ffn_step(*slots[g])
            o3[g] = _pk(jnp.concatenate(parts, axis=0).T.astype(BF16))

    def stage_c(i, routed=None, mid=None):
        r0 = i * T
        o = [o3[k] for k in range(KB)]
        copies = []
        for n in range(0, KB, 2):
            if mid is not None and n == KB - 2:
                mid()
            parts = []
            for m in (n, n + 1):
                halves = []
                for h in range(TB):
                    halves.append(_nn(lhs([w[h * 64:(h + 1) * 64] for w in o]),
                                      wo_buf[:, m * LANE:(m + 1) * LANE]))
                    before_b = h == TB - 1 and (m == KB - 1 or (mid is not None and m == KB - 3))
                    ffn_step(4 if before_b else 2)
                parts.append(jnp.concatenate(halves, axis=0))
            s = _cat(parts)
            cols = slice(n * LANE, (n + 2) * LANE)
            b = xn_rows(r0, T, n, n + 2).astype(F32)
            if routed is None:
                s_buf[r0:r0 + T, cols] = s
            else:
                idx, brow = routed()
                sel = (lax.broadcasted_iota(jnp.int32, (T, 2 * LANE), 0) + r0) == idx
                b = jnp.where(sel, brow[:, cols], b)
            res = x_buf[r0:r0 + T, cols].astype(F32) + s * _silu(b)
            out_buf[r0:r0 + T, cols] = res.astype(BF16)
            if routed is not None:
                win = (pl.ds(r0, T), pl.ds(n * LANE, 2 * LANE))
                copies.append(pltpu.make_async_copy(out_buf.at[win], out_hbm.at[win], sem_o.at[2]))
                copies[-1].start()
        if routed is None:
            copies.append(pltpu.make_async_copy(out_buf.at[pl.ds(r0, T)], out_hbm.at[pl.ds(r0, T)], sem_o.at[0]))
            copies[-1].start()
        return copies

    arrive(0)
    layernorm(0, T, LANE, None)
    wrf = wr_buf[...].reshape(1, D).astype(F32)
    for k in range(KB):
        wk3[k, D // 2:(D + RB) // 2, :] = _pk(
            jnp.broadcast_to(wrf[:, k * LANE:(k + 1) * LANE], (RB, LANE)).astype(BF16))
    sign = lax.shift_right_logical(pltpu.bitcast(wrf[:, 0:LANE], jnp.int32), 31)
    zrt = pl.multiple_of(lax.shift_right_logical(jnp.max(sign), 1), 8)
    zero.append(jnp.full((8, LANE), zrt, jnp.int32).astype(U32))
    blockdiag(0, 2)
    arrive(1)
    fold(1, wk3, 0, 2)
    keys(0, 0, 2)
    keys(1, 0, 2, True)
    arrive(2)
    unpark()
    blockdiag(2, KB)
    fold(1, wk3, 2, 4)
    keys(0, 2, 4)
    keys(1, 2, 4, True)
    arrive(3)
    unpark()
    fold(1, wk3, 4, 5)
    keys(0, 4, 5)
    keys(1, 4, 5)
    for b in (2, 3):
        layernorm(b * LANE, LANE, 64, "scale")
        keys(b, 0, 5, b == 3)
    arrive(4)
    unpark()
    fold(1, wk3, 5, KB)
    for b in range(4):
        keys(b, 5, KB, b == 3)
    layernorm(2 * T, T, RB, "result")
    arrive(5)
    unpark()
    for g in range(KB):
        wt = wraw[2, :, g * LANE:(g + 1) * LANE].T
        for k in range(KB):
            wv3[k, g * 64:(g + 1) * 64, :] = _pk(wt[:, k * LANE:(k + 1) * LANE]) ^ jnp.concatenate(zero * 8, axis=0)
    pin(wv3[0, pl.ds(zrt, 8), :], 2, 480)
    for op in PHASE1.split():
        if op == "|":
            arrive(6)
        elif op == "F":
            fold(0, wq3, 0, KB)
        elif op[0] == "L":
            layernorm(int(op[1]) * T, T, RB, "result" if op == "L3" else "scale")
        else:
            for b in range(int(op[1]) * TB, (int(op[1]) + 1) * TB):
                keys(b) if op[0] == "K" else values(b)
    stage_q(0)
    stage_kv()

    arrive(7)
    r = _rb(r_buf[0:1, :])
    rmax = jnp.max(r)
    pos = lax.broadcasted_iota(jnp.int32, (1, S), 1)
    idx = jnp.clip(jnp.min(jnp.where(r == rmax, pos, S)), 0, S - 1)
    blk = pl.multiple_of((idx // RB) * RB, RB)
    xblk = xn_rows(blk, RB).astype(F32)
    rowsel = (lax.broadcasted_iota(jnp.int32, (RB, D), 0) + blk) == idx
    xs = jnp.broadcast_to(jnp.sum(jnp.where(rowsel, xblk, 0.0), axis=0, keepdims=True), (8, D))
    part, act, y = {}, {}, {}

    def gate_up(w_buf, j, h):
        def f():
            v = _nn(xs[:, h * KH:(h + 1) * KH], w_buf[h * KH:(h + 1) * KH, j * LANE:(j + 1) * LANE])
            key = (w_buf is wu_buf, j)
            part[key] = v if h == 0 else _rb(part[key] + v)
            if h == 1 and w_buf is wu_buf:
                act[j] = _rb(_rb(_silu(part.pop((False, j)))) * part.pop(key))
            return v
        return f

    def down(m, n):
        def f():
            a = _cat([act[j] for j in range(4 * m, 4 * m + 4)])
            v = _nn(a, wd_buf[m * KH:(m + 1) * KH, n * LANE:(n + 1) * LANE])
            y[n] = v if m == 0 else y[n] + v
            return v
        return f

    def routed():
        if "row" not in part:
            rs = _rb(0.5 * jnp.tanh(0.5 * jnp.full((1, 1), rmax, F32)) + 0.5)
            yf = _rb(_rb(_cat([y[n] for n in range(KB)])) * rs)
            part["row"] = _rb(xs + yf)[0:1, :]
        return idx, part["row"]

    sets = []
    for m in range(NG + 1):
        gu = [gate_up(w, j, h) for j in range(4 * m, 4 * m + 4) for w in (wg_buf, wu_buf) for h in range(2)
              ] if m < NG else []
        dn = [down(m - 1, n) for n in range(KB)] if m > 0 else []
        while gu or dn:
            sets += gu[:2] + dn[:1]
            gu, dn = gu[2:], dn[1:]

    for j in range(NPAIR):
        zbuf[j] = jnp.concatenate([zrow[j]] * (LANE // 8), axis=0).T

    b_slots = ((4, 0),) * 5 + ((3, 16), (2, 48))
    outs = []
    for i in range(NTILE - 1):
        stage_b(i, b_slots + ((0, 0),))
        if i == 0:
            ffn_q.extend(sets)
        pin(o3[0, pl.ds(zrt, 8), :], 1, 480)
        stage_q(i + 1)
        ffn_step(2)
        outs += stage_c(i, mid=(lambda: stage_b(NTILE - 1, b_slots + ((2, 0),))) if i == NTILE - 2 else None)
    assert not ffn_q, len(ffn_q)

    sb = pl.multiple_of(jnp.minimum(blk, S - T - RB), RB)
    res = (x_buf[pl.ds(blk, RB), :].astype(F32)
           + s_buf[pl.ds(sb, RB), :] * _silu(jnp.where(rowsel, routed()[1], xblk)))
    fix_buf[...] = res.astype(BF16)

    last = stage_c(NTILE - 1, routed)
    for c in outs:
        c.wait()

    @pl.when(idx < S - T)
    def _():
        c = pltpu.make_async_copy(fix_buf, out_hbm.at[pl.ds(blk, RB)], sem_o.at[1])
        c.start()
        c.wait()

    for c in last:
        c.wait()


def _build():
    any_spec = pl.BlockSpec(memory_space=pl.ANY)
    scratch = [
        pltpu.VMEM((S, D), BF16),
        pltpu.VMEM((KB, S, LANE), BF16),
        pltpu.VMEM((S, D), BF16),
        pltpu.VMEM((3, D, D), BF16),
        pltpu.VMEM((H, DH, DH), BF16),
        pltpu.VMEM((D,), BF16),
        pltpu.VMEM((D, WP), BF16),
        pltpu.VMEM((D, F), BF16),
        pltpu.VMEM((D, F), BF16),
        pltpu.VMEM((F, WP), BF16),
        pltpu.VMEM((KB, D // 2, LANE), U32),
        pltpu.VMEM((KB, (D + RB) // 2, LANE), U32),
        pltpu.VMEM((KB, D // 2, LANE), U32),
        pltpu.VMEM((NB, 2 * D, LANE), BF16),
        pltpu.VMEM((NB, NPAIR * VR, LANE), F32),
        pltpu.VMEM((NPAIR, 8, LANE), F32),
        pltpu.VMEM((NPAIR, LANE, LANE), F32),
        pltpu.VMEM((TB, 2 * D, LANE), BF16),
        pltpu.VMEM((NPAIR, PR // 2, LANE), U32),
        pltpu.VMEM((KB, T // 2, LANE), U32),
        pltpu.VMEM((8, S), F32),
        pltpu.VMEM((S - T, D), F32),
        pltpu.VMEM((RB, D), BF16),
        pltpu.VMEM((4, 64, LANE), F32),
        pltpu.SemaphoreType.DMA((8,)),
        pltpu.SemaphoreType.DMA((3,)),
    ]
    return pl.pallas_call(
        _kernel,
        out_shape=jax.ShapeDtypeStruct((S, D), BF16),
        in_specs=[any_spec] * 8,
        out_specs=any_spec,
        scratch_shapes=scratch,
        compiler_params=pltpu.CompilerParams(vmem_limit_bytes=100 * 1024 * 1024,
                                             disable_semaphore_checks=True),
        name="hedgehog_mod",
    )


@jax.jit
def pallas_recurrent_scan__linear_kernel_hedgehog__moe_arch_mod__prompt_kernel(
    A_x: jax.Array,
    A_wqkv: jax.Array,
    A_w_phi: jax.Array,
    A_wo: jax.Array,
    B_x: jax.Array,
    B_w_r: jax.Array,
    B_w_gate: jax.Array,
    B_w_up: jax.Array,
    B_w_down: jax.Array,
):
    del B_x
    out = _build()(A_x.reshape(S, D), A_wqkv, A_w_phi, A_wo, B_w_r, B_w_gate, B_w_up, B_w_down)
    return out.reshape(1, S, D)
```

```python
import functools

import jax
import jax.numpy as jnp
from jax import lax
import jax.experimental.pallas as pl
import jax.experimental.pallas.tpu as pltpu

S, D, H, DH, F = 2048, 1024, 32, 32, 3584
LANE = 128
KB = D // LANE
KH = D // 2
T = 256
TB = T // LANE
NB = S // LANE
NTILE = S // T
NPAIR = H // 2
VR = 2 * DH + 8
PR = 2 * DH + 16
RB = 16
WP = D + LANE
NG = F // KH
LOG2E = 1.4426950408889634
F32 = jnp.float32
BF16 = jnp.bfloat16
U32 = jnp.uint32

PHASE1 = "K2 V0 V1 | F V2 L3 K3 L4 V3 K4 L5 V4 K5 L6 V5 K6 L7 V6 K7 V7"


def _nt(a, b):
    return lax.dot_general(a, b, (((1,), (1,)), ((), ())), preferred_element_type=F32)


def _nn(a, b):
    return jnp.dot(a, b, preferred_element_type=F32)


def _rb(v):
    return v.astype(BF16).astype(F32)


def _recip(v):
    return pl.reciprocal(v, approx=True)


def _recip_nr(v):
    r = pl.reciprocal(v, approx=True)
    return r * (2.0 - v * r)


def _silu(v):
    return v * (0.5 * jnp.tanh(0.5 * v) + 0.5)


def _cat(parts):
    return jnp.concatenate(parts, axis=1)


def _pk(v):
    return pltpu.bitcast(v, U32)


def _up(v):
    return pltpu.bitcast(v, BF16)


def _pair_allreduce(v, op):
    v = op(v, pltpu.roll(v, 2, 0))
    return op(v, pltpu.roll(v, 4, 0))


def _dual_softmax(p, z=None):
    n = p.shape[-1]
    p = p.reshape(8, 8, n)
    mx = _pair_allreduce(jnp.max(p, axis=0), jnp.maximum)
    mn = _pair_allreduce(jnp.min(p, axis=0), jnp.minimum)
    ep = jnp.exp2(p - mx[None])
    en = jnp.exp2(mn[None] - p)
    sp = _pair_allreduce(jnp.sum(ep, axis=0), jnp.add)
    sn = _pair_allreduce(jnp.sum(en, axis=0), jnp.add)
    if z is None:
        rp, rn = _recip(sp), _recip(sn)
    else:
        dp = _pair_allreduce(jnp.sum(ep * z[:64].reshape(8, 8, n), axis=0), jnp.add)
        dn = _pair_allreduce(jnp.sum(en * z[64:].reshape(8, 8, n), axis=0), jnp.add)
        rd = _recip(dp * sn + (dn + 1e-6 * sn) * sp)
        rp, rn = sn * rd, sp * rd
    return jnp.concatenate([ep * rp[None], en * rn[None]], axis=0).reshape(LANE, n).astype(BF16)


def _kernel(x_hbm, wqkv_hbm, phi_hbm, wo_hbm, wr_hbm, wg_hbm, wu_hbm, wd_hbm, out_hbm,
            x_buf, xn3, out_buf, wraw, phi_buf, wr_buf, wo_buf, wg_buf, wu_buf, wd_buf,
            wq3, wk3, wv3, phik3, vaug3, zrow, zbuf, phiq3, lmat, o3, r_buf, s_buf, fix_buf, pbuf,
            sem, sem_o):
    def cp(src, dst, slot):
        return pltpu.make_async_copy(src, dst, sem.at[slot])

    def x_rows(r0, n, slot):
        return cp(x_hbm.at[pl.ds(r0, n)], x_buf.at[pl.ds(r0, n)], slot)

    def w_cols(j, g0, g1, slot):
        n = (g1 - g0) * LANE
        return cp(wqkv_hbm.at[:, pl.ds(j * D + g0 * LANE, n)], wraw.at[j, :, pl.ds(g0 * LANE, n)], slot)

    def phi_heads(h0, h1, slot):
        return cp(phi_hbm.at[pl.ds(h0, h1 - h0)], phi_buf.at[pl.ds(h0, h1 - h0)], slot)

    groups = [
        [x_rows(0, T, 0), cp(wr_hbm, wr_buf, 0), phi_heads(0, 8, 0)],
        [w_cols(1, 0, 2, 1)],
        [phi_heads(8, H, 2), w_cols(1, 2, 4, 2)],
        [x_rows(T, T, 3), w_cols(1, 4, 5, 3)],
        [w_cols(1, 5, KB, 4), x_rows(2 * T, T, 4)],
        [w_cols(2, 0, KB, 5)],
        [x_rows(3 * T, S - 3 * T, 6), w_cols(0, 0, KB, 6)],
        [cp(wo_hbm, wo_buf.at[:, pl.ds(0, D)], 7), cp(wg_hbm, wg_buf, 7), cp(wu_hbm, wu_buf, 7),
         cp(wd_hbm, wd_buf.at[:, pl.ds(0, D)], 7)],
    ]
    for grp in groups:
        for c in grp:
            c.start()

    def arrive(k):
        for c in groups[k]:
            c.wait()

    zero = []

    def put_blocks(dst, r0, val):
        n = val.shape[0]
        for k in range(KB):
            blk = val[:, k * LANE:(k + 1) * LANE].astype(BF16)
            if dst.dtype == U32:
                dst[k, r0 // 2:(r0 + n) // 2, :] = _pk(blk)
            else:
                dst[k, r0:r0 + n, :] = blk

    def xn_rows(r0, n, k0=0, k1=KB):
        return _cat([xn3[k, pl.ds(r0, n), :] for k in range(k0, k1)])

    def layernorm(row0, n, ch, chain):
        z = None
        eps = _rb(jnp.full((1, 1), 1e-5, F32))
        for r0 in range(row0, row0 + n, ch):
            xf = x_buf[r0:r0 + ch, :].astype(F32)
            mean = jnp.broadcast_to(jnp.sum(xf, axis=-1, keepdims=True) * (1.0 / D), (ch, LANE))
            if z is not None:
                mean = mean + z
            c = xf - _cat([mean] * KB)
            var = jnp.sum(c * c, axis=-1, keepdims=True) * (1.0 / D)
            rs = _recip_nr(_rb(jnp.sqrt(_rb(_rb(var) + eps))))
            xn = (xf - _cat([_rb(mean)] * KB)) * rs
            put_blocks(xn3, r0, xn)
            if chain == "scale":
                z = jnp.where(rs < 0.0, 1.0, 0.0)
            elif chain == "result":
                u = pltpu.bitcast(xn, U32)
                acc = functools.reduce(jnp.bitwise_or, [u[:, k * LANE:(k + 1) * LANE] for k in range(KB)])
                z = pltpu.bitcast(acc & jnp.concatenate(zero * (ch // 8), axis=0), F32)

    er = lax.broadcasted_iota(jnp.int32, (LANE, DH), 0)
    ec = lax.broadcasted_iota(jnp.int32, (LANE, DH), 1)
    eye4 = jnp.where((er % (2 * DH)) // 2 == ec, 1.0, 0.0).astype(BF16)
    br = lax.broadcasted_iota(jnp.int32, (LANE, LANE), 0)
    bc = lax.broadcasted_iota(jnp.int32, (LANE, LANE), 1)
    bmask = (2 * (br // (2 * DH)) + br % 2) == bc // DH
    bd = {}

    def blockdiag(g0, g1):
        for g in range(g0, g1):
            t = _nt(eye4, phi_buf[4 * g:4 * g + 4].reshape(LANE, DH))
            bd[g] = jnp.where(bmask, t, 0.0).astype(BF16)

    def fold(j, dst, g0, g1):
        for g in range(g0, g1):
            put_blocks(dst, g * LANE, _nt(bd[g], wraw[j, :, g * LANE:(g + 1) * LANE]) * LOG2E)

    pending = []

    def pin(value, lag, off=0):
        pending.append((lag, off, value))

    def lhs(words):
        todo = [(lag - 1, off, value) for lag, off, value in pending]
        pending[:] = [p for p in todo if p[0] > 0]
        for _, off, value in [p for p in todo if p[0] == 0]:
            w = words[0]
            tied = w[off:off + 8] ^ (pltpu.bitcast(value, U32) & zero[0])
            words = [jnp.concatenate(([w[:off]] if off else []) + [tied, w[off + 8:]], axis=0)] + words[1:]
        return _cat([_up(w) for w in words])

    parked = []

    def keys(b, g0=0, g1=KB, park=False):
        r0, r1 = g0 * LANE, g1 * LANE
        re = r1 + RB if g1 == KB else r1
        pt = _nt(lhs([wk3[k, r0 // 2:re // 2, :] for k in range(KB)]), xn_rows(b * LANE, LANE))
        if re > r1:
            r_buf[:, b * LANE:(b + 1) * LANE] = pt[r1 - r0:r1 - r0 + 8, :]
        for j in range(r0 // 64, r1 // 64):
            p = pt[j * 64 - r0:(j + 1) * 64 - r0, :]
            if park and j == r1 // 64 - 1:
                pbuf[len(parked)] = p
                parked.append((b, j))
            else:
                phik3[b, j * LANE:(j + 1) * LANE, :] = _dual_softmax(p)

    def unpark():
        b, j = parked[-1]
        phik3[b, j * LANE:(j + 1) * LANE, :] = _dual_softmax(pbuf[len(parked) - 1])

    def values(b):
        vt = _nt(_cat([_up(wv3[k]) for k in range(KB)]), xn_rows(b * LANE, LANE))
        for j in range(NPAIR):
            vaug3[b, j * VR:j * VR + 2 * DH, :] = vt[j * 2 * DH:(j + 1) * 2 * DH]
            vaug3[b, j * VR + 2 * DH:(j + 1) * VR, :] = jnp.ones((8, LANE), F32)

    ffn_q = []

    def ffn_step(lag, off=0):
        if ffn_q and lag:
            pin(ffn_q.pop(0)(), lag, off)

    def stage_q(i):
        for bl in range(TB):
            pt = _nt(lhs([wq3[k] for k in range(KB)]), xn_rows((i * TB + bl) * LANE, LANE))
            for j in range(NPAIR):
                phiq3[bl, j * LANE:(j + 1) * LANE, :] = _dual_softmax(
                    pt[j * 64:(j + 1) * 64, :], None if i == 0 else zbuf[j])

    def stage_kv():
        lr = lax.broadcasted_iota(jnp.int32, (PR, LANE), 0)
        lc = lax.broadcasted_iota(jnp.int32, (PR, LANE), 1)
        keep = jnp.where(lr < 2 * DH, lr // DH, (lr - 2 * DH) // 8) == lc % 2
        for j in range(NPAIR):
            va = _cat([vaug3[b, j * VR:(j + 1) * VR, :] for b in range(NB)])
            pk = _cat([phik3[b, j * LANE:(j + 1) * LANE, :] for b in range(NB)])
            kvt = _nt(va, pk)
            z = kvt[2 * DH:, :]
            lmat[j] = _pk(jnp.where(keep, jnp.concatenate([kvt, z], axis=0), 0.0).astype(BF16))
            zrow[j] = z

    def stage_b(i, slots):
        for g in range(KB):
            parts = []
            for j in (2 * g, 2 * g + 1):
                pq = _cat([phiq3[bl, j * LANE:(j + 1) * LANE, :] for bl in range(TB)])
                if i == 0:
                    nt = _nn(_up(lmat[j]), pq)
                    for h in range(2):
                        den = nt[2 * DH + 8 * h:2 * DH + 8 * h + 8, :] + 1e-6
                        num = nt[h * DH:(h + 1) * DH, :].reshape(4, 8, T)
                        parts.append((num * _recip(den)[None]).reshape(DH, T))
                else:
                    lw = lmat[j, 0:DH, :]
                    parts.append(_nn(lhs([lw]) if j % 2 == 0 else _up(lw), pq))
            ffn_step(*slots[g])
            o3[g] = _pk(jnp.concatenate(parts, axis=0).T.astype(BF16))

    def stage_c(i, routed=None, mid=None):
        r0 = i * T
        o = [o3[k] for k in range(KB)]
        copies = []
        for n in range(0, KB, 2):
            if mid is not None and n == KB - 2:
                mid()
            parts = []
            for m in (n, n + 1):
                halves = []
                for h in range(TB):
                    halves.append(_nn(lhs([w[h * 64:(h + 1) * 64] for w in o]),
                                      wo_buf[:, m * LANE:(m + 1) * LANE]))
                    before_b = h == TB - 1 and (m == KB - 1 or (mid is not None and m == KB - 3))
                    ffn_step(4 if before_b else 2)
                parts.append(jnp.concatenate(halves, axis=0))
            s = _cat(parts)
            cols = slice(n * LANE, (n + 2) * LANE)
            b = xn_rows(r0, T, n, n + 2).astype(F32)
            if routed is None:
                s_buf[r0:r0 + T, cols] = s
            else:
                idx, brow = routed()
                sel = (lax.broadcasted_iota(jnp.int32, (T, 2 * LANE), 0) + r0) == idx
                b = jnp.where(sel, brow[:, cols], b)
            res = x_buf[r0:r0 + T, cols].astype(F32) + s * _silu(b)
            out_buf[r0:r0 + T, cols] = res.astype(BF16)
            if routed is not None:
                win = (pl.ds(r0, T), pl.ds(n * LANE, 2 * LANE))
                copies.append(pltpu.make_async_copy(out_buf.at[win], out_hbm.at[win], sem_o.at[2]))
                copies[-1].start()
        if routed is None:
            copies.append(pltpu.make_async_copy(out_buf.at[pl.ds(r0, T)], out_hbm.at[pl.ds(r0, T)], sem_o.at[0]))
            copies[-1].start()
        return copies

    arrive(0)
    layernorm(0, T, LANE, None)
    wrf = wr_buf[...].reshape(1, D).astype(F32)
    for k in range(KB):
        wk3[k, D // 2:(D + RB) // 2, :] = _pk(
            jnp.broadcast_to(wrf[:, k * LANE:(k + 1) * LANE], (RB, LANE)).astype(BF16))
    sign = lax.shift_right_logical(pltpu.bitcast(wrf[:, 0:LANE], jnp.int32), 31)
    zrt = pl.multiple_of(lax.shift_right_logical(jnp.max(sign), 1), 8)
    zero.append(jnp.full((8, LANE), zrt, jnp.int32).astype(U32))
    blockdiag(0, 2)
    arrive(1)
    fold(1, wk3, 0, 2)
    keys(0, 0, 2)
    keys(1, 0, 2, True)
    arrive(2)
    unpark()
    blockdiag(2, KB)
    fold(1, wk3, 2, 4)
    keys(0, 2, 4)
    keys(1, 2, 4, True)
    arrive(3)
    unpark()
    fold(1, wk3, 4, 5)
    keys(0, 4, 5)
    keys(1, 4, 5)
    for b in (2, 3):
        layernorm(b * LANE, LANE, 64, "scale")
        keys(b, 0, 5, b == 3)
    arrive(4)
    unpark()
    fold(1, wk3, 5, KB)
    for b in range(4):
        keys(b, 5, KB, b == 3)
    layernorm(2 * T, T, RB, "result")
    arrive(5)
    unpark()
    for g in range(KB):
        wt = wraw[2, :, g * LANE:(g + 1) * LANE].T
        for k in range(KB):
            wv3[k, g * 64:(g + 1) * 64, :] = _pk(wt[:, k * LANE:(k + 1) * LANE]) ^ jnp.concatenate(zero * 8, axis=0)
    pin(wv3[0, pl.ds(zrt, 8), :], 2, 480)
    for op in PHASE1.split():
        if op == "|":
            arrive(6)
        elif op == "F":
            fold(0, wq3, 0, KB)
        elif op[0] == "L":
            layernorm(int(op[1]) * T, T, RB, "scale")
        else:
            for b in range(int(op[1]) * TB, (int(op[1]) + 1) * TB):
                keys(b) if op[0] == "K" else values(b)
    stage_q(0)
    stage_kv()

    arrive(7)
    r = _rb(r_buf[0:1, :])
    rmax = jnp.max(r)
    pos = lax.broadcasted_iota(jnp.int32, (1, S), 1)
    idx = jnp.clip(jnp.min(jnp.where(r == rmax, pos, S)), 0, S - 1)
    blk = pl.multiple_of((idx // RB) * RB, RB)
    xblk = xn_rows(blk, RB).astype(F32)
    rowsel = (lax.broadcasted_iota(jnp.int32, (RB, D), 0) + blk) == idx
    xs = jnp.broadcast_to(jnp.sum(jnp.where(rowsel, xblk, 0.0), axis=0, keepdims=True), (8, D))
    part, act, y = {}, {}, {}

    def gate_up(w_buf, j, h):
        def f():
            v = _nn(xs[:, h * KH:(h + 1) * KH], w_buf[h * KH:(h + 1) * KH, j * LANE:(j + 1) * LANE])
            key = (w_buf is wu_buf, j)
            part[key] = v if h == 0 else _rb(part[key] + v)
            if h == 1 and w_buf is wu_buf:
                act[j] = _rb(_rb(_silu(part.pop((False, j)))) * part.pop(key))
            return v
        return f

    def down(m, n):
        def f():
            a = _cat([act[j] for j in range(4 * m, 4 * m + 4)])
            v = _nn(a, wd_buf[m * KH:(m + 1) * KH, n * LANE:(n + 1) * LANE])
            y[n] = v if m == 0 else y[n] + v
            return v
        return f

    def routed():
        if "row" not in part:
            rs = _rb(0.5 * jnp.tanh(0.5 * jnp.full((1, 1), rmax, F32)) + 0.5)
            yf = _rb(_rb(_cat([y[n] for n in range(KB)])) * rs)
            part["row"] = _rb(xs + yf)[0:1, :]
        return idx, part["row"]

    sets = []
    for m in range(NG + 1):
        gu = [gate_up(w, j, h) for j in range(4 * m, 4 * m + 4) for w in (wg_buf, wu_buf) for h in range(2)
              ] if m < NG else []
        dn = [down(m - 1, n) for n in range(KB)] if m > 0 else []
        while gu or dn:
            sets += gu[:2] + dn[:1]
            gu, dn = gu[2:], dn[1:]

    for j in range(NPAIR):
        zbuf[j] = jnp.concatenate([zrow[j]] * (LANE // 8), axis=0).T

    b_slots = ((4, 0),) * 5 + ((3, 16), (2, 48))
    outs = []
    for i in range(NTILE - 1):
        stage_b(i, b_slots + ((0, 0),))
        if i == 0:
            ffn_q.extend(sets)
        pin(o3[0, pl.ds(zrt, 8), :], 1, 480)
        stage_q(i + 1)
        ffn_step(2)
        outs += stage_c(i, mid=(lambda: stage_b(NTILE - 1, b_slots + ((2, 0),))) if i == NTILE - 2 else None)
    assert not ffn_q, len(ffn_q)

    sb = pl.multiple_of(jnp.minimum(blk, S - T - RB), RB)
    res = (x_buf[pl.ds(blk, RB), :].astype(F32)
           + s_buf[pl.ds(sb, RB), :] * _silu(jnp.where(rowsel, routed()[1], xblk)))
    fix_buf[...] = res.astype(BF16)

    last = stage_c(NTILE - 1, routed)
    for c in outs:
        c.wait()

    @pl.when(idx < S - T)
    def _():
        c = pltpu.make_async_copy(fix_buf, out_hbm.at[pl.ds(blk, RB)], sem_o.at[1])
        c.start()
        c.wait()

    for c in last:
        c.wait()


def _build():
    any_spec = pl.BlockSpec(memory_space=pl.ANY)
    scratch = [
        pltpu.VMEM((S, D), BF16),
        pltpu.VMEM((KB, S, LANE), BF16),
        pltpu.VMEM((S, D), BF16),
        pltpu.VMEM((3, D, D), BF16),
        pltpu.VMEM((H, DH, DH), BF16),
        pltpu.VMEM((D,), BF16),
        pltpu.VMEM((D, WP), BF16),
        pltpu.VMEM((D, F), BF16),
        pltpu.VMEM((D, F), BF16),
        pltpu.VMEM((F, WP), BF16),
        pltpu.VMEM((KB, D // 2, LANE), U32),
        pltpu.VMEM((KB, (D + RB) // 2, LANE), U32),
        pltpu.VMEM((KB, D // 2, LANE), U32),
        pltpu.VMEM((NB, 2 * D, LANE), BF16),
        pltpu.VMEM((NB, NPAIR * VR, LANE), F32),
        pltpu.VMEM((NPAIR, 8, LANE), F32),
        pltpu.VMEM((NPAIR, LANE, LANE), F32),
        pltpu.VMEM((TB, 2 * D, LANE), BF16),
        pltpu.VMEM((NPAIR, PR // 2, LANE), U32),
        pltpu.VMEM((KB, T // 2, LANE), U32),
        pltpu.VMEM((8, S), F32),
        pltpu.VMEM((S - T, D), F32),
        pltpu.VMEM((RB, D), BF16),
        pltpu.VMEM((4, 64, LANE), F32),
        pltpu.SemaphoreType.DMA((8,)),
        pltpu.SemaphoreType.DMA((3,)),
    ]
    return pl.pallas_call(
        _kernel,
        out_shape=jax.ShapeDtypeStruct((S, D), BF16),
        in_specs=[any_spec] * 8,
        out_specs=any_spec,
        scratch_shapes=scratch,
        compiler_params=pltpu.CompilerParams(vmem_limit_bytes=100 * 1024 * 1024,
                                             disable_semaphore_checks=True),
        name="hedgehog_mod",
    )


@jax.jit
def pallas_recurrent_scan__linear_kernel_hedgehog__moe_arch_mod__prompt_kernel(
    A_x: jax.Array,
    A_wqkv: jax.Array,
    A_w_phi: jax.Array,
    A_wo: jax.Array,
    B_x: jax.Array,
    B_w_r: jax.Array,
    B_w_gate: jax.Array,
    B_w_up: jax.Array,
    B_w_down: jax.Array,
):
    del B_x
    out = _build()(A_x.reshape(S, D), A_wqkv, A_w_phi, A_wo, B_w_r, B_w_gate, B_w_up, B_w_down)
    return out.reshape(1, S, D)
```

```python
import functools

import jax
import jax.numpy as jnp
from jax import lax
import jax.experimental.pallas as pl
import jax.experimental.pallas.tpu as pltpu

S, D, H, DH, F = 2048, 1024, 32, 32, 3584
LANE = 128
KB = D // LANE
KH = D // 2
T = 256
TB = T // LANE
NB = S // LANE
NTILE = S // T
NPAIR = H // 2
VR = 2 * DH + 8
PR = 2 * DH + 16
RB = 16
WP = D + LANE
NG = F // KH
LOG2E = 1.4426950408889634
F32 = jnp.float32
BF16 = jnp.bfloat16
U32 = jnp.uint32

PHASE1 = "K2 V0 V1 | F V2 L3 K3 L4 V3 K4 L5 V4 K5 L6 V5 K6 L7 V6 K7 V7"


def _nt(a, b):
    return lax.dot_general(a, b, (((1,), (1,)), ((), ())), preferred_element_type=F32)


def _nn(a, b):
    return jnp.dot(a, b, preferred_element_type=F32)


def _rb(v):
    return v.astype(BF16).astype(F32)


def _recip(v):
    return pl.reciprocal(v, approx=True)


def _recip_nr(v):
    r = pl.reciprocal(v, approx=True)
    return r * (2.0 - v * r)


def _silu(v):
    return v * (0.5 * jnp.tanh(0.5 * v) + 0.5)


def _cat(parts):
    return jnp.concatenate(parts, axis=1)


def _pk(v):
    return pltpu.bitcast(v, U32)


def _up(v):
    return pltpu.bitcast(v, BF16)


def _pair_allreduce(v, op):
    v = op(v, pltpu.roll(v, 2, 0))
    return op(v, pltpu.roll(v, 4, 0))


def _dual_softmax(p, z=None):
    n = p.shape[-1]
    p = p.reshape(8, 8, n)
    mx = _pair_allreduce(jnp.max(p, axis=0), jnp.maximum)
    mn = _pair_allreduce(jnp.min(p, axis=0), jnp.minimum)
    ep = jnp.exp2(p - mx[None])
    en = jnp.exp2(mn[None] - p)
    sp = _pair_allreduce(jnp.sum(ep, axis=0), jnp.add)
    sn = _pair_allreduce(jnp.sum(en, axis=0), jnp.add)
    if z is None:
        rp, rn = _recip(sp), _recip(sn)
    else:
        dp = _pair_allreduce(jnp.sum(ep * z[:64].reshape(8, 8, n), axis=0), jnp.add)
        dn = _pair_allreduce(jnp.sum(en * z[64:].reshape(8, 8, n), axis=0), jnp.add)
        rd = _recip(dp * sn + (dn + 1e-6 * sn) * sp)
        rp, rn = sn * rd, sp * rd
    return jnp.concatenate([ep * rp[None], en * rn[None]], axis=0).reshape(LANE, n).astype(BF16)


def _kernel(x_hbm, wqkv_hbm, phi_hbm, wo_hbm, wr_hbm, wg_hbm, wu_hbm, wd_hbm, out_hbm,
            x_buf, xn3, out_buf, wraw, phi_buf, wr_buf, wo_buf, wg_buf, wu_buf, wd_buf,
            wq3, wk3, wv3, phik3, vaug3, zrow, zbuf, phiq3, lmat, o3, r_buf, s_buf, fix_buf, pbuf,
            sem, sem_o):
    def cp(src, dst, slot):
        return pltpu.make_async_copy(src, dst, sem.at[slot])

    def x_rows(r0, n, slot):
        return cp(x_hbm.at[pl.ds(r0, n)], x_buf.at[pl.ds(r0, n)], slot)

    def w_cols(j, g0, g1, slot):
        n = (g1 - g0) * LANE
        return cp(wqkv_hbm.at[:, pl.ds(j * D + g0 * LANE, n)], wraw.at[j, :, pl.ds(g0 * LANE, n)], slot)

    def phi_heads(h0, h1, slot):
        return cp(phi_hbm.at[pl.ds(h0, h1 - h0)], phi_buf.at[pl.ds(h0, h1 - h0)], slot)

    groups = [
        [x_rows(0, T, 0), cp(wr_hbm, wr_buf, 0), phi_heads(0, 8, 0)],
        [w_cols(1, 0, 2, 1)],
        [phi_heads(8, H, 2), w_cols(1, 2, 4, 2)],
        [x_rows(T, T, 3), w_cols(1, 4, 5, 3)],
        [w_cols(1, 5, KB, 4), x_rows(2 * T, T, 4)],
        [w_cols(2, 0, KB, 5)],
        [x_rows(3 * T, S - 3 * T, 6), w_cols(0, 0, KB, 6)],
        [cp(wo_hbm, wo_buf.at[:, pl.ds(0, D)], 7), cp(wg_hbm, wg_buf, 7), cp(wu_hbm, wu_buf, 7),
         cp(wd_hbm, wd_buf.at[:, pl.ds(0, D)], 7)],
    ]
    for grp in groups:
        for c in grp:
            c.start()

    def arrive(k):
        for c in groups[k]:
            c.wait()

    zero = []

    def put_blocks(dst, r0, val):
        n = val.shape[0]
        for k in range(KB):
            blk = val[:, k * LANE:(k + 1) * LANE].astype(BF16)
            if dst.dtype == U32:
                dst[k, r0 // 2:(r0 + n) // 2, :] = _pk(blk)
            else:
                dst[k, r0:r0 + n, :] = blk

    def xn_rows(r0, n, k0=0, k1=KB):
        return _cat([xn3[k, pl.ds(r0, n), :] for k in range(k0, k1)])

    def layernorm(row0, n, ch, chain):
        z = None
        eps = _rb(jnp.full((1, 1), 1e-5, F32))
        for r0 in range(row0, row0 + n, ch):
            xf = x_buf[r0:r0 + ch, :].astype(F32)
            mean = jnp.broadcast_to(jnp.sum(xf, axis=-1, keepdims=True) * (1.0 / D), (ch, LANE))
            if z is not None:
                mean = mean + z
            c = xf - _cat([mean] * KB)
            var = jnp.sum(c * c, axis=-1, keepdims=True) * (1.0 / D)
            rs = _recip_nr(_rb(jnp.sqrt(_rb(_rb(var) + eps))))
            xn = (xf - _cat([_rb(mean)] * KB)) * rs
            put_blocks(xn3, r0, xn)
            if chain == "scale":
                z = jnp.where(rs < 0.0, 1.0, 0.0)
            elif chain == "result":
                u = pltpu.bitcast(xn, U32)
                acc = functools.reduce(jnp.bitwise_or, [u[:, k * LANE:(k + 1) * LANE] for k in range(KB)])
                z = pltpu.bitcast(acc & jnp.concatenate(zero * (ch // 8), axis=0), F32)

    er = lax.broadcasted_iota(jnp.int32, (LANE, DH), 0)
    ec = lax.broadcasted_iota(jnp.int32, (LANE, DH), 1)
    eye4 = jnp.where((er % (2 * DH)) // 2 == ec, 1.0, 0.0).astype(BF16)
    br = lax.broadcasted_iota(jnp.int32, (LANE, LANE), 0)
    bc = lax.broadcasted_iota(jnp.int32, (LANE, LANE), 1)
    bmask = (2 * (br // (2 * DH)) + br % 2) == bc // DH
    bd = {}

    def blockdiag(g0, g1):
        for g in range(g0, g1):
            t = _nt(eye4, phi_buf[4 * g:4 * g + 4].reshape(LANE, DH))
            bd[g] = jnp.where(bmask, t, 0.0).astype(BF16)

    def fold(j, dst, g0, g1):
        for g in range(g0, g1):
            put_blocks(dst, g * LANE, _nt(bd[g], wraw[j, :, g * LANE:(g + 1) * LANE]) * LOG2E)

    pending = []

    def pin(value, lag, off=0):
        pending.append((lag, off, value))

    def lhs(words):
        todo = [(lag - 1, off, value) for lag, off, value in pending]
        pending[:] = [p for p in todo if p[0] > 0]
        for _, off, value in [p for p in todo if p[0] == 0]:
            w = words[0]
            tied = w[off:off + 8] ^ (pltpu.bitcast(value, U32) & zero[0])
            words = [jnp.concatenate(([w[:off]] if off else []) + [tied, w[off + 8:]], axis=0)] + words[1:]
        return _cat([_up(w) for w in words])

    parked = []

    def keys(b, g0=0, g1=KB, park=False):
        r0, r1 = g0 * LANE, g1 * LANE
        re = r1 + RB if g1 == KB else r1
        pt = _nt(lhs([wk3[k, r0 // 2:re // 2, :] for k in range(KB)]), xn_rows(b * LANE, LANE))
        if re > r1:
            r_buf[:, b * LANE:(b + 1) * LANE] = pt[r1 - r0:r1 - r0 + 8, :]
        for j in range(r0 // 64, r1 // 64):
            p = pt[j * 64 - r0:(j + 1) * 64 - r0, :]
            if park and j == r1 // 64 - 1:
                pbuf[len(parked)] = p
                parked.append((b, j))
            else:
                phik3[b, j * LANE:(j + 1) * LANE, :] = _dual_softmax(p)

    def unpark():
        b, j = parked[-1]
        phik3[b, j * LANE:(j + 1) * LANE, :] = _dual_softmax(pbuf[len(parked) - 1])

    def values(b):
        vt = _nt(_cat([_up(wv3[k]) for k in range(KB)]), xn_rows(b * LANE, LANE))
        for j in range(NPAIR):
            vaug3[b, j * VR:j * VR + 2 * DH, :] = vt[j * 2 * DH:(j + 1) * 2 * DH]
            vaug3[b, j * VR + 2 * DH:(j + 1) * VR, :] = jnp.ones((8, LANE), F32)

    ffn_q = []

    def ffn_step(lag, off=0):
        if ffn_q and lag:
            pin(ffn_q.pop(0)(), lag, off)

    def stage_q(i):
        for bl in range(TB):
            pt = _nt(lhs([wq3[k] for k in range(KB)]), xn_rows((i * TB + bl) * LANE, LANE))
            for j in range(NPAIR):
                phiq3[bl, j * LANE:(j + 1) * LANE, :] = _dual_softmax(
                    pt[j * 64:(j + 1) * 64, :], None if i == 0 else zbuf[j])

    def stage_kv():
        lr = lax.broadcasted_iota(jnp.int32, (PR, LANE), 0)
        lc = lax.broadcasted_iota(jnp.int32, (PR, LANE), 1)
        keep = jnp.where(lr < 2 * DH, lr // DH, (lr - 2 * DH) // 8) == lc % 2
        for j in range(NPAIR):
            va = _cat([vaug3[b, j * VR:(j + 1) * VR, :] for b in range(NB)])
            pk = _cat([phik3[b, j * LANE:(j + 1) * LANE, :] for b in range(NB)])
            kvt = _nt(va, pk)
            z = kvt[2 * DH:, :]
            lmat[j] = _pk(jnp.where(keep, jnp.concatenate([kvt, z], axis=0), 0.0).astype(BF16))
            zrow[j] = z

    def stage_b(i, slots):
        for g in range(KB):
            parts = []
            for j in (2 * g, 2 * g + 1):
                pq = _cat([phiq3[bl, j * LANE:(j + 1) * LANE, :] for bl in range(TB)])
                if i == 0:
                    nt = _nn(_up(lmat[j]), pq)
                    for h in range(2):
                        den = nt[2 * DH + 8 * h:2 * DH + 8 * h + 8, :] + 1e-6
                        num = nt[h * DH:(h + 1) * DH, :].reshape(4, 8, T)
                        parts.append((num * _recip(den)[None]).reshape(DH, T))
                else:
                    lw = lmat[j, 0:DH, :]
                    parts.append(_nn(lhs([lw]) if j % 2 == 0 else _up(lw), pq))
            ffn_step(*slots[g])
            o3[g] = _pk(jnp.concatenate(parts, axis=0).T.astype(BF16))

    def stage_c(i, routed=None, mid=None):
        o = [o3[k] for k in range(KB)]
        copies = []

        def project(m, l0, l1):
            before_b = l1 == T and (m == KB - 1 or (mid is not None and m == KB - 3))
            s = _nn(lhs([w[l0 // 2:l1 // 2] for w in o]), wo_buf[:, m * LANE:(m + 1) * LANE])
            ffn_step(4 if before_b else 2)
            return s

        def finish(s, l0, n):
            r0, nr = i * T + l0, s.shape[0]
            cols = slice(n * LANE, (n + 2) * LANE)
            b = xn_rows(r0, nr, n, n + 2).astype(F32)
            if routed is None:
                s_buf[r0:r0 + nr, cols] = s
            else:
                idx, brow = routed()
                sel = (lax.broadcasted_iota(jnp.int32, (nr, 2 * LANE), 0) + r0) == idx
                b = jnp.where(sel, brow[:, cols], b)
            res = x_buf[r0:r0 + nr, cols].astype(F32) + s * _silu(b)
            out_buf[r0:r0 + nr, cols] = res.astype(BF16)
            if routed is not None:
                win = (pl.ds(r0, nr), pl.ds(n * LANE, 2 * LANE))
                copies.append(pltpu.make_async_copy(out_buf.at[win], out_hbm.at[win], sem_o.at[2]))
                copies[-1].start()

        for n in range(0, KB, 2):
            if mid is not None and n == KB - 2:
                mid()
            if routed is not None and n == KB - 2:
                for l0, l1 in ((0, 192), (192, T)):
                    finish(_cat([project(m, l0, l1) for m in (n, n + 1)]), l0, n)
            else:
                finish(_cat([jnp.concatenate([project(m, 0, LANE), project(m, LANE, T)], axis=0)
                             for m in (n, n + 1)]), 0, n)
        r0 = i * T
        if routed is None:
            copies.append(pltpu.make_async_copy(out_buf.at[pl.ds(r0, T)], out_hbm.at[pl.ds(r0, T)], sem_o.at[0]))
            copies[-1].start()
        return copies

    arrive(0)
    layernorm(0, T, LANE, None)
    wrf = wr_buf[...].reshape(1, D).astype(F32)
    for k in range(KB):
        wk3[k, D // 2:(D + RB) // 2, :] = _pk(
            jnp.broadcast_to(wrf[:, k * LANE:(k + 1) * LANE], (RB, LANE)).astype(BF16))
    sign = lax.shift_right_logical(pltpu.bitcast(wrf[:, 0:LANE], jnp.int32), 31)
    zrt = pl.multiple_of(lax.shift_right_logical(jnp.max(sign), 1), 8)
    zero.append(jnp.full((8, LANE), zrt, jnp.int32).astype(U32))
    blockdiag(0, 2)
    arrive(1)
    fold(1, wk3, 0, 2)
    keys(0, 0, 2)
    keys(1, 0, 2, True)
    arrive(2)
    unpark()
    blockdiag(2, KB)
    fold(1, wk3, 2, 4)
    keys(0, 2, 4)
    keys(1, 2, 4, True)
    arrive(3)
    unpark()
    fold(1, wk3, 4, 5)
    keys(0, 4, 5)
    keys(1, 4, 5)
    for b in (2, 3):
        layernorm(b * LANE, LANE, 64, "scale")
        keys(b, 0, 5, b == 3)
    arrive(4)
    unpark()
    fold(1, wk3, 5, KB)
    for b in range(4):
        keys(b, 5, KB, b == 3)
    layernorm(2 * T, T, RB, "result")
    arrive(5)
    unpark()
    for g in range(KB):
        wt = wraw[2, :, g * LANE:(g + 1) * LANE].T
        for k in range(KB):
            wv3[k, g * 64:(g + 1) * 64, :] = _pk(wt[:, k * LANE:(k + 1) * LANE]) ^ jnp.concatenate(zero * 8, axis=0)
    pin(wv3[0, pl.ds(zrt, 8), :], 2, 480)
    for op in PHASE1.split():
        if op == "|":
            arrive(6)
        elif op == "F":
            fold(0, wq3, 0, KB)
        elif op[0] == "L":
            layernorm(int(op[1]) * T, T, RB, "scale")
        else:
            for b in range(int(op[1]) * TB, (int(op[1]) + 1) * TB):
                keys(b) if op[0] == "K" else values(b)
    stage_q(0)
    stage_kv()

    arrive(7)
    r = _rb(r_buf[0:1, :])
    rmax = jnp.max(r)
    pos = lax.broadcasted_iota(jnp.int32, (1, S), 1)
    idx = jnp.clip(jnp.min(jnp.where(r == rmax, pos, S)), 0, S - 1)
    blk = pl.multiple_of((idx // RB) * RB, RB)
    xblk = xn_rows(blk, RB).astype(F32)
    rowsel = (lax.broadcasted_iota(jnp.int32, (RB, D), 0) + blk) == idx
    xs = jnp.broadcast_to(jnp.sum(jnp.where(rowsel, xblk, 0.0), axis=0, keepdims=True), (8, D))
    part, act, y = {}, {}, {}

    def gate_up(w_buf, j, h):
        def f():
            v = _nn(xs[:, h * KH:(h + 1) * KH], w_buf[h * KH:(h + 1) * KH, j * LANE:(j + 1) * LANE])
            key = (w_buf is wu_buf, j)
            part[key] = v if h == 0 else _rb(part[key] + v)
            if h == 1 and w_buf is wu_buf:
                act[j] = _rb(_rb(_silu(part.pop((False, j)))) * part.pop(key))
            return v
        return f

    def down(m, n):
        def f():
            a = _cat([act[j] for j in range(4 * m, 4 * m + 4)])
            v = _nn(a, wd_buf[m * KH:(m + 1) * KH, n * LANE:(n + 1) * LANE])
            y[n] = v if m == 0 else y[n] + v
            return v
        return f

    def routed():
        if "row" not in part:
            rs = _rb(0.5 * jnp.tanh(0.5 * jnp.full((1, 1), rmax, F32)) + 0.5)
            yf = _rb(_rb(_cat([y[n] for n in range(KB)])) * rs)
            part["row"] = _rb(xs + yf)[0:1, :]
        return idx, part["row"]

    sets = []
    for m in range(NG + 1):
        gu = [gate_up(w, j, h) for j in range(4 * m, 4 * m + 4) for w in (wg_buf, wu_buf) for h in range(2)
              ] if m < NG else []
        dn = [down(m - 1, n) for n in range(KB)] if m > 0 else []
        while gu or dn:
            sets += gu[:2] + dn[:1]
            gu, dn = gu[2:], dn[1:]

    for j in range(NPAIR):
        zbuf[j] = jnp.concatenate([zrow[j]] * (LANE // 8), axis=0).T

    b_slots = ((4, 0),) * 5 + ((3, 16), (2, 48))
    outs = []
    for i in range(NTILE - 1):
        stage_b(i, b_slots + ((0, 0),))
        if i == 0:
            ffn_q.extend(sets)
        pin(o3[0, pl.ds(zrt, 8), :], 1, 480)
        stage_q(i + 1)
        ffn_step(2)
        outs += stage_c(i, mid=(lambda: stage_b(NTILE - 1, b_slots + ((2, 0),))) if i == NTILE - 2 else None)
    assert not ffn_q, len(ffn_q)

    sb = pl.multiple_of(jnp.minimum(blk, S - T - RB), RB)
    res = (x_buf[pl.ds(blk, RB), :].astype(F32)
           + s_buf[pl.ds(sb, RB), :] * _silu(jnp.where(rowsel, routed()[1], xblk)))
    fix_buf[...] = res.astype(BF16)

    last = stage_c(NTILE - 1, routed)
    for c in outs:
        c.wait()

    @pl.when(idx < S - T)
    def _():
        c = pltpu.make_async_copy(fix_buf, out_hbm.at[pl.ds(blk, RB)], sem_o.at[1])
        c.start()
        c.wait()

    for c in last:
        c.wait()


def _build():
    any_spec = pl.BlockSpec(memory_space=pl.ANY)
    scratch = [
        pltpu.VMEM((S, D), BF16),
        pltpu.VMEM((KB, S, LANE), BF16),
        pltpu.VMEM((S, D), BF16),
        pltpu.VMEM((3, D, D), BF16),
        pltpu.VMEM((H, DH, DH), BF16),
        pltpu.VMEM((D,), BF16),
        pltpu.VMEM((D, WP), BF16),
        pltpu.VMEM((D, F), BF16),
        pltpu.VMEM((D, F), BF16),
        pltpu.VMEM((F, WP), BF16),
        pltpu.VMEM((KB, D // 2, LANE), U32),
        pltpu.VMEM((KB, (D + RB) // 2, LANE), U32),
        pltpu.VMEM((KB, D // 2, LANE), U32),
        pltpu.VMEM((NB, 2 * D, LANE), BF16),
        pltpu.VMEM((NB, NPAIR * VR, LANE), F32),
        pltpu.VMEM((NPAIR, 8, LANE), F32),
        pltpu.VMEM((NPAIR, LANE, LANE), F32),
        pltpu.VMEM((TB, 2 * D, LANE), BF16),
        pltpu.VMEM((NPAIR, PR // 2, LANE), U32),
        pltpu.VMEM((KB, T // 2, LANE), U32),
        pltpu.VMEM((8, S), F32),
        pltpu.VMEM((S - T, D), F32),
        pltpu.VMEM((RB, D), BF16),
        pltpu.VMEM((4, 64, LANE), F32),
        pltpu.SemaphoreType.DMA((8,)),
        pltpu.SemaphoreType.DMA((3,)),
    ]
    return pl.pallas_call(
        _kernel,
        out_shape=jax.ShapeDtypeStruct((S, D), BF16),
        in_specs=[any_spec] * 8,
        out_specs=any_spec,
        scratch_shapes=scratch,
        compiler_params=pltpu.CompilerParams(vmem_limit_bytes=100 * 1024 * 1024,
                                             disable_semaphore_checks=True),
        name="hedgehog_mod",
    )


@jax.jit
def pallas_recurrent_scan__linear_kernel_hedgehog__moe_arch_mod__prompt_kernel(
    A_x: jax.Array,
    A_wqkv: jax.Array,
    A_w_phi: jax.Array,
    A_wo: jax.Array,
    B_x: jax.Array,
    B_w_r: jax.Array,
    B_w_gate: jax.Array,
    B_w_up: jax.Array,
    B_w_down: jax.Array,
):
    del B_x
    out = _build()(A_x.reshape(S, D), A_wqkv, A_w_phi, A_wo, B_w_r, B_w_gate, B_w_up, B_w_down)
    return out.reshape(1, S, D)
```

```python
import functools

import jax
import jax.numpy as jnp
from jax import lax
import jax.experimental.pallas as pl
import jax.experimental.pallas.tpu as pltpu

S, D, H, DH, F = 2048, 1024, 32, 32, 3584
LANE = 128
KB = D // LANE
KH = D // 2
T = 256
TB = T // LANE
NB = S // LANE
NTILE = S // T
NPAIR = H // 2
VR = 2 * DH + 8
PR = 2 * DH + 16
RB = 16
WP = D + LANE
NG = F // KH
LOG2E = 1.4426950408889634
F32 = jnp.float32
BF16 = jnp.bfloat16
U32 = jnp.uint32

PHASE1 = "K2 V0 V1 | F V2 L3 K3 L4 V3 K4 L5 V4 K5 L6 V5 K6 L7 V6 K7 V7"


def _nt(a, b):
    return lax.dot_general(a, b, (((1,), (1,)), ((), ())), preferred_element_type=F32)


def _nn(a, b):
    return jnp.dot(a, b, preferred_element_type=F32)


def _rb(v):
    return v.astype(BF16).astype(F32)


def _recip(v):
    return pl.reciprocal(v, approx=True)


def _recip_nr(v):
    r = pl.reciprocal(v, approx=True)
    return r * (2.0 - v * r)


def _silu(v):
    return v * (0.5 * jnp.tanh(0.5 * v) + 0.5)


def _cat(parts):
    return jnp.concatenate(parts, axis=1)


def _pk(v):
    return pltpu.bitcast(v, U32)


def _up(v):
    return pltpu.bitcast(v, BF16)


def _pair_allreduce(v, op):
    v = op(v, pltpu.roll(v, 2, 0))
    return op(v, pltpu.roll(v, 4, 0))


def _dual_softmax(p, z=None):
    n = p.shape[-1]
    p = p.reshape(8, 8, n)
    mx = _pair_allreduce(jnp.max(p, axis=0), jnp.maximum)
    mn = _pair_allreduce(jnp.min(p, axis=0), jnp.minimum)
    ep = jnp.exp2(p - mx[None])
    en = jnp.exp2(mn[None] - p)
    sp = _pair_allreduce(jnp.sum(ep, axis=0), jnp.add)
    sn = _pair_allreduce(jnp.sum(en, axis=0), jnp.add)
    if z is None:
        rp, rn = _recip(sp), _recip(sn)
    else:
        dp = _pair_allreduce(jnp.sum(ep * z[:64].reshape(8, 8, n), axis=0), jnp.add)
        dn = _pair_allreduce(jnp.sum(en * z[64:].reshape(8, 8, n), axis=0), jnp.add)
        rd = _recip(dp * sn + (dn + 1e-6 * sn) * sp)
        rp, rn = sn * rd, sp * rd
    return jnp.concatenate([ep * rp[None], en * rn[None]], axis=0).reshape(LANE, n).astype(BF16)


def _kernel(x_hbm, wqkv_hbm, phi_hbm, wo_hbm, wr_hbm, wg_hbm, wu_hbm, wd_hbm, out_hbm,
            x_buf, xn3, out_buf, wraw, phi_buf, wr_buf, wo_buf, wg_buf, wu_buf, wd_buf,
            wq3, wk3, wv3, phik3, vaug3, zrow, zbuf, phiq3, lmat, o3, r_buf, s_buf, fix_buf, pbuf,
            sem, sem_o):
    def cp(src, dst, slot):
        return pltpu.make_async_copy(src, dst, sem.at[slot])

    def x_rows(r0, n, slot):
        return cp(x_hbm.at[pl.ds(r0, n)], x_buf.at[pl.ds(r0, n)], slot)

    def w_cols(j, g0, g1, slot):
        n = (g1 - g0) * LANE
        return cp(wqkv_hbm.at[:, pl.ds(j * D + g0 * LANE, n)], wraw.at[j, :, pl.ds(g0 * LANE, n)], slot)

    def phi_heads(h0, h1, slot):
        return cp(phi_hbm.at[pl.ds(h0, h1 - h0)], phi_buf.at[pl.ds(h0, h1 - h0)], slot)

    groups = [
        [x_rows(0, T, 0), cp(wr_hbm, wr_buf, 0), phi_heads(0, 8, 0)],
        [w_cols(1, 0, 2, 1)],
        [phi_heads(8, H, 2), w_cols(1, 2, 4, 2)],
        [x_rows(T, T, 3), w_cols(1, 4, 5, 3)],
        [w_cols(1, 5, KB, 4), x_rows(2 * T, T, 4)],
        [w_cols(2, 0, KB, 5)],
        [x_rows(3 * T, S - 3 * T, 6), w_cols(0, 0, KB, 6)],
        [cp(wo_hbm, wo_buf.at[:, pl.ds(0, D)], 7), cp(wg_hbm, wg_buf, 7), cp(wu_hbm, wu_buf, 7),
         cp(wd_hbm, wd_buf.at[:, pl.ds(0, D)], 7)],
    ]
    for grp in groups:
        for c in grp:
            c.start()

    def arrive(k):
        for c in groups[k]:
            c.wait()

    zero = []

    def put_blocks(dst, r0, val):
        n = val.shape[0]
        for k in range(KB):
            blk = val[:, k * LANE:(k + 1) * LANE].astype(BF16)
            if dst.dtype == U32:
                dst[k, r0 // 2:(r0 + n) // 2, :] = _pk(blk)
            else:
                dst[k, r0:r0 + n, :] = blk

    def xn_rows(r0, n, k0=0, k1=KB):
        return _cat([xn3[k, pl.ds(r0, n), :] for k in range(k0, k1)])

    def layernorm(row0, n, ch, chain):
        z = None
        eps = _rb(jnp.full((1, 1), 1e-5, F32))
        for r0 in range(row0, row0 + n, ch):
            xf = x_buf[r0:r0 + ch, :].astype(F32)
            mean = jnp.broadcast_to(jnp.sum(xf, axis=-1, keepdims=True) * (1.0 / D), (ch, LANE))
            if z is not None:
                mean = mean + z
            c = xf - _cat([mean] * KB)
            var = jnp.sum(c * c, axis=-1, keepdims=True) * (1.0 / D)
            rs = _recip_nr(_rb(jnp.sqrt(_rb(_rb(var) + eps))))
            xn = (xf - _cat([_rb(mean)] * KB)) * rs
            put_blocks(xn3, r0, xn)
            if chain == "scale":
                z = jnp.where(rs < 0.0, 1.0, 0.0)
            elif chain == "result":
                u = pltpu.bitcast(xn, U32)
                acc = functools.reduce(jnp.bitwise_or, [u[:, k * LANE:(k + 1) * LANE] for k in range(KB)])
                z = pltpu.bitcast(acc & jnp.concatenate(zero * (ch // 8), axis=0), F32)

    er = lax.broadcasted_iota(jnp.int32, (2 * DH, DH), 0)
    ec = lax.broadcasted_iota(jnp.int32, (2 * DH, DH), 1)
    eye2 = jnp.where(er // 2 == ec, 1.0, 0.0).astype(BF16)
    br = lax.broadcasted_iota(jnp.int32, (LANE, LANE), 0)
    bc = lax.broadcasted_iota(jnp.int32, (LANE, LANE), 1)
    bmask = (2 * (br // (2 * DH)) + br % 2) == bc // DH
    bd = {}

    def blockdiag(g0, g1):
        for g in range(g0, g1):
            t = _nt(eye2, phi_buf[4 * g:4 * g + 4].reshape(LANE, DH))
            bd[g] = jnp.where(bmask, jnp.concatenate([t, t], axis=0), 0.0).astype(BF16)

    def fold(j, dst, g0, g1):
        for g in range(g0, g1):
            put_blocks(dst, g * LANE, _nt(bd[g], wraw[j, :, g * LANE:(g + 1) * LANE]) * LOG2E)

    pending = []

    def pin(value, lag, off=0):
        pending.append((lag, off, value))

    def lhs(words):
        todo = [(lag - 1, off, value) for lag, off, value in pending]
        pending[:] = [p for p in todo if p[0] > 0]
        for _, off, value in [p for p in todo if p[0] == 0]:
            w = words[0]
            tied = w[off:off + 8] ^ (pltpu.bitcast(value, U32) & zero[0])
            words = [jnp.concatenate(([w[:off]] if off else []) + [tied, w[off + 8:]], axis=0)] + words[1:]
        return _cat([_up(w) for w in words])

    parked = []

    def keys(b, g0=0, g1=KB, park=False):
        r0, r1 = g0 * LANE, g1 * LANE
        re = r1 + RB if g1 == KB else r1
        pt = _nt(lhs([wk3[k, r0 // 2:re // 2, :] for k in range(KB)]), xn_rows(b * LANE, LANE))
        if re > r1:
            r_buf[:, b * LANE:(b + 1) * LANE] = pt[r1 - r0:r1 - r0 + 8, :]
        for j in range(r0 // 64, r1 // 64):
            p = pt[j * 64 - r0:(j + 1) * 64 - r0, :]
            if park and j == r1 // 64 - 1:
                pbuf[len(parked)] = p
                parked.append((b, j))
            else:
                phik3[b, j * LANE:(j + 1) * LANE, :] = _dual_softmax(p)

    def unpark():
        b, j = parked[-1]
        phik3[b, j * LANE:(j + 1) * LANE, :] = _dual_softmax(pbuf[len(parked) - 1])

    def values(b):
        vt = _nt(_cat([_up(wv3[k]) for k in range(KB)]), xn_rows(b * LANE, LANE))
        for j in range(NPAIR):
            vaug3[b, j * VR:j * VR + 2 * DH, :] = vt[j * 2 * DH:(j + 1) * 2 * DH]
            vaug3[b, j * VR + 2 * DH:(j + 1) * VR, :] = jnp.ones((8, LANE), F32)

    ffn_q = []

    def ffn_step(lag, off=0):
        if ffn_q and lag:
            pin(ffn_q.pop(0)(), lag, off)

    def stage_q(i):
        for bl in range(TB):
            pt = _nt(lhs([wq3[k] for k in range(KB)]), xn_rows((i * TB + bl) * LANE, LANE))
            for j in range(NPAIR):
                phiq3[bl, j * LANE:(j + 1) * LANE, :] = _dual_softmax(
                    pt[j * 64:(j + 1) * 64, :], None if i == 0 else zbuf[j])

    def stage_kv():
        lr = lax.broadcasted_iota(jnp.int32, (PR, LANE), 0)
        lc = lax.broadcasted_iota(jnp.int32, (PR, LANE), 1)
        keep = jnp.where(lr < 2 * DH, lr // DH, (lr - 2 * DH) // 8) == lc % 2
        for j in range(NPAIR):
            va = _cat([vaug3[b, j * VR:(j + 1) * VR, :] for b in range(NB)])
            pk = _cat([phik3[b, j * LANE:(j + 1) * LANE, :] for b in range(NB)])
            kvt = _nt(va, pk)
            z = kvt[2 * DH:, :]
            lmat[j] = _pk(jnp.where(keep, jnp.concatenate([kvt, z], axis=0), 0.0).astype(BF16))
            zrow[j] = z

    def stage_b(i, slots):
        for g in range(KB):
            parts = []
            for j in (2 * g, 2 * g + 1):
                pq = _cat([phiq3[bl, j * LANE:(j + 1) * LANE, :] for bl in range(TB)])
                if i == 0:
                    nt = _nn(_up(lmat[j]), pq)
                    for h in range(2):
                        den = nt[2 * DH + 8 * h:2 * DH + 8 * h + 8, :] + 1e-6
                        num = nt[h * DH:(h + 1) * DH, :].reshape(4, 8, T)
                        parts.append((num * _recip(den)[None]).reshape(DH, T))
                else:
                    lw = lmat[j, 0:DH, :]
                    parts.append(_nn(lhs([lw]) if j % 2 == 0 else _up(lw), pq))
            ffn_step(*slots[g])
            o3[g] = _pk(jnp.concatenate(parts, axis=0).T.astype(BF16))

    def stage_c(i, routed=None, mid=None):
        o = [o3[k] for k in range(KB)]
        copies = []

        def project(m, l0, l1):
            before_b = l1 == T and (m == KB - 1 or (mid is not None and m == KB - 3))
            s = _nn(lhs([w[l0 // 2:l1 // 2] for w in o]), wo_buf[:, m * LANE:(m + 1) * LANE])
            ffn_step(4 if before_b else 2)
            return s

        def finish(s, l0, n):
            r0, nr = i * T + l0, s.shape[0]
            cols = slice(n * LANE, (n + 2) * LANE)
            b = xn_rows(r0, nr, n, n + 2).astype(F32)
            if routed is None:
                s_buf[r0:r0 + nr, cols] = s
            else:
                idx, brow = routed()
                sel = (lax.broadcasted_iota(jnp.int32, (nr, 2 * LANE), 0) + r0) == idx
                b = jnp.where(sel, brow[:, cols], b)
            res = x_buf[r0:r0 + nr, cols].astype(F32) + s * _silu(b)
            out_buf[r0:r0 + nr, cols] = res.astype(BF16)
            if routed is not None:
                win = (pl.ds(r0, nr), pl.ds(n * LANE, 2 * LANE))
                copies.append(pltpu.make_async_copy(out_buf.at[win], out_hbm.at[win], sem_o.at[2]))
                copies[-1].start()

        for n in range(0, KB, 2):
            if mid is not None and n == KB - 2:
                mid()
            if routed is not None and n == KB - 2:
                for l0, l1 in ((0, 192), (192, T)):
                    finish(_cat([project(m, l0, l1) for m in (n, n + 1)]), l0, n)
            else:
                finish(_cat([jnp.concatenate([project(m, 0, LANE), project(m, LANE, T)], axis=0)
                             for m in (n, n + 1)]), 0, n)
        r0 = i * T
        if routed is None:
            copies.append(pltpu.make_async_copy(out_buf.at[pl.ds(r0, T)], out_hbm.at[pl.ds(r0, T)], sem_o.at[0]))
            copies[-1].start()
        return copies

    arrive(0)
    layernorm(0, T, LANE, None)
    wrf = wr_buf[...].reshape(1, D).astype(F32)
    for k in range(KB):
        wk3[k, D // 2:(D + RB) // 2, :] = _pk(
            jnp.broadcast_to(wrf[:, k * LANE:(k + 1) * LANE], (RB, LANE)).astype(BF16))
    sign = lax.shift_right_logical(pltpu.bitcast(wrf[:, 0:LANE], jnp.int32), 31)
    zrt = pl.multiple_of(jnp.clip(lax.shift_right_logical(jnp.max(sign), 1), 0, 1) * 8, 8)
    zero.append(jnp.full((8, LANE), zrt, jnp.int32).astype(U32))
    blockdiag(0, 2)
    arrive(1)
    fold(1, wk3, 0, 2)
    keys(0, 0, 2)
    keys(1, 0, 2, True)
    arrive(2)
    unpark()
    blockdiag(2, KB)
    fold(1, wk3, 2, 4)
    keys(0, 2, 4)
    keys(1, 2, 4, True)
    arrive(3)
    unpark()
    fold(1, wk3, 4, 5)
    keys(0, 4, 5)
    keys(1, 4, 5)
    for b in (2, 3):
        layernorm(b * LANE, LANE, 64, "scale")
        keys(b, 0, 5, b == 3)
    arrive(4)
    unpark()
    fold(1, wk3, 5, KB)
    for b in range(4):
        keys(b, 5, KB, b == 3)
    layernorm(2 * T, T, RB, "result")
    arrive(5)
    unpark()
    for g in range(KB):
        wt = wraw[2, :, g * LANE:(g + 1) * LANE].T
        for k in range(KB):
            wv3[k, g * 64:(g + 1) * 64, :] = _pk(wt[:, k * LANE:(k + 1) * LANE]) ^ jnp.concatenate(zero * 8, axis=0)
    pin(wv3[0, pl.ds(zrt, 8), :], 2, 480)
    for op in PHASE1.split():
        if op == "|":
            arrive(6)
        elif op == "F":
            fold(0, wq3, 0, KB)
        elif op[0] == "L":
            layernorm(int(op[1]) * T, T, RB, "scale")
        else:
            for b in range(int(op[1]) * TB, (int(op[1]) + 1) * TB):
                keys(b) if op[0] == "K" else values(b)
    stage_q(0)
    stage_kv()

    arrive(7)
    r = _rb(r_buf[0:1, :])
    rmax = jnp.max(r)
    pos = lax.broadcasted_iota(jnp.int32, (1, S), 1)
    idx = jnp.clip(jnp.min(jnp.where(r == rmax, pos, S)), 0, S - 1)
    blk = pl.multiple_of((idx // RB) * RB, RB)
    xblk = xn_rows(blk, RB).astype(F32)
    rowsel = (lax.broadcasted_iota(jnp.int32, (RB, D), 0) + blk) == idx
    xs = jnp.broadcast_to(jnp.sum(jnp.where(rowsel, xblk, 0.0), axis=0, keepdims=True), (8, D))
    part, act, y = {}, {}, {}

    def gate_up(w_buf, j, h):
        def f():
            v = _nn(xs[:, h * KH:(h + 1) * KH], w_buf[h * KH:(h + 1) * KH, j * LANE:(j + 1) * LANE])
            key = (w_buf is wu_buf, j)
            part[key] = v if h == 0 else _rb(part[key] + v)
            if h == 1 and w_buf is wu_buf:
                act[j] = _rb(_rb(_silu(part.pop((False, j)))) * part.pop(key))
            return v
        return f

    def down(m, n):
        def f():
            a = _cat([act[j] for j in range(4 * m, 4 * m + 4)])
            v = _nn(a, wd_buf[m * KH:(m + 1) * KH, n * LANE:(n + 1) * LANE])
            y[n] = v if m == 0 else y[n] + v
            return v
        return f

    def routed():
        if "row" not in part:
            rs = _rb(0.5 * jnp.tanh(0.5 * jnp.full((1, 1), rmax, F32)) + 0.5)
            yf = _rb(_rb(_cat([y[n] for n in range(KB)])) * rs)
            part["row"] = _rb(xs + yf)[0:1, :]
        return idx, part["row"]

    sets = []
    for m in range(NG + 1):
        gu = [gate_up(w, j, h) for j in range(4 * m, 4 * m + 4) for w in (wg_buf, wu_buf) for h in range(2)
              ] if m < NG else []
        dn = [down(m - 1, n) for n in range(KB)] if m > 0 else []
        while gu or dn:
            sets += gu[:2] + dn[:1]
            gu, dn = gu[2:], dn[1:]

    for j in range(NPAIR):
        zbuf[j] = jnp.concatenate([zrow[j]] * (LANE // 8), axis=0).T

    b_slots = ((4, 0),) * 5 + ((3, 16), (2, 48))
    outs = []
    for i in range(NTILE - 1):
        stage_b(i, b_slots + ((0, 0),))
        if i == 0:
            ffn_q.extend(sets)
        pin(o3[0, pl.ds(zrt, 8), :], 1, 480)
        stage_q(i + 1)
        ffn_step(2)
        outs += stage_c(i, mid=(lambda: stage_b(NTILE - 1, b_slots + ((2, 0),))) if i == NTILE - 2 else None)
    assert not ffn_q, len(ffn_q)

    sb = pl.multiple_of(jnp.minimum(blk, S - T - RB), RB)
    res = (x_buf[pl.ds(blk, RB), :].astype(F32)
           + s_buf[pl.ds(sb, RB), :] * _silu(jnp.where(rowsel, routed()[1], xblk)))
    fix_buf[...] = res.astype(BF16)

    last = stage_c(NTILE - 1, routed)
    for c in outs:
        c.wait()

    @pl.when(idx < S - T)
    def _():
        c = pltpu.make_async_copy(fix_buf, out_hbm.at[pl.ds(blk, RB)], sem_o.at[1])
        c.start()
        c.wait()

    for c in last:
        c.wait()


def _build():
    any_spec = pl.BlockSpec(memory_space=pl.ANY)
    scratch = [
        pltpu.VMEM((S, D), BF16),
        pltpu.VMEM((KB, S, LANE), BF16),
        pltpu.VMEM((S, D), BF16),
        pltpu.VMEM((3, D, D), BF16),
        pltpu.VMEM((H, DH, DH), BF16),
        pltpu.VMEM((D,), BF16),
        pltpu.VMEM((D, WP), BF16),
        pltpu.VMEM((D, F), BF16),
        pltpu.VMEM((D, F), BF16),
        pltpu.VMEM((F, WP), BF16),
        pltpu.VMEM((KB, D // 2, LANE), U32),
        pltpu.VMEM((KB, (D + RB) // 2, LANE), U32),
        pltpu.VMEM((KB, D // 2, LANE), U32),
        pltpu.VMEM((NB, 2 * D, LANE), BF16),
        pltpu.VMEM((NB, NPAIR * VR, LANE), F32),
        pltpu.VMEM((NPAIR, 8, LANE), F32),
        pltpu.VMEM((NPAIR, LANE, LANE), F32),
        pltpu.VMEM((TB, 2 * D, LANE), BF16),
        pltpu.VMEM((NPAIR, PR // 2, LANE), U32),
        pltpu.VMEM((KB, T // 2, LANE), U32),
        pltpu.VMEM((8, S), F32),
        pltpu.VMEM((S - T, D), F32),
        pltpu.VMEM((RB, D), BF16),
        pltpu.VMEM((4, 64, LANE), F32),
        pltpu.SemaphoreType.DMA((8,)),
        pltpu.SemaphoreType.DMA((3,)),
    ]
    return pl.pallas_call(
        _kernel,
        out_shape=jax.ShapeDtypeStruct((S, D), BF16),
        in_specs=[any_spec] * 8,
        out_specs=any_spec,
        scratch_shapes=scratch,
        compiler_params=pltpu.CompilerParams(vmem_limit_bytes=100 * 1024 * 1024,
                                             disable_semaphore_checks=True),
        name="hedgehog_mod",
    )


@jax.jit
def pallas_recurrent_scan__linear_kernel_hedgehog__moe_arch_mod__prompt_kernel(
    A_x: jax.Array,
    A_wqkv: jax.Array,
    A_w_phi: jax.Array,
    A_wo: jax.Array,
    B_x: jax.Array,
    B_w_r: jax.Array,
    B_w_gate: jax.Array,
    B_w_up: jax.Array,
    B_w_down: jax.Array,
):
    del B_x
    out = _build()(A_x.reshape(S, D), A_wqkv, A_w_phi, A_wo, B_w_r, B_w_gate, B_w_up, B_w_down)
    return out.reshape(1, S, D)
```
